```python
import jax
import jax.numpy as jnp

def _softmax(x, axis=-1):
    return jax.nn.softmax(x, axis=axis)
def _gelu(x):
    return jax.nn.gelu(x, approximate=True)
def _silu(x):
    return jax.nn.silu(x)
def _sigmoid(x):
    return jax.nn.sigmoid(x)
def _layernorm(x, axis=-1, eps=1e-5):
    m = jnp.mean(x, axis=axis, keepdims=True)
    v = jnp.var(x, axis=axis, keepdims=True)
    return (x - m) / jnp.sqrt(v + eps)
def _scatter_add(tgt, idx, src, axis=0):
    return tgt.at[idx].add(src)
def _segment_sum(src, seg, n):
    return jax.ops.segment_sum(src, seg, n)
class _Rng:
    def __init__(self, key):
        self._k = key
    def _next(self):
        self._k, sub = jax.random.split(self._k)
        return sub
    def normal(self, shape):
        return jax.random.normal(self._next(), shape, dtype=jnp.bfloat16)
    def randint(self, lo, hi, shape):
        return jax.random.randint(self._next(), shape, lo, hi, dtype=jnp.int32)
    def uniform(self, shape, lo=0.0, hi=1.0):
        return jax.random.uniform(self._next(), shape, jnp.bfloat16, lo, hi)
    def permutation(self, n):
        return jax.random.permutation(self._next(), n)


kernel_name = 'interleave_layers__ssm_conv_s5__ssm_conv_h3__prompt'

def setup_inputs():
    _rng = _Rng(jax.random.key(int.from_bytes(__import__("os").urandom(4), "little")))
    _w = (lambda a: (lambda t: t.astype(jnp.bfloat16) if jnp.issubdtype(t.dtype, jnp.floating) else t)(jnp.asarray(a)))
    def _A_setup():
        B, S, D = 1, 2048, 640
        P = D
        Lambda_re = -0.5 * jnp.exp((lambda *s: _rng.normal(s) * 0.05)(P))
        Lambda_im = (lambda *s: _rng.normal(s) * 0.05)(P) * 1.0
        B_re = (lambda *s: _rng.normal(s) * 0.05)(P, D) * (D ** -0.5)
        B_im = (lambda *s: _rng.normal(s) * 0.05)(P, D) * (D ** -0.5)
        C_re = (lambda *s: _rng.normal(s) * 0.05)(D, P) * (P ** -0.5)
        C_im = (lambda *s: _rng.normal(s) * 0.05)(D, P) * (P ** -0.5)
        log_dt = (lambda *s: _rng.normal(s) * 0.05)(P) * 0.3 - 2.0
        Dskip = (lambda *s: _rng.normal(s) * 0.05)(D)
        return {
            "x": _w((lambda *s: _rng.normal(s) * 0.05)(B, S, D)),
            "Lambda_re": _w(Lambda_re),
            "Lambda_im": _w(Lambda_im),
            "B_re": _w(B_re),
            "B_im": _w(B_im),
            "C_re": _w(C_re),
            "C_im": _w(C_im),
            "log_dt": _w(log_dt),
            "Dskip": _w(Dskip),
        }
    _A_in = _A_setup()

    def _B_setup():
        B, S, D = 1, 2048, 640
        ks = 4
        return {
            "q": _w((lambda *s: _rng.normal(s) * 0.05)(B, S, D)),
            "k": _w((lambda *s: _rng.normal(s) * 0.05)(B, S, D)),
            "v": _w((lambda *s: _rng.normal(s) * 0.05)(B, S, D)),
            "shift_k": _w((lambda *s: _rng.normal(s) * 0.05)(D, ks) * 0.5),
            "ssm_k": _w((lambda *s: _rng.normal(s) * 0.05)(D, S) * (1.0 / S ** 0.5)),
            "ssm_D": _w((lambda *s: _rng.normal(s) * 0.05)(D)),
        }
    _B_in = _B_setup()

    return {
        "A_x": _A_in["x"],
        "A_Lambda_re": _A_in["Lambda_re"],
        "A_Lambda_im": _A_in["Lambda_im"],
        "A_B_re": _A_in["B_re"],
        "A_B_im": _A_in["B_im"],
        "A_C_re": _A_in["C_re"],
        "A_C_im": _A_in["C_im"],
        "A_log_dt": _A_in["log_dt"],
        "A_Dskip": _A_in["Dskip"],
        "B_q": _B_in["q"],
        "B_k": _B_in["k"],
        "B_v": _B_in["v"],
        "B_shift_k": _B_in["shift_k"],
        "B_ssm_k": _B_in["ssm_k"],
        "B_ssm_D": _B_in["ssm_D"],
    }

def reference(A_x, A_Lambda_re, A_Lambda_im, A_B_re, A_B_im, A_C_re, A_C_im, A_log_dt, A_Dskip, B_q, B_k, B_v, B_shift_k, B_ssm_k, B_ssm_D):
    def _A_ref(x, Lambda_re, Lambda_im, B_re, B_im, C_re, C_im, log_dt, Dskip):
        Bsz, L, H = x.shape
        Lam = Lambda_re + 1j * Lambda_im
        Bmat = B_re + 1j * B_im
        Cmat = C_re + 1j * C_im
        dt = jnp.exp(log_dt)
        Lam_bar = jnp.exp(dt * Lam)
        B_bar = ((Lam_bar - 1.0) / Lam)[:, None] * Bmat
        Bu = jnp.einsum("bld,pd->blp", x + 0j, B_bar)
        h = jnp.zeros_like(Bu[:, 0, :])
        hs = []
        for t in range(L):
            h = Lam_bar[None, :] * h + Bu[:, t, :]
            hs.append(h)
        hseq = jnp.stack(hs, 1)
        y = 2.0 * jnp.einsum("blp,dp->bld", hseq, Cmat).real + x * Dskip[None, None, :]
        return y

    def _B_ref(q, k, v, shift_k, ssm_k, ssm_D):
        B, S, D = q.shape
        ks = shift_k.shape[-1]
        k_pad = jnp.pad(k, ((0, 0), (ks - 1, 0), (0, 0)))
        k_shift = jnp.zeros_like(k)
        for t in range(ks):
            k_shift = k_shift + k_pad[:, t:t + S, :] * shift_k[:, ks - 1 - t][None, None, :]
        kv = k_shift * v
        L = 2 * S
        kv_pad = jnp.pad(kv, ((0, 0), (0, S), (0, 0)))
        kf_pad = jnp.pad(ssm_k, ((0, 0), (0, S)))
        kv_f = (lambda x, axes=(-2,-1): jnp.fft.rfft2(x.astype(jnp.float32), axes=axes))(kv_pad[:, None, :, :], axes=(1, 2))
        kf_f = (lambda x, axes=(-2,-1): jnp.fft.rfft2(x.astype(jnp.float32), axes=axes))(kf_pad[:, None, :], axes=(1, 2))
        kf_f = (lambda x, *d: x.transpose(*d))(kf_f, 1, 2, 0)
        y_f = kv_f * kf_f[None, :, :, :]
        y = (lambda x, s, axes=(-2,-1): jnp.fft.irfft2(x, s=s, axes=axes).astype(jnp.bfloat16))(y_f, (1, L), axes=(1, 2))[:, 0, :S, :]
        y = y + kv * ssm_D[None, None, :]
        return q * y

    x = A_x
    x = x + _A_ref(_layernorm(x, axis=-1), A_Lambda_re, A_Lambda_im, A_B_re, A_B_im, A_C_re, A_C_im, A_log_dt, A_Dskip)
    x = x + _B_ref(_layernorm(x, axis=-1), B_k, B_v, B_shift_k, B_ssm_k, B_ssm_D)
    x = x + _A_ref(_layernorm(x, axis=-1), A_Lambda_re, A_Lambda_im, A_B_re, A_B_im, A_C_re, A_C_im, A_log_dt, A_Dskip)
    x = x + _B_ref(_layernorm(x, axis=-1), B_k, B_v, B_shift_k, B_ssm_k, B_ssm_D)
    return x
```

```python
import numpy as np
import jax
import jax.numpy as jnp
import jax.experimental.pallas as pl
import jax.experimental.pallas.tpu as pltpu

S, D = 2048, 640
NT = D // 128
TS = 32
T = 8 * TS
NCH = S // T
PITCH = TS + 1
PADR = 304
NFFT = 4096
NK1 = 33
C8 = float(np.sqrt(0.5))
F32 = jnp.float32
BF16 = jnp.bfloat16


class _Bfly:
    def __init__(self):
        self.tab = {}
        self.keep = []

    def _plus(self, va, vb):
        key = ('+',) + tuple(sorted((id(va), id(vb))))
        if key not in self.tab:
            self.tab[key] = va + vb
            self.keep.append((va, vb))
        return self.tab[key]

    def _minus(self, va, vb):
        k1 = ('-', id(va), id(vb))
        k2 = ('-', id(vb), id(va))
        if k1 in self.tab:
            return (1, self.tab[k1])
        if k2 in self.tab:
            return (-1, self.tab[k2])
        self.tab[k1] = va - vb
        self.keep.append((va, vb))
        return (1, self.tab[k1])

    def _times(self, va, c):
        key = ('*', id(va), c)
        if key not in self.tab:
            self.tab[key] = va * c
            self.keep.append(va)
        return self.tab[key]

    def radd(self, a, b):
        if a is None:
            return b
        if b is None:
            return a
        sa, va = a
        sb, vb = b
        if sa == sb:
            return (sa, self._plus(va, vb))
        s, v = self._minus(va, vb)
        return (s * sa, v)

    @staticmethod
    def rneg(a):
        return None if a is None else (-a[0], a[1])

    def rsub(self, a, b):
        return self.radd(a, self.rneg(b))

    def rmul(self, a, c):
        if a is None or c == 0.0:
            return None
        s = 1 if c > 0 else -1
        c = abs(c)
        if c == 1.0:
            return (a[0] * s, a[1])
        return (a[0] * s, self._times(a[1], c))

    def cadd(self, a, b):
        return (self.radd(a[0], b[0]), self.radd(a[1], b[1]))

    def csub(self, a, b):
        return (self.rsub(a[0], b[0]), self.rsub(a[1], b[1]))

    def cconj(self, a):
        return (a[0], self.rneg(a[1]))

    def cmuli(self, a, p):
        p %= 4
        if p == 0:
            return a
        if p == 1:
            return (self.rneg(a[1]), a[0])
        if p == 2:
            return (self.rneg(a[0]), self.rneg(a[1]))
        return (a[1], self.rneg(a[0]))

    def cmul_w(self, a, num, den):
        num %= den
        if (4 * num) % den == 0:
            return self.cmuli(a, 4 * num // den)
        if (8 * num) % den == 0:
            o = 8 * num // den
            re = self.rmul(self.rsub(a[0], a[1]), C8)
            im = self.rmul(self.radd(a[0], a[1]), C8)
            return self.cmuli((re, im), (o - 1) // 2)
        wr = float(np.cos(2 * np.pi * num / den))
        wi = float(np.sin(2 * np.pi * num / den))
        re = self.rsub(self.rmul(a[0], wr), self.rmul(a[1], wi))
        im = self.radd(self.rmul(a[0], wi), self.rmul(a[1], wr))
        return (re, im)

    def re_mul_w(self, a, num, den):
        num %= den
        if (4 * num) % den == 0:
            return self.cmuli(a, 4 * num // den)[0]
        if (8 * num) % den == 0:
            o = 8 * num // den
            a2 = self.cmuli(a, (o - 1) // 2)
            return self.rmul(self.rsub(a2[0], a2[1]), C8)
        wr = float(np.cos(2 * np.pi * num / den))
        wi = float(np.sin(2 * np.pi * num / den))
        return self.rsub(self.rmul(a[0], wr), self.rmul(a[1], wi))

    def fft4(self, x, sgn):
        a = self.cadd(x[0], x[2])
        b = self.csub(x[0], x[2])
        c = self.cadd(x[1], x[3])
        d = self.csub(x[1], x[3])
        wd = self.cmuli(d, sgn)
        return [self.cadd(a, c), self.cadd(b, wd), self.csub(a, c), self.csub(b, wd)]

    def fft8(self, x, sgn, want=range(8)):
        e = self.fft4(x[0::2], sgn)
        o = self.fft4(x[1::2], sgn)
        y = [None] * 8
        want = set(want)
        for k in range(4):
            if k not in want and (k + 4) not in want:
                continue
            t = self.cmul_w(o[k], sgn * k, 8)
            if k in want:
                y[k] = self.cadd(e[k], t)
            if k + 4 in want:
                y[k + 4] = self.csub(e[k], t)
        return y

    def fft8_re(self, x, sgn):
        e = self.fft4(x[0::2], sgn)
        o = self.fft4(x[1::2], sgn)
        y = [None] * 8
        for k in range(4):
            t = self.re_mul_w(o[k], sgn * k, 8)
            y[k] = self.radd(e[k][0], t)
            y[k + 4] = self.rsub(e[k][0], t)
        return y

    def fwd64(self, x):
        Z = (None, None)
        xr = [((1, v), None) for v in x]
        A = {}
        for b2 in range(8):
            ins = [xr[8 * b1 + b2] for b1 in range(4)] + [Z] * 4
            y = self.fft8(ins, -1, want=range(5))
            for k in range(5):
                A[(k, b2)] = y[k]
        Y = {}
        for k1 in range(5):
            tw = [self.cmul_w(A[(k1, b2)], -k1 * b2, 64) for b2 in range(8)]
            want = range(5) if k1 == 0 else (range(4) if k1 == 4 else range(8))
            y = self.fft8(tw, -1, want=want)
            for k2 in want:
                k = k1 + 8 * k2
                if k <= 32:
                    Y[k] = y[k2]
                else:
                    Y[64 - k] = self.cconj(y[k2])
        return Y

    def inv64(self, V):
        Z = (None, None)
        Tm = {}
        for k1 in (1, 2, 3):
            ins = [V[k1 + 8 * k2] for k2 in range(4)] + [
                self.cconj(V[(8 - k1) + 8 * (7 - k2)]) for k2 in range(4, 8)]
            y = self.fft8(ins, +1)
            for b2 in range(8):
                Tm[(k1, b2)] = self.cmul_w(y[b2], k1 * b2, 64)
        ins = [V[8 * k2] for k2 in range(5)] + [Z] * 3
        t0 = self.fft8_re(ins, +1)
        ins = [V[4 + 8 * k2] for k2 in range(4)] + [Z] * 4
        y4 = self.fft8(ins, +1)
        t4 = [self.re_mul_w(y4[b2], 4 * b2, 64) for b2 in range(8)]
        out = [None] * 32
        for b2 in range(8):
            T1, T2, T3 = Tm[(1, b2)], Tm[(2, b2)], Tm[(3, b2)]
            sp = self.radd(t0[b2], t4[b2])
            sm = self.rsub(t0[b2], t4[b2])
            out[b2] = self.radd(self.radd(sp, T2[0]), self.radd(T1[0], T3[0]))
            out[16 + b2] = self.radd(self.rsub(sp, T2[0]), self.rsub(T3[1], T1[1]))
            p = self.rsub(T1[0], T3[0])
            q = self.radd(T1[1], T3[1])
            out[8 + b2] = self.radd(self.rsub(sm, T2[1]), self.rmul(self.rsub(p, q), C8))
            out[24 + b2] = self.rsub(self.radd(sm, T2[1]), self.rmul(self.radd(p, q), C8))
        return out


def _fwd_signs():
    bf = _Bfly()
    Y = bf.fwd64([np.full((1,), float(i + 1) ** 1.37) for i in range(32)])
    sg = {}
    for k in range(NK1):
        sg[k] = tuple(0 if c is None else c[0] for c in Y[k])
    return sg


_FSG = _fwd_signs()


def _dft_matrices():
    r = np.arange(64)
    k2 = np.arange(64)
    Fm = np.zeros((NK1, 128, 128), np.float64)
    Gm = np.zeros((NK1, 128, 128), np.float64)
    col = (16 * (r // 8) + (r % 8))
    for k1 in range(NK1):
        th = 2 * np.pi * np.outer(k1 + 64 * k2, r) / NFFT
        c, s = np.cos(th), np.sin(th)
        sr, si = _FSG[k1]
        if k1 == 0:
            Fm[k1][0:64][:, col] = c * sr
            Fm[k1][64:128][:, col] = -s * sr
        elif k1 == 32:
            Fm[k1][0:64][:, col + 8] = c * sr
            Fm[k1][64:128][:, col + 8] = -s * sr
        else:
            Fm[k1][0:64][:, col] = c * sr
            Fm[k1][0:64][:, col + 8] = s * si
            Fm[k1][64:128][:, col] = -s * sr
            Fm[k1][64:128][:, col + 8] = c * si
        sc = (1.0 if k1 in (0, 32) else 2.0) / NFFT
        ct, st = c.T * sc, s.T * sc
        Gm[k1][0:64][:, col] = ct
        Gm[k1][0:64][:, col + 8] = -st
        Gm[k1][64:128][:, col] = st
        Gm[k1][64:128][:, col + 8] = ct
    return Fm.astype(np.float32).astype(jnp.bfloat16), Gm.astype(np.float32).astype(jnp.bfloat16)


_FM, _GM = _dft_matrices()


def _cmul(ar, ai, br, bi):
    return ar * br - ai * bi, ar * bi + ai * br


def _cmul_add(lr, li, hr, hi, ur, ui):
    return (lr * hr - li * hi) + ur, (lr * hi + li * hr) + ui


def _layernorm(x):
    m = jnp.mean(x, axis=-1, keepdims=True)
    xc = x - m
    v = jnp.mean(xc * xc, axis=-1, keepdims=True)
    return xc * jax.lax.rsqrt(v + 1e-5)


def _nt_dot(a, b):
    return jax.lax.dot_general(a, b, (((1,), (1,)), ((), ())), preferred_element_type=F32)


def _kernel(lre_ref, lim_ref, ldt_ref, dsk_ref, shk_ref, sD_ref,
            x_hbm, bre_hbm, bim_hbm, cre_hbm, cim_hbm, k_hbm, v_hbm, sk_hbm, f_hbm, g_hbm,
            o_hbm,
            xin, bw, cst, cw, tab, par, carry, kin, vin, skin, fm, gm,
            kf, vf, skt, ybf, vscr, yscr, x1, pad, ostg,
            sem_x, sem_w, sem_kv, sem_fg, sem_o):

    def cp_x(c):
        return pltpu.make_async_copy(x_hbm.at[pl.ds(T * c, T), :], xin.at[pl.ds(T * c, T), :], sem_x.at[c])

    def cp_w(n, which):
        src = (bre_hbm, bim_hbm, cre_hbm, cim_hbm)[which]
        if which < 2:
            return pltpu.make_async_copy(src.at[pl.ds(128 * n, 128), :],
                                         bw.at[pl.ds(256 * n + 128 * which, 128), :], sem_w.at[4 * n + which])
        return pltpu.make_async_copy(src.at[:, pl.ds(128 * n, 128)],
                                     cst.at[which - 2, :, pl.ds(128 * n, 128)], sem_w.at[4 * n + which])

    def cp_kv(c, which):
        if which == 0:
            return pltpu.make_async_copy(k_hbm.at[:, pl.ds(128 * c, 128)], kin.at[c], sem_kv.at[3 * c])
        if which == 1:
            return pltpu.make_async_copy(v_hbm.at[:, pl.ds(128 * c, 128)], vin.at[c], sem_kv.at[3 * c + 1])
        return pltpu.make_async_copy(sk_hbm.at[pl.ds(128 * c, 128), :], skin.at[c], sem_kv.at[3 * c + 2])

    cp_f = pltpu.make_async_copy(f_hbm, fm, sem_fg.at[0])
    cp_g = pltpu.make_async_copy(g_hbm, gm, sem_fg.at[1])

    def cp_o(c):
        return pltpu.make_async_copy(ostg.at[c % 2], o_hbm.at[pl.ds(T * c, T), :], sem_o.at[c % 2])

    cp_x(0).start()
    for n in range(NT):
        cp_w(n, 0).start()
        cp_w(n, 1).start()
    for n in range(NT):
        cp_w(n, 2).start()
        cp_w(n, 3).start()
    for c in range(1, NCH):
        cp_x(c).start()
    cp_f.start()
    cp_g.start()
    for c in range(NT):
        for w in range(3):
            cp_kv(c, w).start()

    def row(ref):
        return ref[...].astype(F32)[None, :]

    lre, lim, ldt = row(lre_ref), row(lim_ref), row(ldt_ref)
    dt = jnp.exp(ldt).astype(BF16).astype(F32)
    zr, zi = dt * lre, dt * lim
    mag = jnp.exp(zr)
    lbr, lbi = mag * jnp.cos(zi), mag * jnp.sin(zi)
    inv = 1.0 / (lre * lre + lim * lim)
    nr, ni = lbr - 1.0, lbi
    fr, fi = (nr * lre + ni * lim) * inv, (ni * lre - nr * lim) * inv
    sub = jax.lax.broadcasted_iota(jnp.int32, (8, D), 0)

    def b8(v):
        return jnp.broadcast_to(v, (8, D))

    tab[0] = b8(lbr)
    tab[1] = b8(lbi)
    pr, pi = lbr, lbi
    for _ in range(5):
        pr, pi = _cmul(pr, pi, pr, pi)
    tab[2] = b8(pr)
    tab[3] = b8(pi)
    for q, sh in enumerate((1, 2, 4)):
        tab[4 + 2 * q] = jnp.where(sub >= sh, b8(pr), 0.0)
        tab[5 + 2 * q] = jnp.where(sub >= sh, b8(pi), 0.0)
        pr, pi = _cmul(pr, pi, pr, pi)
    par[0] = b8(row(dsk_ref))
    par[1] = b8(row(sD_ref))
    shk = shk_ref[...].astype(F32)
    for lag in range(4):
        par[2 + lag] = b8(shk[lag:lag + 1, :])
    carry[...] = jnp.zeros(carry.shape, F32)

    def conv_tile(c):
        ls = slice(128 * c, 128 * (c + 1))
        for w in range(3):
            cp_kv(c, w).wait()
        kf[0:8, :] = jnp.zeros((8, 128), F32)
        kf[8:8 + S, :] = kin[c].astype(F32)
        vf[...] = vin[c].astype(F32)
        skt[...] = skin[c].astype(F32).T
        w = [par[2 + lag, :, ls] for lag in range(4)]
        for rho in range(8):
            for sig in range(2):
                xs = []
                for b in range(32):
                    t0 = 64 * b + 8 * rho
                    if sig == 0:
                        acc = kf[pl.ds(8 + t0 - 3, 8), :] * w[3]
                        acc = acc + kf[pl.ds(8 + t0 - 2, 8), :] * w[2]
                        acc = acc + kf[pl.ds(8 + t0 - 1, 8), :] * w[1]
                        acc = acc + kf[pl.ds(8 + t0, 8), :] * w[0]
                        xs.append(acc * vf[pl.ds(t0, 8), :])
                    else:
                        xs.append(skt[pl.ds(t0, 8), :])
                bf = _Bfly()
                Y = bf.fwd64(xs)
                for k1 in range(32):
                    if k1 == 0:
                        a, b_ = Y[0][0], Y[32][0]
                    else:
                        a, b_ = Y[k1]
                    pk = jnp.concatenate([a[1], b_[1]], axis=0).astype(BF16)
                    ybf[k1, pl.ds(16 * rho, 16), pl.ds(128 * sig, 128)] = pk
        dD = par[1, :, ls]
        for k1 in range(NK1):
            z = jnp.dot(fm[k1], ybf[k1 % 32], preferred_element_type=F32)
            parts = []
            for g in range(8):
                ur = z[8 * g:8 * g + 8, 0:128]
                ui = z[64 + 8 * g:64 + 8 * g + 8, 0:128]
                kr = z[8 * g:8 * g + 8, 128:256] + dD
                ki = z[64 + 8 * g:64 + 8 * g + 8, 128:256]
                pr_, pi_ = _cmul(ur, ui, kr, ki)
                parts += [pr_, pi_]
            p = jnp.concatenate(parts, axis=0).astype(BF16)
            if k1 in (0, 32):
                vscr[k1, 0:64, :] = jnp.dot(gm[k1, 0:64, :], p, preferred_element_type=F32)
            else:
                vscr[k1] = jnp.dot(gm[k1], p, preferred_element_type=F32)
        for rho in range(8):
            V = {}
            for k1 in range(NK1):
                re = (1, vscr[k1, pl.ds(8 * rho, 8), :])
                im = None if k1 in (0, 32) else (1, vscr[k1, pl.ds(64 + 8 * rho, 8), :])
                V[k1] = (re, im)
            bf = _Bfly()
            out = bf.inv64(V)
            for b in range(32):
                tau = 64 * (b % 4) + 8 * rho
                s_, v_ = out[b]
                val = v_ if s_ > 0 else -v_
                yscr[b // 4, c, pl.ds(PITCH * (tau // TS) + tau % TS, 8), :] = val

    def gather_perm(src_ref_fn):
        cols = []
        for ct in range(NT):
            ref = src_ref_fn(ct)
            cols.append(jnp.concatenate([ref[pl.ds(j, 8, stride=PITCH), :] for j in range(TS)], axis=0))
        return jnp.concatenate(cols, axis=1)

    def scan_tile(u, n, layer):
        sl = slice(128 * n, 128 * (n + 1))
        lr, li = tab[0, :, sl], tab[1, :, sl]
        ur = [u[8 * j:8 * j + 8, 0:128] for j in range(TS)]
        ui = [u[8 * j:8 * j + 8, 128:256] for j in range(TS)]
        er, ei = ur[0], ui[0]
        for j in range(1, TS):
            er, ei = _cmul_add(lr, li, er, ei, ur[j], ui[j])
        sub1 = jax.lax.broadcasted_iota(jnp.int32, (8, 128), 0)
        gr = jnp.where(sub1 == 0, carry[layer, 0, :, sl], pltpu.roll(er, 1, 0))
        gi = jnp.where(sub1 == 0, carry[layer, 1, :, sl], pltpu.roll(ei, 1, 0))
        for q, sh in enumerate((1, 2, 4)):
            gr, gi = _cmul_add(tab[4 + 2 * q, :, sl], tab[5 + 2 * q, :, sl],
                               pltpu.roll(gr, sh, 0), pltpu.roll(gi, sh, 0), gr, gi)
        nr_, ni_ = _cmul_add(tab[2, :, sl], tab[3, :, sl], gr, gi, er, ei)
        carry[layer, 0, :, sl] = jnp.broadcast_to(nr_[7:8, :], (8, 128))
        carry[layer, 1, :, sl] = jnp.broadcast_to(ni_[7:8, :], (8, 128))
        hr, hi = gr, gi
        hs = []
        for j in range(TS):
            hr, hi = _cmul_add(lr, li, hr, hi, ur[j], ui[j])
            hs.append(jnp.concatenate([hr, hi], axis=1))
        return jnp.concatenate(hs, axis=0).astype(BF16)

    def a_layer(x, layer):
        ln = _layernorm(x)
        lnb = ln.astype(BF16)
        xres = x + ln * par[0, 0:1, :]
        y = None
        us, hs = {}, {}
        for n in range(NT + 2):
            if n < NT:
                us[n] = _nt_dot(lnb, bw[256 * n:256 * (n + 1), :])
            if 1 <= n <= NT:
                hs[n - 1] = scan_tile(us[n - 1], n - 1, layer)
            if n >= 2:
                yn = _nt_dot(hs[n - 2], cw[:, 256 * (n - 2):256 * (n - 1)])
                y = yn if y is None else y + yn
        return xres + y

    for n in range(NT):
        for w_ in range(4):
            cp_w(n, w_).wait()
        sl = slice(128 * n, 128 * (n + 1))
        cr = cst[0, :, sl].astype(F32)
        ci = cst[1, :, sl].astype(F32)
        f_r, f_i = 2.0 * fr[:, sl], 2.0 * fi[:, sl]
        cw[:, 256 * n:256 * n + 128] = (cr * f_r - ci * f_i).astype(BF16)
        cw[:, 256 * n + 128:256 * (n + 1)] = (-(cr * f_i + ci * f_r)).astype(BF16)

    for c in range(NCH):
        cp_x(c).wait()
        xv = xin[pl.ds(T * c, T), :].astype(F32)
        for ct in range(NT):
            for seg in range(8):
                pad[ct, pl.ds(PITCH * seg, TS), :] = xv[TS * seg:TS * (seg + 1), 128 * ct:128 * (ct + 1)]
        xp = gather_perm(lambda ct: pad.at[ct])
        x1[pl.ds(T * c, T), :] = a_layer(xp, 0)

    cp_f.wait()
    cp_g.wait()
    for c in range(NT):
        conv_tile(c)

    for c in range(NCH):
        x = x1[pl.ds(T * c, T), :]
        yc = gather_perm(lambda ct: yscr.at[c, ct])
        x = x + _layernorm(x) * yc
        x = a_layer(x, 1)
        yc = gather_perm(lambda ct: yscr.at[c, ct])
        x = x + _layernorm(x) * yc
        for ct in range(NT):
            for j in range(TS):
                pad[ct, pl.ds(j, 8, stride=PITCH), :] = x[8 * j:8 * j + 8, 128 * ct:128 * (ct + 1)]
        if c >= 2:
            cp_o(c - 2).wait()
        for ct in range(NT):
            for seg in range(8):
                ostg[c % 2, TS * seg:TS * (seg + 1), 128 * ct:128 * (ct + 1)] = pad[ct, pl.ds(PITCH * seg, TS), :]
        cp_o(c).start()
    cp_o(NCH - 2).wait()
    cp_o(NCH - 1).wait()


@jax.jit
def pallas_interleave_layers__ssm_conv_s5__ssm_conv_h3__prompt_kernel(
    A_x, A_Lambda_re, A_Lambda_im, A_B_re, A_B_im, A_C_re, A_C_im, A_log_dt, A_Dskip,
    B_q, B_k, B_v, B_shift_k, B_ssm_k, B_ssm_D,
):
    del B_q
    x2 = A_x.reshape(S, D)
    k2 = B_k.reshape(S, D)
    v2 = B_v.reshape(S, D)
    shkT = B_shift_k.T
    hbm = pl.BlockSpec(memory_space=pltpu.HBM)
    vm = pl.BlockSpec(memory_space=pltpu.VMEM)
    out = pl.pallas_call(
        _kernel,
        out_shape=jax.ShapeDtypeStruct((S, D), F32),
        in_specs=[vm] * 6 + [hbm] * 10,
        out_specs=hbm,
        scratch_shapes=[
            pltpu.VMEM((S, D), BF16),
            pltpu.VMEM((2 * D, D), BF16),
            pltpu.VMEM((2, D, D), BF16),
            pltpu.VMEM((D, 2 * D), BF16),
            pltpu.VMEM((10, 8, D), F32),
            pltpu.VMEM((6, 8, D), F32),
            pltpu.VMEM((2, 2, 8, D), F32),
            pltpu.VMEM((NT, S, 128), BF16),
            pltpu.VMEM((NT, S, 128), BF16),
            pltpu.VMEM((NT, 128, S), BF16),
            pltpu.VMEM((NK1, 128, 128), BF16),
            pltpu.VMEM((NK1, 128, 128), BF16),
            pltpu.VMEM((S + 8, 128), F32),
            pltpu.VMEM((S, 128), F32),
            pltpu.VMEM((S, 128), F32),
            pltpu.VMEM((32, 128, 256), BF16),
            pltpu.VMEM((NK1, 128, 128), F32),
            pltpu.VMEM((NCH, NT, PADR, 128), F32),
            pltpu.VMEM((S, D), F32),
            pltpu.VMEM((NT, PADR, 128), F32),
            pltpu.VMEM((2, T, D), F32),
            pltpu.SemaphoreType.DMA((NCH,)),
            pltpu.SemaphoreType.DMA((4 * NT,)),
            pltpu.SemaphoreType.DMA((3 * NT,)),
            pltpu.SemaphoreType.DMA((2,)),
            pltpu.SemaphoreType.DMA((2,)),
        ],
        compiler_params=pltpu.CompilerParams(vmem_limit_bytes=100 * 1024 * 1024),
    )(A_Lambda_re, A_Lambda_im, A_log_dt, A_Dskip, shkT, B_ssm_D,
      x2, A_B_re, A_B_im, A_C_re, A_C_im, k2, v2, B_ssm_k, _FM, _GM)
    return out.reshape(1, S, D)
```

```python
import numpy as np
import jax
import jax.numpy as jnp
import jax.experimental.pallas as pl
import jax.experimental.pallas.tpu as pltpu

S, D = 2048, 640
NT = D // 128
TS = 32
T = 8 * TS
NCH = S // T
PITCH = TS + 1
PADR = 304
NFFT = 4096
NK1 = 33
C8 = float(np.sqrt(0.5))
F32 = jnp.float32
BF16 = jnp.bfloat16


class Bf:
    def __init__(self):
        self.tab = {}; self.keep = []
    def _plus(self, va, vb):
        key = ('+',) + tuple(sorted((id(va), id(vb))))
        if key not in self.tab:
            self.tab[key] = va + vb; self.keep.append((va, vb))
        return self.tab[key]
    def _minus(self, va, vb):
        k1 = ('-', id(va), id(vb)); k2 = ('-', id(vb), id(va))
        if k1 in self.tab: return (1, self.tab[k1])
        if k2 in self.tab: return (-1, self.tab[k2])
        self.tab[k1] = va - vb; self.keep.append((va, vb))
        return (1, self.tab[k1])
    def _times(self, va, c):
        key = ('*', id(va), c)
        if key not in self.tab:
            self.tab[key] = va * c; self.keep.append(va)
        return self.tab[key]
    def radd(self, a, b):
        if a is None: return b
        if b is None: return a
        sa, va = a; sb, vb = b
        if sa == sb: return (sa, self._plus(va, vb))
        s, v = self._minus(va, vb)
        return (s * sa, v)
    @staticmethod
    def rneg(a):
        return None if a is None else (-a[0], a[1])
    def rsub(self, a, b):
        return self.radd(a, self.rneg(b))
    def rmul(self, a, c):
        if a is None or c == 0.0: return None
        s = 1 if c > 0 else -1
        c = abs(c)
        if c == 1.0: return (a[0] * s, a[1])
        return (a[0] * s, self._times(a[1], c))
    def cadd(self, a, b): return (self.radd(a[0], b[0]), self.radd(a[1], b[1]))
    def csub(self, a, b): return (self.rsub(a[0], b[0]), self.rsub(a[1], b[1]))
    def cconj(self, a): return (a[0], self.rneg(a[1]))
    def cmuli(self, a, p):
        p %= 4
        if p == 0: return a
        if p == 1: return (self.rneg(a[1]), a[0])
        if p == 2: return (self.rneg(a[0]), self.rneg(a[1]))
        return (a[1], self.rneg(a[0]))
    def cmul_w(self, a, num, den):
        num %= den
        if (4 * num) % den == 0: return self.cmuli(a, 4 * num // den)
        if (8 * num) % den == 0:
            o = 8 * num // den
            re = self.rmul(self.rsub(a[0], a[1]), C8)
            im = self.rmul(self.radd(a[0], a[1]), C8)
            return self.cmuli((re, im), (o - 1) // 2)
        wr = float(np.cos(2 * np.pi * num / den)); wi = float(np.sin(2 * np.pi * num / den))
        re = self.rsub(self.rmul(a[0], wr), self.rmul(a[1], wi))
        im = self.radd(self.rmul(a[0], wi), self.rmul(a[1], wr))
        return (re, im)
    def fft(self, x, sgn):
        n = len(x)
        def get(v): return v() if callable(v) else v
        if n == 1: return [get(x[0])]
        if n == 2:
            a, b = get(x[0]), get(x[1])
            return [self.cadd(a, b), self.csub(a, b)]
        if n == 4:
            x0, x2 = get(x[0]), get(x[2])
            a = self.cadd(x0, x2); b = self.csub(x0, x2)
            x1, x3 = get(x[1]), get(x[3])
            c = self.cadd(x1, x3); d = self.csub(x1, x3)
            wd = self.cmuli(d, sgn)
            return [self.cadd(a, c), self.cadd(b, wd), self.csub(a, c), self.csub(b, wd)]
        m = n // 4
        u = [self.fft([x[b2 + m * b1] for b1 in range(4)], sgn) for b2 in range(m)]
        out = [None] * n
        for k1 in range(4):
            t = [self.cmul_w(u[b2][k1], sgn * b2 * k1, n) for b2 in range(m)]
            y = self.fft(t, sgn)
            for k2 in range(m):
                out[k1 + 4 * k2] = y[k2]
        return out

    def odd_fwd(self, d, N, emit, scale):
        q = N // 4
        def z(b):
            def th():
                p = d[b]() if callable(d[b]) else d[b]
                r = d[b + q]() if callable(d[b + q]) else d[b + q]
                return self.cmul_w((p, self.rneg(r)), -b, N)
            return th
        Y = self.fft([z(b) for b in range(q)], -1)
        for j in range(q):
            k = 4 * j + 1
            if 2 * k <= N: emit(k * scale, Y[j])
            else: emit((N - k) * scale, self.cconj(Y[j]))
    def real_fwd(self, x, N, emit, scale):
        if N == 2:
            emit(0, (self.radd(x[0], x[1]), None)); emit(scale, (self.rsub(x[0], x[1]), None)); return
        h = N // 2
        s = [self.radd(x[b], x[b + h]) for b in range(h)]
        d = [self.rsub(x[b], x[b + h]) for b in range(h)]
        if N == 4:
            emit(scale, (d[0], self.rneg(d[1])))
        else:
            self.odd_fwd(d, N, emit, scale)
        self.real_fwd(s, h, emit, 2 * scale)

    def odd_inv(self, V, N, scale):
        q = N // 4
        def U(j):
            k = 4 * j + 1
            if 2 * k <= N: return lambda: V(k * scale)
            return lambda: self.cconj(V((N - k) * scale))
        zt = self.fft([U(j) for j in range(q)], +1)
        out = [None] * (2 * q)
        for b in range(q):
            t = self.cmul_w(zt[b], b, N)
            out[b] = t[0]; out[b + q] = self.rneg(t[1])
        return out
    def real_inv(self, V, N, scale):
        if N == 2:
            a, b = V(0)[0], V(scale)[0]
            return [self.radd(a, b), self.rsub(a, b)]
        h = N // 2
        if N == 4:
            v1 = V(scale)
            qq = [v1[0], self.rneg(v1[1])]
        else:
            qq = self.odd_inv(V, N, scale)
        p = self.real_inv(V, h, 2 * scale)
        return [self.radd(p[b], qq[b]) for b in range(h)] + [self.rsub(p[b], qq[b]) for b in range(h)]


def _vals(*cs):
    out = []
    for c in cs:
        for p in c:
            if p is not None:
                out.append(p[1])
    return out


class BfH(Bf):
    def __init__(self):
        super().__init__()
        self.n0 = 0

    def dw(self):
        n = len(self.tab)
        w, self.n0 = n - self.n0, n
        return w

    def odd_fwd_g(self, d, N, emit, scale):
        q = N // 4

        def z(b):
            def th():
                p = d[b]() if callable(d[b]) else d[b]
                r = d[b + q]() if callable(d[b + q]) else d[b + q]
                return self.cmul_w((p, self.rneg(r)), -b, N)
            return th
        zs = [z(b) for b in range(q)]
        m = q // 4
        u = []
        for b2 in range(m):
            g = self.fft([zs[b2 + m * b1] for b1 in range(4)], -1)
            u.append(g)
            yield _vals(g[3])[:1], self.dw() + 8
        for k1 in range(4):
            t = [self.cmul_w(u[b2][k1], -b2 * k1, q) for b2 in range(m)]
            y = self.fft(t, -1)
            outs = []
            for k2 in range(m):
                k = 4 * (k1 + 4 * k2) + 1
                if 2 * k <= N:
                    outs.append((k * scale, y[k2]))
                else:
                    outs.append(((N - k) * scale, self.cconj(y[k2])))
            dd = emit(outs)
            yield dd, self.dw() + 12

    def fwd_q2(self, x, emit):
        def d(b):
            return lambda: self.rsub(x[b](), x[b + 16]())
        yield from self.odd_fwd_g([d(b) for b in range(16)], 32, emit, 2)

    def fwd_q0(self, x, emit):
        s = [None] * 16
        for b in range(8):
            s[b] = self.radd(x[b](), x[b + 16]())
            s[b + 8] = self.radd(x[b + 8](), x[b + 24]())
        outs = []
        self.real_fwd(s, 16, lambda k, c: outs.append((k, c)), 4)
        outs.sort(key=lambda kc: (kc[0] not in (0, 32), kc[0]))
        w = self.dw()
        yield emit(outs[:5]), w + 12
        yield emit(outs[5:]), 12

    def fwd_even_g(self, x, emit):
        s = [self.radd(x[b], x[b + 16]) for b in range(16)]
        d = [self.rsub(x[b], x[b + 16]) for b in range(16)]
        yield from self.odd_fwd_g(d, 32, emit, 2)
        outs = []
        self.real_fwd(s, 16, lambda k, c: outs.append((k, c)), 4)
        outs.sort(key=lambda kc: (kc[0] not in (0, 32), kc[0]))
        w = self.dw()
        yield emit(outs[:5]), w + 12
        yield emit(outs[5:]), 12

    def inv_g(self, V, emit, rel=lambda: None):
        def odd_stage1(N, scale):
            q = N // 4
            m = q // 4

            def U(j):
                k = 4 * j + 1
                if 2 * k <= N:
                    return lambda: V(k * scale)
                return lambda: self.cconj(V((N - k) * scale))
            u = []
            deps = []
            for b2 in range(m):
                g = self.fft([U(b2 + m * b1) for b1 in range(4)], +1)
                u.append(g)
                deps.append((_vals(g[3])[:1], self.dw() + 8))
            return u, deps

        def odd_stage2(u, N, k1):
            q = N // 4
            m = q // 4
            t = [self.cmul_w(u[b2][k1], b2 * k1, q) for b2 in range(m)]
            y = self.fft(t, +1)
            res = {}
            for k2 in range(m):
                b = k1 + 4 * k2
                tt = self.cmul_w(y[k2], b, N)
                res[b] = tt[0]
                res[b + q] = self.rneg(tt[1])
            return res
        rel()
        uo, deps = odd_stage1(64, 1)
        for dd in deps:
            yield dd
        o = {}
        for k1 in range(4):
            o.update(odd_stage2(uo, 64, k1))
            yield [o[b][1] for b in sorted(o) if b % 4 == k1 and (b // 4) % 2 == 0], self.dw() + 4
        rel()
        uq, deps = odd_stage1(32, 2)
        for dd in deps:
            yield dd
        y1 = {}
        for k1 in range(4):
            qq = odd_stage2(uq, 32, k1)
            for b in sorted(qq):
                y1[b] = self.radd(o[b], qq[b])
                y1[b + 16] = self.rsub(o[b + 16], qq[b])
            yield [y1[b][1] for b in sorted(qq)], self.dw() + 4
        rel()
        p = self.real_inv(V, 16, 4)
        yield [p[5][1]], self.dw() + 16
        for k1 in range(4):
            outs = []
            for b in range(k1, 32, 4):
                outs.append((b, self.radd(y1[b], p[b % 16])))
            dd = emit(outs)
            yield dd, self.dw() + 16


def _fwd_plan():
    Y = {}
    order = []

    def emit(outs):
        for k, c in outs:
            Y[k] = c
            if k != 32:
                order.append(k)
        return []
    xs = [(1, np.full((1,), float(i + 1) ** 1.37)) for i in range(32)]
    xl = [(lambda v=v: v) for v in xs]
    we = sum(w for _, w in BfH().fwd_q2(xl, emit)) + sum(w for _, w in BfH().fwd_q0(xl, emit))
    wo = sum(w for _, w in BfH().odd_fwd_g(xs, 64, emit, 1))
    full = {k: ((1, np.full((1,), 1.0 + k)), None if k in (0, 32) else (1, np.full((1,), 2.5 + k)))
            for k in range(NK1)}
    wi = sum(w for _, w in BfH().inv_g(lambda k: full[k], lambda o: []))
    sg = {k: tuple(0 if c is None else c[0] for c in Y[k]) for k in range(NK1)}
    slot = {k: (i // 2, i % 2) for i, k in enumerate(order)}
    slot[32] = slot[0]
    return sg, slot, we + wo, wi


_FSG, _FSLOT, _W_FWD, _W_INV = _fwd_plan()

def _pack_rows(m):
    b = m.astype(np.float32).astype(jnp.bfloat16).view(np.uint16).astype(np.uint32)
    w = b[..., 0::2, :] | (b[..., 1::2, :] << 16)
    return w.view(np.int32)


def _dft_matrices():
    r = np.arange(64)
    k2 = np.arange(64)
    Fm = np.zeros((NK1, 128, 128), np.float64)
    Gm = np.zeros((NK1, 128, 128), np.float64)
    col = (16 * (r // 8) + (r % 8))
    for k1 in range(NK1):
        th = 2 * np.pi * np.outer(k1 + 64 * k2, r) / NFFT
        c, s = np.cos(th), np.sin(th)
        sr, si = _FSG[k1]
        if k1 == 0:
            Fm[k1][0:64][:, col] = c * sr
            Fm[k1][64:128][:, col] = -s * sr
        elif k1 == 32:
            Fm[k1][0:64][:, col + 8] = c * sr
            Fm[k1][64:128][:, col + 8] = -s * sr
        else:
            Fm[k1][0:64][:, col] = c * sr
            Fm[k1][0:64][:, col + 8] = s * si
            Fm[k1][64:128][:, col] = -s * sr
            Fm[k1][64:128][:, col + 8] = c * si
        sc = (1.0 if k1 in (0, 32) else 2.0) / NFFT
        ct, st = c.T * sc, s.T * sc
        Gm[k1][0:64][:, col] = ct
        Gm[k1][0:64][:, col + 8] = -st
        Gm[k1][64:128][:, col] = st
        Gm[k1][64:128][:, col + 8] = ct
    return _pack_rows(Fm), _pack_rows(Gm)


_FM, _GM = _dft_matrices()


def _cmul(ar, ai, br, bi):
    return ar * br - ai * bi, ar * bi + ai * br


def _cmul_add(lr, li, hr, hi, ur, ui):
    return (lr * hr - li * hi) + ur, (lr * hi + li * hr) + ui


def _layernorm(x):
    m = jnp.mean(x, axis=-1, keepdims=True)
    xc = x - m
    v = jnp.mean(xc * xc, axis=-1, keepdims=True)
    return xc * jax.lax.rsqrt(v + 1e-5)


def _nt_dot(a, b):
    return jax.lax.dot_general(a, b, (((1,), (1,)), ((), ())), preferred_element_type=F32)


I32 = jnp.int32
import os as _os
CFG = dict(
    bench=_os.environ.get("BENCH", ""),
    opq=int(_os.environ.get("OPQ", "0")),
    pin_scan=int(_os.environ.get("PINSCAN", "1")),
    nch=int(_os.environ.get("NCHB", "4")),
    orw=int(_os.environ.get("ORW", "1")),
    lock=int(_os.environ.get("LOCKB", "1")),
    gate=int(_os.environ.get("GATE", "0")),
    glag=int(_os.environ.get("GLAG", "2")),
    rel=int(_os.environ.get("REL", "1")),
    lhs2=int(_os.environ.get("LHS2", "0")),
    sc0=int(_os.environ.get("SC0", "700")),
    scw=int(_os.environ.get("SCW", "650")),
    rslot=int(_os.environ.get("RSLOT", "1")),
    skip=_os.environ.get("SKIP", "").split(","),
    lhs=int(_os.environ.get("LHS", "3")),
    orw_tr=int(_os.environ.get("ORWTR", "0")),
    orw_fin=int(_os.environ.get("ORWFIN", "0")),
    orw_s1=int(_os.environ.get("ORWS1", "0")),
    scopes=int(_os.environ.get("SCOPES", "0")),
    nodma=int(_os.environ.get("NODMA", "0")),
    lead1=int(_os.environ.get("LEAD1", "300")),
    lead2=int(_os.environ.get("LEAD2", "500")),
    slotmax=int(_os.environ.get("SLOTMAX", "384")),
)


LOCK, UNLOCK = object(), object()


class _Dot:
    def __init__(self, t0, slots, emit):
        self.t0 = t0
        self.slots = sorted(((t0 + rt, key) for rt, key in slots), key=lambda tk: tk[0])
        self.emit = emit
        self.att = {}
        self.requires = []


class _Barrier:
    def __init__(self, f):
        self.f = f
        self.emitted = False
        self.requires = []


class _Stream:
    def __init__(self, gen, wtot, t0, t1, after=(), needs=(), orw=None):
        self.gen, self.wtot, self.t0, self.t1 = gen, float(wtot), t0, t1
        self.after, self.needs = list(after), list(needs)
        self.orw = orw or CFG["orw"]
        self.cum = 0.0
        self.done = False

    def now(self):
        return self.t0 + (self.t1 - self.t0) * min(1.0, self.cum / self.wtot)


class _Sched:
    def __init__(self):
        self.items, self.streams = [], []
        self.t, self.pos = 0.0, 0
        self.lock = None
        self.scope, self.nseg = None, 0
        self.dropped = 0
        self.cur = None
        self.tokens = []

    def fn(self, f):
        self.items.append(f)

    def barrier(self, f):
        b = _Barrier(f)
        self.items.append(b)
        return b

    def dot(self, dur, slots, emit):
        d = _Dot(self.t, slots, emit)
        self.items.append(d)
        self.t += dur
        return d

    def stream(self, gen, wtot, t0, t1, after=(), needs=(), orw=None):
        s = _Stream(gen, wtot, t0, t1, after, needs, orw)
        self.streams.append(s)
        return s

    def token_at(self, t):
        best = None
        for ts, th in self.tokens[-400:]:
            if ts <= t and (best is None or ts > best[0]):
                best = (ts, th)
        return best

    def _attach1(self, t, d):
        stop = self.pos
        while stop < len(self.items) and not isinstance(self.items[stop], _Barrier):
            stop += 1
        for it in self.items[self.pos:stop]:
            if isinstance(it, _Dot):
                for ts, key in it.slots:
                    if ts >= t and key not in it.att:
                        it.att[key] = d
                        return ts
        for it in reversed(self.items[self.pos:stop]):
            if isinstance(it, _Dot):
                for ts, key in reversed(it.slots):
                    if key not in it.att:
                        it.att[key] = d
                        return ts
        self.dropped += 1
        return t

    def _attach(self, t0, t1, deps, n):
        if not deps:
            return
        chunks = [deps[i:i + n] for i in range(0, len(deps), n)]
        for i, ch in enumerate(chunks):
            d = None
            for v in ch:
                vi = v if v.dtype == I32 else pltpu.bitcast(v, I32)
                d = vi if d is None else d | vi
            self._attach1(t0 + (t1 - t0) * (i + 1.0) / len(chunks), d)

    def _step(self, s):
        for b in s.needs:
            while not b.emitted:
                self._emit_next()
        for a in s.after:
            self._drain(a)
        try:
            self.cur = s
            deps, w = next(s.gen)
        except StopIteration:
            s.done = True
            if self.lock is s:
                self.lock = None
            return
        if deps is LOCK:
            self.lock = s
            return
        if deps is UNLOCK:
            self.lock = None
            return
        ta = s.now()
        s.cum += w
        self._attach(ta, s.now(), deps, s.orw)

    def _drain(self, s):
        while not s.done:
            self._step(s)

    def _emit_next(self):
        it = self.items[self.pos]
        if isinstance(it, _Dot):
            for s in it.requires:
                self._drain(s)
            self.pos += 1
            it.emit(it.att)
        elif isinstance(it, _Barrier):
            for s in it.requires:
                self._drain(s)
            self.pos += 1
            if CFG["scopes"]:
                if self.scope is not None:
                    self.scope.__exit__(None, None, None)
                self.nseg += 1
                with jax.named_scope("s_wait%02d" % self.nseg):
                    it.f()
                self.scope = jax.named_scope("s_seg%02d" % self.nseg)
                self.scope.__enter__()
            else:
                it.f()
            it.emitted = True
        else:
            self.pos += 1
            it()

    def _advance(self, t):
        while self.pos < len(self.items):
            it = self.items[self.pos]
            if isinstance(it, _Dot) and any(ts >= t and key not in it.att for ts, key in it.slots):
                return
            self._emit_next()

    def run(self):
        while True:
            live = [s for s in self.streams if not s.done]
            if not live:
                break
            s = self.lock if self.lock is not None else min(live, key=lambda z: z.now())
            self._advance(s.now())
            if not s.done:
                self._step(s)
        while self.pos < len(self.items):
            self._emit_next()
        if self.scope is not None:
            self.scope.__exit__(None, None, None)


def _kernel(lre_ref, lim_ref, ldt_ref, dsk_ref, shk_ref, sD_ref, zm_ref, zs_ref,
            x_hbm, bre_hbm, bim_hbm, cre_hbm, cim_hbm, k_hbm, v_hbm, sk_hbm, f_hbm, g_hbm,
            o_hbm,
            xin, wst, bw, cw, tab, par, carry, kin, vin, skin, fm, gm,
            kf, kvf, skt, ybf0, ybf1, vscr0, vscr1, yscr, x1, xa0, xa1, xa2, lnb0, lnb1, hb0, hb1, hb2, hb3, pad, ostg,
            sem_x, sem_w, sem_kv, sem_fg, sem_o):

    started = set()

    class _Cp:
        def __init__(self, key, desc):
            self.key, self.desc = key, desc

        def start(self):
            assert self.key not in started, self.key
            started.add(self.key)
            if not CFG["nodma"]:
                self.desc.start()

        def wait(self):
            assert self.key in started, self.key
            started.remove(self.key)
            if not CFG["nodma"]:
                self.desc.wait()

    def cp_x(c):
        rs = pl.ds(T * c, T)
        return _Cp(("x", c), pltpu.make_async_copy(x_hbm.at[rs, :], xin.at[rs, :], sem_x.at[c]))

    def cp_w(n, which):
        src = (bre_hbm, bim_hbm, cre_hbm, cim_hbm)[which]
        if which < 2:
            return _Cp(("w", n, which), pltpu.make_async_copy(
                src.at[pl.ds(128 * n, 128), :], wst.at[which, pl.ds(128 * n, 128), :], sem_w.at[4 * n + which]))
        return _Cp(("w", n, which), pltpu.make_async_copy(
            src.at[:, pl.ds(128 * n, 128)], wst.at[which, :, pl.ds(128 * n, 128)], sem_w.at[4 * n + which]))

    def cp_kv(c, which):
        src, dst = ((k_hbm.at[:, pl.ds(128 * c, 128)], kin), (v_hbm.at[:, pl.ds(128 * c, 128)], vin),
                    (sk_hbm.at[pl.ds(128 * c, 128), :], skin))[which]
        return _Cp(("kv", c, which), pltpu.make_async_copy(src, dst.at[c], sem_kv.at[3 * c + which]))

    cp_f = _Cp(("f",), pltpu.make_async_copy(f_hbm, fm, sem_fg.at[0]))
    cp_g = _Cp(("g",), pltpu.make_async_copy(g_hbm, gm, sem_fg.at[1]))
    OSPLIT = ((0, 4), (4, 7), (7, 8))

    def cp_o(i):
        lo, hi = OSPLIT[i]
        rs = pl.ds(T * lo, T * (hi - lo))
        return _Cp(("o", i), pltpu.make_async_copy(ostg.at[rs, :], o_hbm.at[rs, :], sem_o.at[i]))

    def tile_start(c):
        for w in range(3):
            cp_kv(c, w).start()

    def tile_wait(c):
        for w in range(3):
            cp_kv(c, w).wait()

    if CFG["bench"] == "":
        cp_x(0).start()
        for w in range(4):
            cp_w(0, w).start()

    def row(ref):
        return ref[...].astype(F32)[None, :]

    lre, lim, ldt = row(lre_ref), row(lim_ref), row(ldt_ref)
    dt = jnp.exp(ldt).astype(BF16).astype(F32)
    zr, zi = dt * lre, dt * lim
    mag = jnp.exp(zr)
    lbr, lbi = mag * jnp.cos(zi), mag * jnp.sin(zi)
    inv = 1.0 / (lre * lre + lim * lim)
    nr, ni = lbr - 1.0, lbi
    fr, fi = (nr * lre + ni * lim) * inv, (ni * lre - nr * lim) * inv
    sub = jax.lax.broadcasted_iota(jnp.int32, (8, D), 0)

    def b8(v):
        return jnp.broadcast_to(v, (8, D))

    tab[0] = b8(lbr)
    tab[1] = b8(lbi)
    pr, pi = lbr, lbi
    for _ in range(5):
        pr, pi = _cmul(pr, pi, pr, pi)
    tab[2] = b8(pr)
    tab[3] = b8(pi)
    for q, sh in enumerate((1, 2, 4)):
        tab[4 + 2 * q] = jnp.where(sub >= sh, b8(pr), 0.0)
        tab[5 + 2 * q] = jnp.where(sub >= sh, b8(pi), 0.0)
        pr, pi = _cmul(pr, pi, pr, pi)
    par[0] = b8(row(dsk_ref))
    par[1] = b8(row(sD_ref))
    shk = shk_ref[...].astype(F32)
    for lag in range(4):
        par[2 + lag] = b8(shk[lag:lag + 1, :])
    par[6] = b8(2.0 * fr)
    par[7] = b8(2.0 * fi)
    carry[...] = jnp.zeros(carry.shape, F32)
    kf[0:8, :] = jnp.zeros((8, 128), F32)

    fmask = zm_ref[:, 0:128] != 0
    z8 = pl.multiple_of(zs_ref[0], 8)

    def lt(n):
        return slice(128 * n, 128 * (n + 1))

    def tiles(v):
        r, l = v.shape
        return [v[8 * i:8 * i + 8, 128 * j:128 * (j + 1)] for i in range(r // 8) for j in range(l // 128)]

    def opq(r0, n, bit=1):
        if not (CFG["opq"] & bit):
            return pl.ds(r0, n)
        return pl.ds(pl.multiple_of(z8 + r0, 8), n)

    def dyn(r0, n, stride=None):
        if stride is None:
            return pl.ds(pl.multiple_of(z8 + r0, 8), n)
        return pl.ds(z8 + r0, n, stride=stride)

    zvec = zm_ref[:, 0:128]

    def release(lead):
        if not CFG["rel"]:
            return z8
        tk = sc.token_at(sc.cur.now() - lead)
        if tk is None:
            return z8
        v = pltpu.bitcast(tk[1](), I32) & zvec
        return pl.multiple_of(v[0, 0], 8)

    def at(z, r0, n, stride=None, aligned=True):
        if stride is not None:
            return pl.ds(z + r0, n, stride=stride)
        if aligned:
            return pl.ds(pl.multiple_of(z + r0, 8), n)
        return pl.ds(z + r0, n)

    def add_tokens(val, t0, tmap):
        r, l = val.shape
        for j in range(0, r // 8, 4):
            for i in range(l // 128):
                sc.tokens.append((t0 + tmap(j, i), lambda j=j, i=i: val[8 * j:8 * j + 8, 128 * i:128 * (i + 1)]))

    class Gate:
        def __init__(self, lag):
            self.lag, self.hist = lag, []

        def done(self, token):
            self.hist.append(token)

        def open(self, *stores):
            if len(self.hist) >= self.lag:
                tok = self.hist[-self.lag]
                for f in stores:
                    f(tok)

    def load_hooked(get, nrb, nk, att, keyf):
        rows_ = []
        for rb in range(nrb):
            cols = []
            for kk in range(nk):
                w = get(rb, kk)
                key = keyf(rb, kk)
                if key in att:
                    w = jnp.where(fmask, att[key], w)
                cols.append(w)
            rows_.append(cols[0] if nk == 1 else jnp.concatenate(cols, axis=1))
        return pltpu.bitcast(jnp.concatenate(rows_, axis=0), BF16)

    def a_slots(nk, it):
        sl_ = [(64 * tau - 256 + 32 * p, (tau, 7 - p)) for tau in range(10) for p in range(8)
               if 64 * tau - 256 + 32 * p < CFG["slotmax"]]
        lm = CFG["lhs"] if SEQ[min(it, NIT - 1)][0] == 0 else CFG["lhs2"]
        if lm & (1 if nk == 5 else 2):
            sl_ += [(64 * k + 16 * a, ("l", k, a)) for k in range(nk) for a in range(16)]
        return sl_

    sc = _Sched()
    st = {}

    def mm1(g, att):
        l, c, n = dec(g)
        lb = (lnb0, lnb1)[c % 2]
        lhs = load_hooked(lambda rb, kk: lb[pl.ds(8 * rb, 8), pl.ds(128 * kk, 128)], 16, 5, att,
                          lambda rb, kk: ("l", kk, rb))
        rhs = load_hooked(lambda rb, kk: bw[pl.ds(128 * n + 8 * rb, 8), pl.ds(128 * kk, 128)], 16, 5, att,
                          lambda rb, kk: (5 * (rb // 8) + kk, rb % 8))
        st["u", g] = _nt_dot(lhs, rhs)
        add_tokens(st["u", g], mm1_d[g].t0, lambda j, i: 64 * (5 * i + 4) + 8 * j + 60)

    hbufs = (hb0, hb1, hb2, hb3)
    ybfs = (ybf0, ybf1)
    vscrs = (vscr0, vscr1)
    xas = (xa0, xa1, xa2)

    W_SCAN = 8 * 36 + 70 + 16 * 24

    def scan(g):
        layer, c, n = dec(g)
        u = st.pop(("u", g))
        sl = lt(n)
        lr, li = tab[0, :, sl], tab[1, :, sl]
        ur = [u[8 * j:8 * j + 8, 0:128] for j in range(TS)]
        ui = [u[8 * j:8 * j + 8, 128:256] for j in range(TS)]
        er, ei = ur[0], ui[0]
        for j in range(1, TS):
            er, ei = _cmul_add(lr, li, er, ei, ur[j], ui[j])
            if j % 4 == 3:
                yield [er], 36
        sub1 = jax.lax.broadcasted_iota(jnp.int32, (8, 128), 0)
        gr = jnp.where(sub1 == 0, carry[layer, 0, :, sl], pltpu.roll(er, 1, 0))
        gi = jnp.where(sub1 == 0, carry[layer, 1, :, sl], pltpu.roll(ei, 1, 0))
        for q, sh in enumerate((1, 2, 4)):
            gr, gi = _cmul_add(tab[4 + 2 * q, :, sl], tab[5 + 2 * q, :, sl],
                               pltpu.roll(gr, sh, 0), pltpu.roll(gi, sh, 0), gr, gi)
        nr_, ni_ = _cmul_add(tab[2, :, sl], tab[3, :, sl], gr, gi, er, ei)
        cr_ = jnp.broadcast_to(nr_[7:8, :], (8, 128))
        ci_ = jnp.broadcast_to(ni_[7:8, :], (8, 128))
        carry[layer, 0, :, sl] = cr_
        carry[layer, 1, :, sl] = ci_
        yield [gr, gi, cr_, ci_], 70
        hr, hi = gr, gi
        for a in range(TS // 2):
            two = []
            for j in (2 * a, 2 * a + 1):
                hr, hi = _cmul_add(lr, li, hr, hi, ur[j], ui[j])
                two.append(jnp.concatenate([hr, hi], axis=1))
            hbuf = hbufs[g % 4]
            hbuf[pl.ds(8 * a, 8), :] = pltpu.bitcast(jnp.concatenate(two, axis=0).astype(BF16), I32)
            yield [hbuf[pl.ds(8 * a, 8), pl.ds(128 * h_, 128)] for h_ in range(2)], 24

    def mm2(g, att):
        layer, c, n = dec(g)
        hb = hbufs[g % 4]
        h = load_hooked(lambda rb, kk: hb[pl.ds(8 * rb, 8), pl.ds(128 * kk, 128)], 16, 2, att,
                        lambda rb, kk: ("l", kk, rb))
        rhs = load_hooked(lambda rb, kk: cw[pl.ds(8 * rb, 8), pl.ds(256 * n + 128 * kk, 128)], 40, 2, att,
                          lambda rb, kk: (2 * (rb // 8) + kk, rb % 8))
        yn = _nt_dot(h, rhs)
        add_tokens(yn, mm2_d[g].t0, lambda j, i: 64 * (2 * i + 1) + 8 * j + 60)
        st["y", layer, c] = yn if n == 0 else st["y", layer, c] + yn

    def wwait(n):
        for w in range(4):
            cp_w(n, w).wait()
        if n + 2 < NT:
            for w in range(4):
                cp_w(n + 2, w).start()
        if n == 1:
            cp_x(2).start()
        if n == 2:
            cp_x(1).wait()
        if n == 3:
            tile_start(0)
        if n == NT - 1:
            cp_x(2).wait()
            cp_x(3).start()

    def wprep(n):
        for w in range(2):
            bw[pl.ds(128 * n + 64 * w, 64), :] = pltpu.bitcast(wst[w, pl.ds(128 * n, 128), :], I32)
        cr = wst[2, :, lt(n)].astype(F32)
        ci = wst[3, :, lt(n)].astype(F32)
        f_r, f_i = par[6, 0:1, lt(n)], par[7, 0:1, lt(n)]
        cc_ = jnp.concatenate([cr * f_r - ci * f_i, -(cr * f_i + ci * f_r)], axis=1).astype(BF16)
        cw[:, 256 * n:256 * (n + 1)] = pltpu.bitcast(cc_, I32)

    def yrow(c, sig, p):
        return (sig * 16 + p) * 64

    W_S1 = 32 * 80 + 16 * _W_FWD

    def conv_tr(c):
        for m in range(16 if "tr" not in CFG["skip"] else 0):
            z = release(330)
            val = skin[z + c, :, pl.ds(128 * m, 128)].astype(F32).T
            skt[pl.ds(128 * m, 128), :] = val
            yield tiles(val), 1

    def conv_s1(c):
        w = [par[2 + lag, :, lt(c)] for lag in range(4)]
        for m in range(32 if "kvc" not in CFG["skip"] else 0):
            z = release(110)
            kf[pl.ds(8 + 64 * m, 64), :] = kin[z + c, pl.ds(64 * m, 64), :].astype(F32)
            vv = vin[z + c, pl.ds(64 * m, 64), :].astype(F32)
            deps = []
            for i in range(8):
                t0 = 8 + 64 * m + 8 * i
                acc = kf[at(z, t0 - 3, 8, aligned=False), :] * w[3]
                acc = acc + kf[at(z, t0 - 2, 8, aligned=False), :] * w[2]
                acc = acc + kf[at(z, t0 - 1, 8, aligned=False), :] * w[1]
                acc = acc + kf[at(z, t0, 8), :] * w[0]
                kv = acc * vv[8 * i:8 * i + 8, :]
                kvf[pl.ds(t0 - 8, 8), :] = kv
                deps.append(kv)
            yield deps, 90
        for sig in ((0, 1) if "cols" not in CFG["skip"] else ()):
            if sig == 1:
                sc._drain(tr_s[c])
                sc.cur = s1_s[c]
            src = kvf if sig == 0 else skt
            for rho in range(8):
                pend = {}

                def emit(outs):
                    vals = []
                    for k1, v in outs:
                        if k1 in (0, 32):
                            pend[k1] = v[0]
                            if len(pend) == 2:
                                vals.append((0, pend[0][1], pend[32][1]))
                        else:
                            vals.append((k1, v[0][1], v[1][1]))
                    deps = []
                    for i in range(0, len(vals), 2):
                        r0 = yrow(c, sig, _FSLOT[vals[i][0]][0]) + 8 * rho
                        two = jnp.concatenate(
                            [jnp.concatenate([vals[i + e][1], vals[i + e][2]], axis=0) for e in range(2)], axis=1)
                        ybf = ybfs[c % 2]
                        ybf[pl.ds(r0, 8), :] = pltpu.bitcast(two.astype(BF16), I32)
                        deps += [ybf[pl.ds(r0, 8), pl.ds(128 * h_, 128)] for h_ in range(2)]
                    return deps

                def xs(z):
                    return [(lambda b=b: (1, src[at(z, 64 * b + 8 * rho, 8), :])) for b in range(32)]
                for part in range(3):
                    if CFG["lock"]:
                        yield LOCK, 0
                    z = release(90)
                    if part == 0:
                        yield from BfH().fwd_q2(xs(z), emit)
                    elif part == 1:
                        yield from BfH().fwd_q0(xs(z), emit)
                    else:
                        yield from BfH().odd_fwd_g(xs(z), 64, emit, 1)
                    if CFG["lock"]:
                        yield UNLOCK, 0

    def f_slots(n):
        return [(8 * a, (0, a)) for a in range(n)]

    def conv_mx_steps(c):
        def fwd(k1, att):
            lhs = load_hooked(lambda rb, kk: fm[k1, pl.ds(8 * rb, 8), :], 8, 1, att, lambda rb, kk: (0, rb))
            p, s_ = _FSLOT[k1]
            rhs = load_hooked(lambda rb, kk: ybfs[c % 2][pl.ds(yrow(c, kk, p) + 8 * rb, 8), pl.ds(128 * s_, 128)],
                              8, 2, att, lambda rb, kk: ("r", kk, rb))
            st["z", c, k1] = jnp.dot(lhs, rhs, preferred_element_type=F32)

        def pw(k1):
            z = st.pop(("z", c, k1))
            dD = par[1, :, lt(c)]
            parts = []
            for g in range(8):
                ur = z[8 * g:8 * g + 8, 0:128]
                ui = z[64 + 8 * g:64 + 8 * g + 8, 0:128]
                kr = z[8 * g:8 * g + 8, 128:256] + dD
                ki = z[64 + 8 * g:64 + 8 * g + 8, 128:256]
                pr_, pi_ = _cmul(ur, ui, kr, ki)
                parts += [pr_, pi_]
            st["p", c, k1] = jnp.concatenate(parts, axis=0).astype(BF16)

        def inv_(k1, att):
            p = st.pop(("p", c, k1))
            nrb = 4 if k1 in (0, 32) else 8
            lhs = load_hooked(lambda rb, kk: gm[k1, pl.ds(8 * rb, 8), :], nrb, 1, att, lambda rb, kk: (0, rb))
            vscrs[c % 2][pl.ds(k1 * 128, 16 * nrb), :] = jnp.dot(lhs, p, preferred_element_type=F32)

        steps = []
        for i in range(NK1 + 2):
            def f(i=i):
                first = None
                if i < NK1:
                    first = sc.dot(64, f_slots(8) + [(-100 + 32 * kk + 8 * a, ("r", kk, a)) for kk in range(2) for a in range(8)
                                                     if CFG["rslot"]],
                                   lambda att, i=i: fwd(i, att))
                if 1 <= i <= NK1:
                    sc.fn(lambda i=i: pw(i - 1))
                if i >= 2:
                    sc.dot(32, f_slots(4 if i - 2 in (0, 32) else 8), lambda att, i=i: inv_(i - 2, att))
                return first
            steps.append(f)
        return steps

    W_FIN = 8 * _W_INV

    def conv_fin(c):
        vscr = vscrs[c % 2]
        for rho in range(8 if "fin" not in CFG["skip"] else 0):
            zz = {}

            def V(k1):
                r0 = k1 * 128 + 8 * rho
                re = (1, vscr[at(zz["z"], r0, 8), :])
                im = None if k1 in (0, 32) else (1, vscr[at(zz["z"], r0 + 64, 8), :])
                return (re, im)

            def emit(outs):
                deps = []
                for b, (s_, v_) in outs:
                    tau = 64 * (b % 4) + 8 * rho
                    val = v_ if s_ > 0 else -v_
                    yscr[b // 4, c, pl.ds(PITCH * (tau // TS) + tau % TS, 8), :] = val
                    deps.append(val)
                return deps

            def rel():
                zz["z"] = release(90)
            if CFG["lock"]:
                yield LOCK, 0
            yield from BfH().inv_g(V, emit, rel)
            if CFG["lock"]:
                yield UNLOCK, 0

    def gather16(ref_fn, q, z):
        return jnp.concatenate(
            [jnp.concatenate([ref_fn(ct)[at(z, 2 * q + e, 8, PITCH), :] for ct in range(NT)], axis=1)
             for e in range(2)], axis=0)

    def ln_to_mm(c, q, x, l):
        ln = _layernorm(x)
        lb = (lnb0, lnb1)[c % 2]
        lb[pl.ds(8 * q, 8), :] = pltpu.bitcast(ln.astype(BF16), I32)
        dsk = par[0]
        xr = x + ln * jnp.concatenate([dsk, dsk], axis=0)
        xas[(l * NCH + c) % 3][pl.ds(16 * q, 16), :] = xr
        return [lb[pl.ds(8 * q, 8), lt(ct)] for ct in range(NT)] + tiles(xr)

    def pre1(c):
        for i in range(4 if "prepost" not in CFG["skip"] else 0):
            z = release(CFG["lead1"] + 60)
            for ct in range(NT):
                for s_ in range(8):
                    pad[ct, pl.ds(PITCH * s_ + 8 * i, 8), :] = \
                        xin[at(z, T * c + TS * s_ + 8 * i, 8), lt(ct)].astype(F32)
            for q in range(4 * i, 4 * i + 4):
                if q % 4:
                    z = release(CFG["lead1"])
                yield ln_to_mm(c, q, gather16(lambda ct: pad.at[ct], q, z), 0), 1

    def post1(c):
        y = st["y", 0, c]
        for q in range(16 if "prepost" not in CFG["skip"] else 0):
            z = release(60)
            v_ = xas[c % 3][at(z, 16 * q, 16), :] + y[16 * q:16 * q + 16, :]
            x1[pl.ds(T * c + 16 * q, 16), :] = v_
            yield tiles(v_), 1

    def pre2(c):
        for q in range(16):
            z = release(CFG["lead2"])
            x = x1[at(z, T * c + 16 * q, 16), :]
            yc = gather16(lambda ct: yscr.at[c, ct], q, z)
            x = x + _layernorm(x) * yc
            yield ln_to_mm(c, q, x, 1), 1

    def post2(c):
        y = st["y", 1, c]
        for i in range(4):
            for q in range(4 * i, 4 * i + 4):
                z = release(CFG["lead1"])
                x = xas[(NCH + c) % 3][at(z, 16 * q, 16), :] + y[16 * q:16 * q + 16, :]
                yc = gather16(lambda ct: yscr.at[c, ct], q, z)
                x = x + _layernorm(x) * yc
                for ct in range(NT):
                    for e in range(2):
                        pad[ct, pl.ds(2 * q + e, 8, stride=PITCH), :] = x[8 * e:8 * e + 8, lt(ct)]
                yield tiles(x), 2
            deps = []
            z = release(80)
            for ct in range(NT):
                for s_ in range(8):
                    v_ = pad[ct, at(z, PITCH * s_ + 8 * i, 8, aligned=False), :]
                    ostg[pl.ds(T * c + TS * s_ + 8 * i, 8), lt(ct)] = v_
                    deps.append(v_)
            yield deps, 1

    if CFG["bench"] == "p2":
        SEQ = [(1, c) for c in range(CFG["nch"])]
    elif CFG["bench"] in ("p1", "f"):
        SEQ = [(0, c) for c in range(CFG["nch"])]
    else:
        SEQ = [(l, c) for l in range(2) for c in range(NCH)]
    NIT = len(SEQ)
    G = NIT * NT
    FULL = CFG["bench"] == ""
    FFT_TILES = list(range(NT)) if FULL else ([0, 1] if CFG["bench"] == "f" else [])

    def dec(g):
        return SEQ[g // NT] + (g % NT,)

    TS1, DELTA = (9000.0 if FULL else 0.0), 9000.0
    m_start = {c: TS1 + (c + 1) * DELTA for c in range(NT)}
    m_quota = {c: (4 if c < NT - 1 else 7) for c in range(NT)}
    m_steps = {c: (conv_mx_steps(c) if c in FFT_TILES else []) for c in range(NT)}
    mx_first, mx_end = {}, {}

    def b_a():
        tile_wait(0)
        cp_x(3).wait()
        tile_start(1)
        cp_f.start()
        cp_g.start()
        cp_x(4).start()

    def b_tile(c):
        def f():
            tile_wait(c)
            cp_x(c + 3).wait()
            if c == 1:
                cp_f.wait()
                cp_g.wait()
            if c + 1 < NT:
                tile_start(c + 1)
                cp_x(c + 4).start()
        return f
    timed = [(TS1, "t0", b_a)] + [(TS1 + c * DELTA, "t%d" % c, b_tile(c)) for c in range(1, NT)]
    if not FULL:
        timed = []
    bar = {}
    tr_s = {}

    def before_dot():
        while timed and sc.t >= timed[0][0]:
            _, name, f = timed.pop(0)
            bar[name] = sc.barrier(f)

    def after_dot():
        before_dot()
        for c in range(NT):
            if sc.t >= m_start[c] and m_steps[c]:
                for _ in range(m_quota[c]):
                    if m_steps[c]:
                        f0 = m_steps[c].pop(0)()
                        if c not in mx_first:
                            mx_first[c] = f0
                if not m_steps[c]:
                    mx_end[c] = sc.t
                break

    t_it, mm1_d, mm2_d = {}, {}, {}
    if FULL:
        def x0w():
            cp_x(0).wait()
            for w in range(4):
                cp_w(1, w).start()
            cp_x(1).start()
        bar["x0"] = sc.barrier(x0w)
    for it in range(NIT + 1):
        t_it[it] = sc.t
        if FULL and it == 13:
            bar["o0"] = sc.barrier(lambda: cp_o(0).start())
        if FULL and it == 16:
            bar["o1"] = sc.barrier(lambda: cp_o(1).start())
        for n in range(NT):
            g = NT * it + n
            if g < G:
                before_dot()
                if FULL and g < NT:
                    bar["w%d" % n] = sc.barrier(lambda n=n: wwait(n))
                    sc.fn(lambda n=n: wprep(n))
                mm1_d[g] = sc.dot(640, a_slots(5, it), lambda att, g=g: mm1(g, att))
                after_dot()
            if 2 <= g < G + 2:
                before_dot()
                mm2_d[g - 2] = sc.dot(640, a_slots(2, it), lambda att, g=g: mm2(g - 2, att))
                after_dot()
    t_it[NIT + 1] = sc.t

    prev = None
    for g in range(G):
        if CFG["pin_scan"]:
            s_ = sc.stream(scan(g), W_SCAN, mm1_d[g].t0 + CFG["sc0"],
                           min(mm2_d[g].t0 - 100, mm1_d[g].t0 + CFG["sc0"] + CFG["scw"]), after=[prev] if prev else [])
        else:
            def nat(g=g):
                for _ in scan(g):
                    pass
                return
                yield
            s_ = sc.stream(nat(g), 1, mm1_d[g].t0 + 700, mm1_d[g].t0 + 700, after=[prev] if prev else [])
        mm2_d[g].requires.append(s_)
        prev = s_
    s1_s, fin_s = {}, {}
    for c in FFT_TILES:
        s1_s[c] = sc.stream(conv_s1(c), W_S1, TS1 + c * DELTA, TS1 + (c + 1) * DELTA - 200,
                            after=[s1_s[c - 1]] if c else [], needs=[bar["t%d" % c]] if FULL else [], orw=CFG["orw_s1"])
        tr_s[c] = sc.stream(conv_tr(c), 16, TS1 + c * DELTA, TS1 + (c + 0.5) * DELTA,
                            after=[s1_s[c - 1]] if c else [], needs=[bar["t%d" % c]] if FULL else [],
                            orw=CFG["orw_tr"])
        mx_first[c].requires.append(s1_s[c])
        span = 5500 if c < NT - 1 else 3000
        fin_s[c] = sc.stream(conv_fin(c), W_FIN, mx_end[c] + 200, mx_end[c] + 200 + span,
                             after=[fin_s[c - 1]] if c else [], orw=CFG["orw_fin"])
    pre_s, post_s = {}, {}
    for it in range(NIT):
        l, c = SEQ[it]
        gen = pre1(c) if l == 0 else pre2(c)
        if it == 0:
            pre_s[it] = sc.stream(gen, 16, -2000, -1000, needs=[bar["x0"]] if FULL else [])
        else:
            t0 = t_it[it - 1] + 100
            aft = [pre_s[it - 1]]
            nd = []
            if not FULL:
                pass
            elif it == 1:
                t0 = t_it[0] + 0.5 * (t_it[1] - t_it[0])
                nd = [bar["w2"]]
            elif it == 2:
                nd = [bar["w4"]]
            elif it == 3:
                nd = [bar["t0"]]
            elif 4 <= it <= 7:
                nd = [bar["t%d" % (it - 3)]]
            if it >= 3:
                aft.append(post_s[it - 3])
            if FULL and it == NCH:
                t0 = max(t0, fin_s[NT - 1].t1)
                aft.append(fin_s[NT - 1])
            pre_s[it] = sc.stream(gen, 16, t0, t_it[it] - 450, after=aft, needs=nd)
        mm1_d[NT * it].requires.append(pre_s[it])
        gen = post1(c) if l == 0 else post2(c)
        t0 = mm2_d[NT * it + NT - 1].t0 + 640 + 150
        t1 = t_it[it + 2] - 100 if it + 2 <= NIT else t0 + 1000
        post_s[it] = sc.stream(gen, 16 if l == 0 else 36, t0, t1, after=[post_s[it - 1]] if it else [])
    if FULL:
        bar["o0"].requires.append(post_s[NCH + OSPLIT[0][1] - 1])
        bar["o1"].requires.append(post_s[NCH + OSPLIT[1][1] - 1])
    sc.run()
    if _os.environ.get("VERBOSE"):
        print("dropped pins:", sc.dropped)
    if FULL:
        cp_o(2).start()
        for i in range(3):
            cp_o(i).wait()
        assert not started


_ZMASK = np.concatenate([np.zeros((8, 128), np.int32), np.arange(1024, dtype=np.int32).reshape(8, 128)], axis=1)
_ZS = np.array([0, 7, 3, 11], np.int32)


@jax.jit
def pallas_interleave_layers__ssm_conv_s5__ssm_conv_h3__prompt_kernel(
    A_x, A_Lambda_re, A_Lambda_im, A_B_re, A_B_im, A_C_re, A_C_im, A_log_dt, A_Dskip,
    B_q, B_k, B_v, B_shift_k, B_ssm_k, B_ssm_D,
):
    del B_q
    x2 = A_x.reshape(S, D)
    k2 = B_k.reshape(S, D)
    v2 = B_v.reshape(S, D)
    shkT = B_shift_k.T
    hbm = pl.BlockSpec(memory_space=pltpu.HBM)
    vm = pl.BlockSpec(memory_space=pltpu.VMEM)
    sm = pl.BlockSpec(memory_space=pltpu.SMEM)
    out = pl.pallas_call(
        _kernel,
        out_shape=jax.ShapeDtypeStruct((S, D), F32),
        in_specs=[vm] * 7 + [sm] + [hbm] * 10,
        out_specs=hbm,
        scratch_shapes=[
            pltpu.VMEM((S, D), BF16),
            pltpu.VMEM((4, D, D), BF16),
            pltpu.VMEM((D, D), I32),
            pltpu.VMEM((D // 2, 2 * D), I32),
            pltpu.VMEM((10, 8, D), F32),
            pltpu.VMEM((8, 8, D), F32),
            pltpu.VMEM((2, 2, 8, D), F32),
            pltpu.VMEM((NT, S, 128), BF16),
            pltpu.VMEM((NT, S, 128), BF16),
            pltpu.VMEM((NT, 128, S), BF16),
            pltpu.VMEM((NK1, 64, 128), I32),
            pltpu.VMEM((NK1, 64, 128), I32),
            pltpu.VMEM((S + 8, 128), F32),
            pltpu.VMEM((S + 8, 128), F32),
            pltpu.VMEM((S + 8, 128), F32),
            pltpu.VMEM((2 * 16 * 64, 256), I32),
            pltpu.VMEM((2 * 16 * 64, 256), I32),
            pltpu.VMEM((NK1 * 128 + 8, 128), F32),
            pltpu.VMEM((NK1 * 128 + 8, 128), F32),
            pltpu.VMEM((NCH, NT, PADR, 128), F32),
            pltpu.VMEM((S + 8, D), F32),
            pltpu.VMEM((T + 8, D), F32),
            pltpu.VMEM((T + 8, D), F32),
            pltpu.VMEM((T + 8, D), F32),
            pltpu.VMEM((T // 2, D), I32),
            pltpu.VMEM((T // 2, D), I32),
            pltpu.VMEM((T // 2, 256), I32),
            pltpu.VMEM((T // 2, 256), I32),
            pltpu.VMEM((T // 2, 256), I32),
            pltpu.VMEM((T // 2, 256), I32),
            pltpu.VMEM((NT, PADR, 128), F32),
            pltpu.VMEM((S, D), F32),
            pltpu.SemaphoreType.DMA((NCH,)),
            pltpu.SemaphoreType.DMA((4 * NT,)),
            pltpu.SemaphoreType.DMA((3 * NT,)),
            pltpu.SemaphoreType.DMA((2,)),
            pltpu.SemaphoreType.DMA((3,)),
        ],
        compiler_params=pltpu.CompilerParams(vmem_limit_bytes=100 * 1024 * 1024),
    )(A_Lambda_re, A_Lambda_im, A_log_dt, A_Dskip, shkT, B_ssm_D, _ZMASK, _ZS,
      x2, A_B_re, A_B_im, A_C_re, A_C_im, k2, v2, B_ssm_k, _FM, _GM)
    return out.reshape(1, S, D)
```

```python
import numpy as np
import jax
import jax.numpy as jnp
import jax.experimental.pallas as pl
import jax.experimental.pallas.tpu as pltpu

S, D = 2048, 640
NT = D // 128
TS = 32
T = 8 * TS
NCH = S // T
PITCH = TS + 1
PADR = 304
NFFT = 4096
NK1 = 33
C8 = float(np.sqrt(0.5))
F32 = jnp.float32
BF16 = jnp.bfloat16


class Bf:
    def __init__(self):
        self.tab = {}; self.keep = []
    def _plus(self, va, vb):
        key = ('+',) + tuple(sorted((id(va), id(vb))))
        if key not in self.tab:
            self.tab[key] = va + vb; self.keep.append((va, vb))
        return self.tab[key]
    def _minus(self, va, vb):
        k1 = ('-', id(va), id(vb)); k2 = ('-', id(vb), id(va))
        if k1 in self.tab: return (1, self.tab[k1])
        if k2 in self.tab: return (-1, self.tab[k2])
        self.tab[k1] = va - vb; self.keep.append((va, vb))
        return (1, self.tab[k1])
    def _times(self, va, c):
        key = ('*', id(va), c)
        if key not in self.tab:
            self.tab[key] = va * c; self.keep.append(va)
        return self.tab[key]
    def radd(self, a, b):
        if a is None: return b
        if b is None: return a
        sa, va = a; sb, vb = b
        if sa == sb: return (sa, self._plus(va, vb))
        s, v = self._minus(va, vb)
        return (s * sa, v)
    @staticmethod
    def rneg(a):
        return None if a is None else (-a[0], a[1])
    def rsub(self, a, b):
        return self.radd(a, self.rneg(b))
    def rmul(self, a, c):
        if a is None or c == 0.0: return None
        s = 1 if c > 0 else -1
        c = abs(c)
        if c == 1.0: return (a[0] * s, a[1])
        return (a[0] * s, self._times(a[1], c))
    def cadd(self, a, b): return (self.radd(a[0], b[0]), self.radd(a[1], b[1]))
    def csub(self, a, b): return (self.rsub(a[0], b[0]), self.rsub(a[1], b[1]))
    def cconj(self, a): return (a[0], self.rneg(a[1]))
    def cmuli(self, a, p):
        p %= 4
        if p == 0: return a
        if p == 1: return (self.rneg(a[1]), a[0])
        if p == 2: return (self.rneg(a[0]), self.rneg(a[1]))
        return (a[1], self.rneg(a[0]))
    def cmul_w(self, a, num, den):
        num %= den
        if (4 * num) % den == 0: return self.cmuli(a, 4 * num // den)
        if (8 * num) % den == 0:
            o = 8 * num // den
            re = self.rmul(self.rsub(a[0], a[1]), C8)
            im = self.rmul(self.radd(a[0], a[1]), C8)
            return self.cmuli((re, im), (o - 1) // 2)
        wr = float(np.cos(2 * np.pi * num / den)); wi = float(np.sin(2 * np.pi * num / den))
        re = self.rsub(self.rmul(a[0], wr), self.rmul(a[1], wi))
        im = self.radd(self.rmul(a[0], wi), self.rmul(a[1], wr))
        return (re, im)
    def fft(self, x, sgn):
        n = len(x)
        def get(v): return v() if callable(v) else v
        if n == 1: return [get(x[0])]
        if n == 2:
            a, b = get(x[0]), get(x[1])
            return [self.cadd(a, b), self.csub(a, b)]
        if n == 4:
            x0, x2 = get(x[0]), get(x[2])
            a = self.cadd(x0, x2); b = self.csub(x0, x2)
            x1, x3 = get(x[1]), get(x[3])
            c = self.cadd(x1, x3); d = self.csub(x1, x3)
            wd = self.cmuli(d, sgn)
            return [self.cadd(a, c), self.cadd(b, wd), self.csub(a, c), self.csub(b, wd)]
        m = n // 4
        u = [self.fft([x[b2 + m * b1] for b1 in range(4)], sgn) for b2 in range(m)]
        out = [None] * n
        for k1 in range(4):
            t = [self.cmul_w(u[b2][k1], sgn * b2 * k1, n) for b2 in range(m)]
            y = self.fft(t, sgn)
            for k2 in range(m):
                out[k1 + 4 * k2] = y[k2]
        return out

    def odd_fwd(self, d, N, emit, scale):
        q = N // 4
        def z(b):
            def th():
                p = d[b]() if callable(d[b]) else d[b]
                r = d[b + q]() if callable(d[b + q]) else d[b + q]
                return self.cmul_w((p, self.rneg(r)), -b, N)
            return th
        Y = self.fft([z(b) for b in range(q)], -1)
        for j in range(q):
            k = 4 * j + 1
            if 2 * k <= N: emit(k * scale, Y[j])
            else: emit((N - k) * scale, self.cconj(Y[j]))
    def real_fwd(self, x, N, emit, scale):
        if N == 2:
            emit(0, (self.radd(x[0], x[1]), None)); emit(scale, (self.rsub(x[0], x[1]), None)); return
        h = N // 2
        s = [self.radd(x[b], x[b + h]) for b in range(h)]
        d = [self.rsub(x[b], x[b + h]) for b in range(h)]
        if N == 4:
            emit(scale, (d[0], self.rneg(d[1])))
        else:
            self.odd_fwd(d, N, emit, scale)
        self.real_fwd(s, h, emit, 2 * scale)

    def odd_inv(self, V, N, scale):
        q = N // 4
        def U(j):
            k = 4 * j + 1
            if 2 * k <= N: return lambda: V(k * scale)
            return lambda: self.cconj(V((N - k) * scale))
        zt = self.fft([U(j) for j in range(q)], +1)
        out = [None] * (2 * q)
        for b in range(q):
            t = self.cmul_w(zt[b], b, N)
            out[b] = t[0]; out[b + q] = self.rneg(t[1])
        return out
    def real_inv(self, V, N, scale):
        if N == 2:
            a, b = V(0)[0], V(scale)[0]
            return [self.radd(a, b), self.rsub(a, b)]
        h = N // 2
        if N == 4:
            v1 = V(scale)
            qq = [v1[0], self.rneg(v1[1])]
        else:
            qq = self.odd_inv(V, N, scale)
        p = self.real_inv(V, h, 2 * scale)
        return [self.radd(p[b], qq[b]) for b in range(h)] + [self.rsub(p[b], qq[b]) for b in range(h)]


def _vals(*cs):
    out = []
    for c in cs:
        for p in c:
            if p is not None:
                out.append(p[1])
    return out


class BfH(Bf):
    def __init__(self):
        super().__init__()
        self.n0 = 0

    def dw(self):
        n = len(self.tab)
        w, self.n0 = n - self.n0, n
        return w

    def odd_fwd_g(self, d, N, emit, scale):
        q = N // 4

        def z(b):
            def th():
                p = d[b]() if callable(d[b]) else d[b]
                r = d[b + q]() if callable(d[b + q]) else d[b + q]
                return self.cmul_w((p, self.rneg(r)), -b, N)
            return th
        zs = [z(b) for b in range(q)]
        m = q // 4
        u = []
        for b2 in range(m):
            g = self.fft([zs[b2 + m * b1] for b1 in range(4)], -1)
            u.append(g)
            yield _vals(g[3])[:1], self.dw() + 8
        for k1 in range(4):
            t = [self.cmul_w(u[b2][k1], -b2 * k1, q) for b2 in range(m)]
            y = self.fft(t, -1)
            outs = []
            for k2 in range(m):
                k = 4 * (k1 + 4 * k2) + 1
                if 2 * k <= N:
                    outs.append((k * scale, y[k2]))
                else:
                    outs.append(((N - k) * scale, self.cconj(y[k2])))
            dd = emit(outs)
            yield dd, self.dw() + 12

    def fwd_q2(self, x, emit):
        def d(b):
            return lambda: self.rsub(x[b](), x[b + 16]())
        yield from self.odd_fwd_g([d(b) for b in range(16)], 32, emit, 2)

    def fwd_q0(self, x, emit):
        s = [None] * 16
        for b in range(8):
            s[b] = self.radd(x[b](), x[b + 16]())
            s[b + 8] = self.radd(x[b + 8](), x[b + 24]())
        outs = []
        self.real_fwd(s, 16, lambda k, c: outs.append((k, c)), 4)
        outs.sort(key=lambda kc: (kc[0] not in (0, 32), kc[0]))
        w = self.dw()
        yield emit(outs[:5]), w + 12
        yield emit(outs[5:]), 12

    def fwd_even_g(self, x, emit):
        s = [self.radd(x[b], x[b + 16]) for b in range(16)]
        d = [self.rsub(x[b], x[b + 16]) for b in range(16)]
        yield from self.odd_fwd_g(d, 32, emit, 2)
        outs = []
        self.real_fwd(s, 16, lambda k, c: outs.append((k, c)), 4)
        outs.sort(key=lambda kc: (kc[0] not in (0, 32), kc[0]))
        w = self.dw()
        yield emit(outs[:5]), w + 12
        yield emit(outs[5:]), 12

    def inv_g(self, V, emit, rel=lambda: None):
        def odd_stage1(N, scale):
            q = N // 4
            m = q // 4

            def U(j):
                k = 4 * j + 1
                if 2 * k <= N:
                    return lambda: V(k * scale)
                return lambda: self.cconj(V((N - k) * scale))
            u = []
            deps = []
            for b2 in range(m):
                g = self.fft([U(b2 + m * b1) for b1 in range(4)], +1)
                u.append(g)
                deps.append((_vals(g[3])[:1], self.dw() + 8))
            return u, deps

        def odd_stage2(u, N, k1):
            q = N // 4
            m = q // 4
            t = [self.cmul_w(u[b2][k1], b2 * k1, q) for b2 in range(m)]
            y = self.fft(t, +1)
            res = {}
            for k2 in range(m):
                b = k1 + 4 * k2
                tt = self.cmul_w(y[k2], b, N)
                res[b] = tt[0]
                res[b + q] = self.rneg(tt[1])
            return res
        rel()
        uo, deps = odd_stage1(64, 1)
        for dd in deps:
            yield dd
        o = {}
        for k1 in range(4):
            o.update(odd_stage2(uo, 64, k1))
            yield [o[b][1] for b in sorted(o) if b % 4 == k1 and (b // 4) % 2 == 0], self.dw() + 4
        rel()
        uq, deps = odd_stage1(32, 2)
        for dd in deps:
            yield dd
        y1 = {}
        for k1 in range(4):
            qq = odd_stage2(uq, 32, k1)
            for b in sorted(qq):
                y1[b] = self.radd(o[b], qq[b])
                y1[b + 16] = self.rsub(o[b + 16], qq[b])
            yield [y1[b][1] for b in sorted(qq)], self.dw() + 4
        rel()
        p = self.real_inv(V, 16, 4)
        yield [p[5][1]], self.dw() + 16
        for k1 in range(4):
            outs = []
            for b in range(k1, 32, 4):
                outs.append((b, self.radd(y1[b], p[b % 16])))
            dd = emit(outs)
            yield dd, self.dw() + 16


def _fwd_plan():
    Y = {}
    order = []

    def emit(outs):
        for k, c in outs:
            Y[k] = c
            if k != 32:
                order.append(k)
        return []
    xs = [(1, np.full((1,), float(i + 1) ** 1.37)) for i in range(32)]
    xl = [(lambda v=v: v) for v in xs]
    we = sum(w for _, w in BfH().fwd_q2(xl, emit)) + sum(w for _, w in BfH().fwd_q0(xl, emit))
    wo = sum(w for _, w in BfH().odd_fwd_g(xs, 64, emit, 1))
    full = {k: ((1, np.full((1,), 1.0 + k)), None if k in (0, 32) else (1, np.full((1,), 2.5 + k)))
            for k in range(NK1)}
    wi = sum(w for _, w in BfH().inv_g(lambda k: full[k], lambda o: []))
    sg = {k: tuple(0 if c is None else c[0] for c in Y[k]) for k in range(NK1)}
    slot = {k: (i // 2, i % 2) for i, k in enumerate(order)}
    slot[32] = slot[0]
    return sg, slot, we + wo, wi


_FSG, _FSLOT, _W_FWD, _W_INV = _fwd_plan()

def _pack_rows(m):
    b = m.astype(np.float32).astype(jnp.bfloat16).view(np.uint16).astype(np.uint32)
    w = b[..., 0::2, :] | (b[..., 1::2, :] << 16)
    return w.view(np.int32)


def _dft_matrices():
    r = np.arange(64)
    k2 = np.arange(64)
    Fm = np.zeros((NK1, 128, 128), np.float64)
    Gm = np.zeros((NK1, 128, 128), np.float64)
    col = (16 * (r // 8) + (r % 8))
    for k1 in range(NK1):
        th = 2 * np.pi * np.outer(k1 + 64 * k2, r) / NFFT
        c, s = np.cos(th), np.sin(th)
        sr, si = _FSG[k1]
        if k1 == 0:
            Fm[k1][0:64][:, col] = c * sr
            Fm[k1][64:128][:, col] = -s * sr
        elif k1 == 32:
            Fm[k1][0:64][:, col + 8] = c * sr
            Fm[k1][64:128][:, col + 8] = -s * sr
        else:
            Fm[k1][0:64][:, col] = c * sr
            Fm[k1][0:64][:, col + 8] = s * si
            Fm[k1][64:128][:, col] = -s * sr
            Fm[k1][64:128][:, col + 8] = c * si
        sc = (1.0 if k1 in (0, 32) else 2.0) / NFFT
        ct, st = c.T * sc, s.T * sc
        Gm[k1][0:64][:, col] = ct
        Gm[k1][0:64][:, col + 8] = -st
        Gm[k1][64:128][:, col] = st
        Gm[k1][64:128][:, col + 8] = ct
    return _pack_rows(Fm), _pack_rows(Gm)


_FM, _GM = _dft_matrices()


def _cmul(ar, ai, br, bi):
    return ar * br - ai * bi, ar * bi + ai * br


def _cmul_add(lr, li, hr, hi, ur, ui):
    return (lr * hr - li * hi) + ur, (lr * hi + li * hr) + ui


def _layernorm(x):
    m = jnp.mean(x, axis=-1, keepdims=True)
    xc = x - m
    v = jnp.mean(xc * xc, axis=-1, keepdims=True)
    return xc * jax.lax.rsqrt(v + 1e-5)


def _nt_dot(a, b):
    return jax.lax.dot_general(a, b, (((1,), (1,)), ((), ())), preferred_element_type=F32)


I32 = jnp.int32
import os as _os
CFG = dict(
    bench=_os.environ.get("BENCH", ""),
    opq=int(_os.environ.get("OPQ", "0")),
    pin_scan=int(_os.environ.get("PINSCAN", "0")),
    nch=int(_os.environ.get("NCHB", "4")),
    orw=int(_os.environ.get("ORW", "1")),
    lock=int(_os.environ.get("LOCKB", "1")),
    gate=int(_os.environ.get("GATE", "0")),
    glag=int(_os.environ.get("GLAG", "2")),
    rel=int(_os.environ.get("REL", "0")),
    lhs2=int(_os.environ.get("LHS2", "0")),
    sc0=int(_os.environ.get("SC0", "700")),
    scw=int(_os.environ.get("SCW", "650")),
    rslot=int(_os.environ.get("RSLOT", "1")),
    skip=_os.environ.get("SKIP", "").split(","),
    lhs=int(_os.environ.get("LHS", "3")),
    orw_tr=int(_os.environ.get("ORWTR", "0")),
    orw_fin=int(_os.environ.get("ORWFIN", "0")),
    orw_s1=int(_os.environ.get("ORWS1", "0")),
    scopes=int(_os.environ.get("SCOPES", "0")),
    nodma=int(_os.environ.get("NODMA", "0")),
    lead1=int(_os.environ.get("LEAD1", "300")),
    lead2=int(_os.environ.get("LEAD2", "500")),
    slotmax=int(_os.environ.get("SLOTMAX", "384")),
)


LOCK, UNLOCK = object(), object()


class _Dot:
    def __init__(self, t0, slots, emit):
        self.t0 = t0
        self.slots = sorted(((t0 + rt, key) for rt, key in slots), key=lambda tk: tk[0])
        self.emit = emit
        self.att = {}
        self.requires = []


class _Barrier:
    def __init__(self, f):
        self.f = f
        self.emitted = False
        self.requires = []


class _Stream:
    def __init__(self, gen, wtot, t0, t1, after=(), needs=(), orw=None):
        self.gen, self.wtot, self.t0, self.t1 = gen, float(wtot), t0, t1
        self.after, self.needs = list(after), list(needs)
        self.orw = orw or CFG["orw"]
        self.cum = 0.0
        self.done = False

    def now(self):
        return self.t0 + (self.t1 - self.t0) * min(1.0, self.cum / self.wtot)


class _Sched:
    def __init__(self):
        self.items, self.streams = [], []
        self.t, self.pos = 0.0, 0
        self.lock = None
        self.scope, self.nseg = None, 0
        self.dropped = 0
        self.cur = None
        self.tokens = []

    def fn(self, f):
        self.items.append(f)

    def barrier(self, f):
        b = _Barrier(f)
        self.items.append(b)
        return b

    def dot(self, dur, slots, emit):
        d = _Dot(self.t, slots, emit)
        self.items.append(d)
        self.t += dur
        return d

    def stream(self, gen, wtot, t0, t1, after=(), needs=(), orw=None):
        s = _Stream(gen, wtot, t0, t1, after, needs, orw)
        self.streams.append(s)
        return s

    def token_at(self, t):
        best = None
        for ts, th in self.tokens[-400:]:
            if ts <= t and (best is None or ts > best[0]):
                best = (ts, th)
        return best

    def _attach1(self, t, d):
        stop = self.pos
        while stop < len(self.items) and not isinstance(self.items[stop], _Barrier):
            stop += 1
        for it in self.items[self.pos:stop]:
            if isinstance(it, _Dot):
                for ts, key in it.slots:
                    if ts >= t and key not in it.att:
                        it.att[key] = d
                        return ts
        for it in reversed(self.items[self.pos:stop]):
            if isinstance(it, _Dot):
                for ts, key in reversed(it.slots):
                    if key not in it.att:
                        it.att[key] = d
                        return ts
        self.dropped += 1
        return t

    def _attach(self, t0, t1, deps, n):
        if not deps:
            return
        chunks = [deps[i:i + n] for i in range(0, len(deps), n)]
        for i, ch in enumerate(chunks):
            d = None
            for v in ch:
                vi = v if v.dtype == I32 else pltpu.bitcast(v, I32)
                d = vi if d is None else d | vi
            self._attach1(t0 + (t1 - t0) * (i + 1.0) / len(chunks), d)

    def _step(self, s):
        for b in s.needs:
            while not b.emitted:
                self._emit_next()
        for a in s.after:
            self._drain(a)
        try:
            self.cur = s
            deps, w = next(s.gen)
        except StopIteration:
            s.done = True
            if self.lock is s:
                self.lock = None
            return
        if deps is LOCK:
            self.lock = s
            return
        if deps is UNLOCK:
            self.lock = None
            return
        ta = s.now()
        s.cum += w
        self._attach(ta, s.now(), deps, s.orw)

    def _drain(self, s):
        while not s.done:
            self._step(s)

    def _emit_next(self):
        it = self.items[self.pos]
        if isinstance(it, _Dot):
            for s in it.requires:
                self._drain(s)
            self.pos += 1
            it.emit(it.att)
        elif isinstance(it, _Barrier):
            for s in it.requires:
                self._drain(s)
            self.pos += 1
            if CFG["scopes"]:
                if self.scope is not None:
                    self.scope.__exit__(None, None, None)
                self.nseg += 1
                with jax.named_scope("s_wait%02d" % self.nseg):
                    it.f()
                self.scope = jax.named_scope("s_seg%02d" % self.nseg)
                self.scope.__enter__()
            else:
                it.f()
            it.emitted = True
        else:
            self.pos += 1
            it()

    def _advance(self, t):
        while self.pos < len(self.items):
            it = self.items[self.pos]
            if isinstance(it, _Dot) and any(ts >= t and key not in it.att for ts, key in it.slots):
                return
            self._emit_next()

    def run(self):
        while True:
            live = [s for s in self.streams if not s.done]
            if not live:
                break
            s = self.lock if self.lock is not None else min(live, key=lambda z: z.now())
            self._advance(s.now())
            if not s.done:
                self._step(s)
        while self.pos < len(self.items):
            self._emit_next()
        if self.scope is not None:
            self.scope.__exit__(None, None, None)


def _kernel(lre_ref, lim_ref, ldt_ref, dsk_ref, shk_ref, sD_ref, zm_ref, zs_ref,
            x_hbm, bre_hbm, bim_hbm, cre_hbm, cim_hbm, k_hbm, v_hbm, sk_hbm, f_hbm, g_hbm,
            o_hbm,
            xin, wst, bw, cw, tab, par, carry, kin, vin, skin, fm, gm,
            kf, kvf, skt, ybf0, ybf1, vscr0, vscr1, yscr, x1, xa0, xa1, xa2, lnb0, lnb1, hb0, hb1, hb2, hb3, pad, ostg,
            sem_x, sem_w, sem_kv, sem_fg, sem_o):

    started = set()

    class _Cp:
        def __init__(self, key, desc):
            self.key, self.desc = key, desc

        def start(self):
            assert self.key not in started, self.key
            started.add(self.key)
            if not CFG["nodma"]:
                self.desc.start()

        def wait(self):
            assert self.key in started, self.key
            started.remove(self.key)
            if not CFG["nodma"]:
                self.desc.wait()

    def cp_x(c):
        rs = pl.ds(T * c, T)
        return _Cp(("x", c), pltpu.make_async_copy(x_hbm.at[rs, :], xin.at[rs, :], sem_x.at[c]))

    def cp_w(n, which):
        src = (bre_hbm, bim_hbm, cre_hbm, cim_hbm)[which]
        if which < 2:
            return _Cp(("w", n, which), pltpu.make_async_copy(
                src.at[pl.ds(128 * n, 128), :], wst.at[which, pl.ds(128 * n, 128), :], sem_w.at[4 * n + which]))
        return _Cp(("w", n, which), pltpu.make_async_copy(
            src.at[:, pl.ds(128 * n, 128)], wst.at[which, :, pl.ds(128 * n, 128)], sem_w.at[4 * n + which]))

    def cp_kv(c, which):
        src, dst = ((k_hbm.at[:, pl.ds(128 * c, 128)], kin), (v_hbm.at[:, pl.ds(128 * c, 128)], vin),
                    (sk_hbm.at[pl.ds(128 * c, 128), :], skin))[which]
        return _Cp(("kv", c, which), pltpu.make_async_copy(src, dst.at[c], sem_kv.at[3 * c + which]))

    cp_f = _Cp(("f",), pltpu.make_async_copy(f_hbm, fm, sem_fg.at[0]))
    cp_g = _Cp(("g",), pltpu.make_async_copy(g_hbm, gm, sem_fg.at[1]))
    OSPLIT = ((0, 4), (4, 6), (6, 7), (7, 8))

    def cp_o(i):
        lo, hi = OSPLIT[i]
        rs = pl.ds(T * lo, T * (hi - lo))
        return _Cp(("o", i), pltpu.make_async_copy(ostg.at[rs, :], o_hbm.at[rs, :], sem_o.at[i]))

    def tile_start(c):
        for w in range(3):
            cp_kv(c, w).start()

    def tile_wait(c):
        for w in range(3):
            cp_kv(c, w).wait()

    if CFG["bench"] == "":
        cp_x(0).start()
        for w in range(4):
            cp_w(0, w).start()

    def row(ref):
        return ref[...].astype(F32)[None, :]

    lre, lim, ldt = row(lre_ref), row(lim_ref), row(ldt_ref)
    dt = jnp.exp(ldt).astype(BF16).astype(F32)
    zr, zi = dt * lre, dt * lim
    mag = jnp.exp(zr)
    lbr, lbi = mag * jnp.cos(zi), mag * jnp.sin(zi)
    inv = 1.0 / (lre * lre + lim * lim)
    nr, ni = lbr - 1.0, lbi
    fr, fi = (nr * lre + ni * lim) * inv, (ni * lre - nr * lim) * inv
    sub = jax.lax.broadcasted_iota(jnp.int32, (8, D), 0)

    def b8(v):
        return jnp.broadcast_to(v, (8, D))

    tab[0] = b8(lbr)
    tab[1] = b8(lbi)
    pr, pi = lbr, lbi
    for _ in range(5):
        pr, pi = _cmul(pr, pi, pr, pi)
    tab[2] = b8(pr)
    tab[3] = b8(pi)
    for q, sh in enumerate((1, 2, 4)):
        tab[4 + 2 * q] = jnp.where(sub >= sh, b8(pr), 0.0)
        tab[5 + 2 * q] = jnp.where(sub >= sh, b8(pi), 0.0)
        pr, pi = _cmul(pr, pi, pr, pi)
    par[0] = b8(row(dsk_ref))
    par[1] = b8(row(sD_ref))
    shk = shk_ref[...].astype(F32)
    for lag in range(4):
        par[2 + lag] = b8(shk[lag:lag + 1, :])
    par[6] = b8(2.0 * fr)
    par[7] = b8(2.0 * fi)
    carry[...] = jnp.zeros(carry.shape, F32)
    kf[0:8, :] = jnp.zeros((8, 128), F32)

    fmask = zm_ref[:, 0:128] != 0
    z8 = pl.multiple_of(zs_ref[0], 8)

    def lt(n):
        return slice(128 * n, 128 * (n + 1))

    def tiles(v):
        r, l = v.shape
        return [v[8 * i:8 * i + 8, 128 * j:128 * (j + 1)] for i in range(r // 8) for j in range(l // 128)]

    def opq(r0, n, bit=1):
        if not (CFG["opq"] & bit):
            return pl.ds(r0, n)
        return pl.ds(pl.multiple_of(z8 + r0, 8), n)

    def dyn(r0, n, stride=None):
        if stride is None:
            return pl.ds(pl.multiple_of(z8 + r0, 8), n)
        return pl.ds(z8 + r0, n, stride=stride)

    zvec = zm_ref[:, 0:128]

    def release(lead, kind=1):
        if not (CFG["rel"] & kind):
            return None
        tk = sc.token_at(sc.cur.now() - lead)
        if tk is None:
            return None
        v = pltpu.bitcast(tk[1](), I32) & zvec
        return pl.multiple_of(v[0, 0], 8)

    def at(z, r0, n, stride=None, aligned=True):
        if z is None:
            return pl.ds(r0, n) if stride is None else pl.ds(r0, n, stride=stride)
        if stride is not None:
            return pl.ds(z + r0, n, stride=stride)
        if aligned:
            return pl.ds(pl.multiple_of(z + r0, 8), n)
        return pl.ds(z + r0, n)

    def add_tokens(val, t0, tmap):
        r, l = val.shape
        for j in range(0, r // 8, 4):
            for i in range(l // 128):
                sc.tokens.append((t0 + tmap(j, i), lambda j=j, i=i: val[8 * j:8 * j + 8, 128 * i:128 * (i + 1)]))

    class Gate:
        def __init__(self, lag):
            self.lag, self.hist = lag, []

        def done(self, token):
            self.hist.append(token)

        def open(self, *stores):
            if len(self.hist) >= self.lag:
                tok = self.hist[-self.lag]
                for f in stores:
                    f(tok)

    def load_hooked(get, nrb, nk, att, keyf):
        rows_ = []
        for rb in range(nrb):
            cols = []
            for kk in range(nk):
                w = get(rb, kk)
                key = keyf(rb, kk)
                if key in att:
                    w = jnp.where(fmask, att[key], w)
                cols.append(w)
            rows_.append(cols[0] if nk == 1 else jnp.concatenate(cols, axis=1))
        return pltpu.bitcast(jnp.concatenate(rows_, axis=0), BF16)

    def a_slots(nk, it):
        sl_ = [(64 * tau - 256 + 32 * p, (tau, 7 - p)) for tau in range(10) for p in range(8)
               if 64 * tau - 256 + 32 * p < CFG["slotmax"]]
        lm = CFG["lhs"] if SEQ[min(it, NIT - 1)][0] == 0 else CFG["lhs2"]
        if lm & (1 if nk == 5 else 2):
            sl_ += [(64 * k + 16 * a, ("l", k, a)) for k in range(nk) for a in range(16)]
        return sl_

    sc = _Sched()
    st = {}

    def mm1(g, att):
        l, c, n = dec(g)
        lb = (lnb0, lnb1)[c % 2]
        lhs = load_hooked(lambda rb, kk: lb[pl.ds(8 * rb, 8), pl.ds(128 * kk, 128)], 16, 5, att,
                          lambda rb, kk: ("l", kk, rb))
        rhs = load_hooked(lambda rb, kk: bw[pl.ds(128 * n + 8 * rb, 8), pl.ds(128 * kk, 128)], 16, 5, att,
                          lambda rb, kk: (5 * (rb // 8) + kk, rb % 8))
        st["u", g] = _nt_dot(lhs, rhs)
        add_tokens(st["u", g], mm1_d[g].t0, lambda j, i: 64 * (5 * i + 4) + 8 * j + 60)

    hbufs = (hb0, hb1, hb2, hb3)
    ybfs = (ybf0, ybf1)
    vscrs = (vscr0, vscr1)
    xas = (xa0, xa1, xa2)

    W_SCAN = 8 * 36 + 70 + 16 * 24

    def scan(g):
        layer, c, n = dec(g)
        u = st.pop(("u", g))
        sl = lt(n)
        lr, li = tab[0, :, sl], tab[1, :, sl]
        ur = [u[8 * j:8 * j + 8, 0:128] for j in range(TS)]
        ui = [u[8 * j:8 * j + 8, 128:256] for j in range(TS)]
        er, ei = ur[0], ui[0]
        for j in range(1, TS):
            er, ei = _cmul_add(lr, li, er, ei, ur[j], ui[j])
            if j % 4 == 3:
                yield [er], 36
        sub1 = jax.lax.broadcasted_iota(jnp.int32, (8, 128), 0)
        gr = jnp.where(sub1 == 0, carry[layer, 0, :, sl], pltpu.roll(er, 1, 0))
        gi = jnp.where(sub1 == 0, carry[layer, 1, :, sl], pltpu.roll(ei, 1, 0))
        for q, sh in enumerate((1, 2, 4)):
            gr, gi = _cmul_add(tab[4 + 2 * q, :, sl], tab[5 + 2 * q, :, sl],
                               pltpu.roll(gr, sh, 0), pltpu.roll(gi, sh, 0), gr, gi)
        nr_, ni_ = _cmul_add(tab[2, :, sl], tab[3, :, sl], gr, gi, er, ei)
        cr_ = jnp.broadcast_to(nr_[7:8, :], (8, 128))
        ci_ = jnp.broadcast_to(ni_[7:8, :], (8, 128))
        carry[layer, 0, :, sl] = cr_
        carry[layer, 1, :, sl] = ci_
        yield [gr, gi, cr_, ci_], 70
        hr, hi = gr, gi
        for a in range(TS // 2):
            two = []
            for j in (2 * a, 2 * a + 1):
                hr, hi = _cmul_add(lr, li, hr, hi, ur[j], ui[j])
                two.append(jnp.concatenate([hr, hi], axis=1))
            hbuf = hbufs[g % 4]
            hbuf[pl.ds(8 * a, 8), :] = pltpu.bitcast(jnp.concatenate(two, axis=0).astype(BF16), I32)
            yield [hbuf[pl.ds(8 * a, 8), pl.ds(128 * h_, 128)] for h_ in range(2)], 24

    def mm2(g, att):
        layer, c, n = dec(g)
        hb = hbufs[g % 4]
        h = load_hooked(lambda rb, kk: hb[pl.ds(8 * rb, 8), pl.ds(128 * kk, 128)], 16, 2, att,
                        lambda rb, kk: ("l", kk, rb))
        rhs = load_hooked(lambda rb, kk: cw[pl.ds(8 * rb, 8), pl.ds(256 * n + 128 * kk, 128)], 40, 2, att,
                          lambda rb, kk: (2 * (rb // 8) + kk, rb % 8))
        yn = _nt_dot(h, rhs)
        add_tokens(yn, mm2_d[g].t0, lambda j, i: 64 * (2 * i + 1) + 8 * j + 60)
        st["y", layer, c] = yn if n == 0 else st["y", layer, c] + yn

    def wwait(n):
        for w in range(4):
            cp_w(n, w).wait()
        if n + 2 < NT:
            for w in range(4):
                cp_w(n + 2, w).start()
        if n == 1:
            cp_x(2).start()
        if n == 2:
            cp_x(1).wait()
        if n == 3:
            tile_start(0)
        if n == NT - 1:
            cp_x(2).wait()
            cp_x(3).start()

    def wprep(n):
        for w in range(2):
            bw[pl.ds(128 * n + 64 * w, 64), :] = pltpu.bitcast(wst[w, pl.ds(128 * n, 128), :], I32)
        cr = wst[2, :, lt(n)].astype(F32)
        ci = wst[3, :, lt(n)].astype(F32)
        f_r, f_i = par[6, 0:1, lt(n)], par[7, 0:1, lt(n)]
        cc_ = jnp.concatenate([cr * f_r - ci * f_i, -(cr * f_i + ci * f_r)], axis=1).astype(BF16)
        cw[:, 256 * n:256 * (n + 1)] = pltpu.bitcast(cc_, I32)

    def yrow(c, sig, p):
        return (sig * 16 + p) * 64

    W_S1 = 32 * 80 + 16 * _W_FWD

    def conv_tr(c):
        for m in range(16 if "tr" not in CFG["skip"] else 0):
            z = release(330, 2)
            val = skin[c if z is None else z + c, :, pl.ds(128 * m, 128)].astype(F32).T
            skt[pl.ds(128 * m, 128), :] = val
            yield tiles(val), 1

    def conv_s1(c):
        w = [par[2 + lag, :, lt(c)] for lag in range(4)]
        for m in range(32 if "kvc" not in CFG["skip"] else 0):
            z = release(110, 4)
            kf[pl.ds(8 + 64 * m, 64), :] = kin[c if z is None else z + c, pl.ds(64 * m, 64), :].astype(F32)
            vv = vin[c if z is None else z + c, pl.ds(64 * m, 64), :].astype(F32)
            deps = []
            for i in range(8):
                t0 = 8 + 64 * m + 8 * i
                acc = kf[at(z, t0 - 3, 8, aligned=False), :] * w[3]
                acc = acc + kf[at(z, t0 - 2, 8, aligned=False), :] * w[2]
                acc = acc + kf[at(z, t0 - 1, 8, aligned=False), :] * w[1]
                acc = acc + kf[at(z, t0, 8), :] * w[0]
                kv = acc * vv[8 * i:8 * i + 8, :]
                kvf[pl.ds(t0 - 8, 8), :] = kv
                deps.append(kv)
            yield deps, 90
        for sig in ((0, 1) if "cols" not in CFG["skip"] else ()):
            if sig == 1:
                sc._drain(tr_s[c])
                sc.cur = s1_s[c]
            src = kvf if sig == 0 else skt
            for rho in range(8):
                pend = {}

                def emit(outs):
                    vals = []
                    for k1, v in outs:
                        if k1 in (0, 32):
                            pend[k1] = v[0]
                            if len(pend) == 2:
                                vals.append((0, pend[0][1], pend[32][1]))
                        else:
                            vals.append((k1, v[0][1], v[1][1]))
                    deps = []
                    for i in range(0, len(vals), 2):
                        r0 = yrow(c, sig, _FSLOT[vals[i][0]][0]) + 8 * rho
                        two = jnp.concatenate(
                            [jnp.concatenate([vals[i + e][1], vals[i + e][2]], axis=0) for e in range(2)], axis=1)
                        ybf = ybfs[c % 2]
                        ybf[pl.ds(r0, 8), :] = pltpu.bitcast(two.astype(BF16), I32)
                        deps += [ybf[pl.ds(r0, 8), pl.ds(128 * h_, 128)] for h_ in range(2)]
                    return deps

                def xs(z):
                    return [(lambda b=b: (1, src[at(z, 64 * b + 8 * rho, 8), :])) for b in range(32)]
                for part in range(3):
                    if CFG["lock"]:
                        yield LOCK, 0
                    z = release(90, 8)
                    if part == 0:
                        yield from BfH().fwd_q2(xs(z), emit)
                    elif part == 1:
                        yield from BfH().fwd_q0(xs(z), emit)
                    else:
                        yield from BfH().odd_fwd_g(xs(z), 64, emit, 1)
                    if CFG["lock"]:
                        yield UNLOCK, 0

    def f_slots(n):
        return [(8 * a, (0, a)) for a in range(n)]

    def conv_mx_steps(c):
        def fwd(k1, att):
            lhs = load_hooked(lambda rb, kk: fm[k1, pl.ds(8 * rb, 8), :], 8, 1, att, lambda rb, kk: (0, rb))
            p, s_ = _FSLOT[k1]
            rhs = load_hooked(lambda rb, kk: ybfs[c % 2][pl.ds(yrow(c, kk, p) + 8 * rb, 8), pl.ds(128 * s_, 128)],
                              8, 2, att, lambda rb, kk: ("r", kk, rb))
            st["z", c, k1] = jnp.dot(lhs, rhs, preferred_element_type=F32)

        def pw(k1):
            z = st.pop(("z", c, k1))
            dD = par[1, :, lt(c)]
            parts = []
            for g in range(8):
                ur = z[8 * g:8 * g + 8, 0:128]
                ui = z[64 + 8 * g:64 + 8 * g + 8, 0:128]
                kr = z[8 * g:8 * g + 8, 128:256] + dD
                ki = z[64 + 8 * g:64 + 8 * g + 8, 128:256]
                pr_, pi_ = _cmul(ur, ui, kr, ki)
                parts += [pr_, pi_]
            st["p", c, k1] = jnp.concatenate(parts, axis=0).astype(BF16)

        def inv_(k1, att):
            p = st.pop(("p", c, k1))
            nrb = 4 if k1 in (0, 32) else 8
            lhs = load_hooked(lambda rb, kk: gm[k1, pl.ds(8 * rb, 8), :], nrb, 1, att, lambda rb, kk: (0, rb))
            vscrs[c % 2][pl.ds(k1 * 128, 16 * nrb), :] = jnp.dot(lhs, p, preferred_element_type=F32)

        steps = []
        for i in range(NK1 + 2):
            def f(i=i):
                first = None
                if i < NK1:
                    first = sc.dot(64, f_slots(8) + [(-100 + 32 * kk + 8 * a, ("r", kk, a)) for kk in range(2) for a in range(8)
                                                     if CFG["rslot"]],
                                   lambda att, i=i: fwd(i, att))
                if 1 <= i <= NK1:
                    sc.fn(lambda i=i: pw(i - 1))
                if i >= 2:
                    sc.dot(32, f_slots(4 if i - 2 in (0, 32) else 8), lambda att, i=i: inv_(i - 2, att))
                return first
            steps.append(f)
        return steps

    W_FIN = 8 * _W_INV

    def conv_fin(c):
        vscr = vscrs[c % 2]
        for rho in range(8 if "fin" not in CFG["skip"] else 0):
            zz = {}

            def V(k1):
                r0 = k1 * 128 + 8 * rho
                re = (1, vscr[at(zz["z"], r0, 8), :])
                im = None if k1 in (0, 32) else (1, vscr[at(zz["z"], r0 + 64, 8), :])
                return (re, im)

            def emit(outs):
                deps = []
                for b, (s_, v_) in outs:
                    tau = 64 * (b % 4) + 8 * rho
                    val = v_ if s_ > 0 else -v_
                    yscr[b // 4, c, pl.ds(PITCH * (tau // TS) + tau % TS, 8), :] = val
                    deps.append(val)
                return deps

            def rel():
                zz["z"] = release(90, 16)
            if CFG["lock"]:
                yield LOCK, 0
            yield from BfH().inv_g(V, emit, rel)
            if CFG["lock"]:
                yield UNLOCK, 0

    def gather16(ref_fn, q, z):
        return jnp.concatenate(
            [jnp.concatenate([ref_fn(ct)[at(z, 2 * q + e, 8, PITCH), :] for ct in range(NT)], axis=1)
             for e in range(2)], axis=0)

    def ln_to_mm(c, q, x, l):
        ln = _layernorm(x)
        lb = (lnb0, lnb1)[c % 2]
        lb[pl.ds(8 * q, 8), :] = pltpu.bitcast(ln.astype(BF16), I32)
        dsk = par[0]
        xr = x + ln * jnp.concatenate([dsk, dsk], axis=0)
        xas[(l * NCH + c) % 3][pl.ds(16 * q, 16), :] = xr
        return [lb[pl.ds(8 * q, 8), lt(ct)] for ct in range(NT)] + tiles(xr)

    def pre1(c):
        for i in range(4 if "prepost" not in CFG["skip"] else 0):
            z = release(CFG["lead1"] + 60, 32)
            for ct in range(NT):
                for s_ in range(8):
                    pad[ct, pl.ds(PITCH * s_ + 8 * i, 8), :] = \
                        xin[at(z, T * c + TS * s_ + 8 * i, 8), lt(ct)].astype(F32)
            for q in range(4 * i, 4 * i + 4):
                if q % 4:
                    z = release(CFG["lead1"], 32)
                yield ln_to_mm(c, q, gather16(lambda ct: pad.at[ct], q, z), 0), 1

    def post1(c):
        y = st["y", 0, c]
        for q in range(16 if "prepost" not in CFG["skip"] else 0):
            z = release(60, 32)
            v_ = xas[c % 3][at(z, 16 * q, 16), :] + y[16 * q:16 * q + 16, :]
            x1[pl.ds(T * c + 16 * q, 16), :] = v_
            yield tiles(v_), 1

    def pre2(c):
        for q in range(16):
            z = release(CFG["lead2"], 64)
            x = x1[at(z, T * c + 16 * q, 16), :]
            yc = gather16(lambda ct: yscr.at[c, ct], q, z)
            x = x + _layernorm(x) * yc
            yield ln_to_mm(c, q, x, 1), 1

    def post2(c):
        y = st["y", 1, c]
        for i in range(4):
            for q in range(4 * i, 4 * i + 4):
                z = release(CFG["lead1"], 64)
                x = xas[(NCH + c) % 3][at(z, 16 * q, 16), :] + y[16 * q:16 * q + 16, :]
                yc = gather16(lambda ct: yscr.at[c, ct], q, z)
                x = x + _layernorm(x) * yc
                for ct in range(NT):
                    for e in range(2):
                        pad[ct, pl.ds(2 * q + e, 8, stride=PITCH), :] = x[8 * e:8 * e + 8, lt(ct)]
                yield tiles(x), 2
            deps = []
            z = release(80, 64)
            for ct in range(NT):
                for s_ in range(8):
                    v_ = pad[ct, at(z, PITCH * s_ + 8 * i, 8, aligned=False), :]
                    ostg[pl.ds(T * c + TS * s_ + 8 * i, 8), lt(ct)] = v_
                    deps.append(v_)
            yield deps, 1

    if CFG["bench"] == "p2":
        SEQ = [(1, c) for c in range(CFG["nch"])]
    elif CFG["bench"] in ("p1", "f"):
        SEQ = [(0, c) for c in range(CFG["nch"])]
    else:
        SEQ = [(l, c) for l in range(2) for c in range(NCH)]
    NIT = len(SEQ)
    G = NIT * NT
    FULL = CFG["bench"] == ""
    FFT_TILES = list(range(NT)) if FULL else ([0, 1] if CFG["bench"] == "f" else [])

    def dec(g):
        return SEQ[g // NT] + (g % NT,)

    TS1, DELTA = (9000.0 if FULL else 0.0), 9000.0
    m_start = {c: TS1 + (c + 1) * DELTA for c in range(NT)}
    m_quota = {c: (4 if c < NT - 1 else 7) for c in range(NT)}
    m_steps = {c: (conv_mx_steps(c) if c in FFT_TILES else []) for c in range(NT)}
    mx_first, mx_end = {}, {}

    def b_a():
        tile_wait(0)
        cp_x(3).wait()
        tile_start(1)
        cp_f.start()
        cp_g.start()
        cp_x(4).start()

    def b_tile(c):
        def f():
            tile_wait(c)
            cp_x(c + 3).wait()
            if c == 1:
                cp_f.wait()
                cp_g.wait()
            if c + 1 < NT:
                tile_start(c + 1)
                cp_x(c + 4).start()
        return f
    timed = [(TS1, "t0", b_a)] + [(TS1 + c * DELTA, "t%d" % c, b_tile(c)) for c in range(1, NT)]
    if not FULL:
        timed = []
    bar = {}
    tr_s = {}

    def before_dot():
        while timed and sc.t >= timed[0][0]:
            _, name, f = timed.pop(0)
            bar[name] = sc.barrier(f)

    def after_dot():
        before_dot()
        for c in range(NT):
            if sc.t >= m_start[c] and m_steps[c]:
                for _ in range(m_quota[c]):
                    if m_steps[c]:
                        f0 = m_steps[c].pop(0)()
                        if c not in mx_first:
                            mx_first[c] = f0
                if not m_steps[c]:
                    mx_end[c] = sc.t
                break

    t_it, mm1_d, mm2_d = {}, {}, {}
    if FULL:
        def x0w():
            cp_x(0).wait()
            for w in range(4):
                cp_w(1, w).start()
            cp_x(1).start()
        bar["x0"] = sc.barrier(x0w)
    for it in range(NIT + 1):
        t_it[it] = sc.t
        if FULL and it == 13:
            bar["o0"] = sc.barrier(lambda: cp_o(0).start())
        if FULL and it == 15:
            bar["o1"] = sc.barrier(lambda: cp_o(1).start())
        if FULL and it == 16:
            bar["o2"] = sc.barrier(lambda: cp_o(2).start())
        for n in range(NT):
            g = NT * it + n
            if g < G:
                before_dot()
                if FULL and g < NT:
                    bar["w%d" % n] = sc.barrier(lambda n=n: wwait(n))
                    sc.fn(lambda n=n: wprep(n))
                mm1_d[g] = sc.dot(640, a_slots(5, it), lambda att, g=g: mm1(g, att))
                after_dot()
            if 2 <= g < G + 2:
                before_dot()
                mm2_d[g - 2] = sc.dot(640, a_slots(2, it), lambda att, g=g: mm2(g - 2, att))
                after_dot()
    t_it[NIT + 1] = sc.t

    prev = None
    for g in range(G):
        if CFG["pin_scan"] & (1 << SEQ[g // NT][0]):
            s_ = sc.stream(scan(g), W_SCAN, mm1_d[g].t0 + CFG["sc0"],
                           min(mm2_d[g].t0 - 100, mm1_d[g].t0 + CFG["sc0"] + CFG["scw"]), after=[prev] if prev else [])
        else:
            def nat(g=g):
                for _ in scan(g):
                    pass
                return
                yield
            s_ = sc.stream(nat(g), 1, mm1_d[g].t0 + 700, mm1_d[g].t0 + 700, after=[prev] if prev else [])
        mm2_d[g].requires.append(s_)
        prev = s_
    s1_s, fin_s = {}, {}
    for c in FFT_TILES:
        s1_s[c] = sc.stream(conv_s1(c), W_S1, TS1 + c * DELTA, TS1 + (c + 1) * DELTA - 200,
                            after=[s1_s[c - 1]] if c else [], needs=[bar["t%d" % c]] if FULL else [], orw=CFG["orw_s1"])
        tr_s[c] = sc.stream(conv_tr(c), 16, TS1 + c * DELTA, TS1 + (c + 0.5) * DELTA,
                            after=[s1_s[c - 1]] if c else [], needs=[bar["t%d" % c]] if FULL else [],
                            orw=CFG["orw_tr"])
        mx_first[c].requires.append(s1_s[c])
        span = 5500 if c < NT - 1 else 3000
        fin_s[c] = sc.stream(conv_fin(c), W_FIN, mx_end[c] + 200, mx_end[c] + 200 + span,
                             after=[fin_s[c - 1]] if c else [], orw=CFG["orw_fin"])
    pre_s, post_s = {}, {}
    for it in range(NIT):
        l, c = SEQ[it]
        gen = pre1(c) if l == 0 else pre2(c)
        if it == 0:
            pre_s[it] = sc.stream(gen, 16, -2000, -1000, needs=[bar["x0"]] if FULL else [])
        else:
            t0 = t_it[it - 1] + 100
            aft = [pre_s[it - 1]]
            nd = []
            if not FULL:
                pass
            elif it == 1:
                t0 = t_it[0] + 0.5 * (t_it[1] - t_it[0])
                nd = [bar["w2"]]
            elif it == 2:
                nd = [bar["w4"]]
            elif it == 3:
                nd = [bar["t0"]]
            elif 4 <= it <= 7:
                nd = [bar["t%d" % (it - 3)]]
            if it >= 3:
                aft.append(post_s[it - 3])
            if FULL and it == NCH:
                t0 = max(t0, fin_s[NT - 1].t1)
                aft.append(fin_s[NT - 1])
            pre_s[it] = sc.stream(gen, 16, t0, t_it[it] - 450, after=aft, needs=nd)
        mm1_d[NT * it].requires.append(pre_s[it])
        gen = post1(c) if l == 0 else post2(c)
        t0 = mm2_d[NT * it + NT - 1].t0 + 640 + 150
        t1 = t_it[it + 2] - 100 if it + 2 <= NIT else t0 + 1000
        post_s[it] = sc.stream(gen, 16 if l == 0 else 36, t0, t1, after=[post_s[it - 1]] if it else [])
    if FULL:
        bar["o0"].requires.append(post_s[NCH + OSPLIT[0][1] - 1])
        bar["o1"].requires.append(post_s[NCH + OSPLIT[1][1] - 1])
        bar["o2"].requires.append(post_s[NCH + OSPLIT[2][1] - 1])
    sc.run()
    if _os.environ.get("VERBOSE"):
        print("dropped pins:", sc.dropped)
    if FULL:
        cp_o(3).start()
        for i in range(4):
            cp_o(i).wait()
        assert not started


_ZMASK = np.concatenate([np.zeros((8, 128), np.int32), np.arange(1024, dtype=np.int32).reshape(8, 128)], axis=1)
_ZS = np.array([0, 7, 3, 11], np.int32)


@jax.jit
def pallas_interleave_layers__ssm_conv_s5__ssm_conv_h3__prompt_kernel(
    A_x, A_Lambda_re, A_Lambda_im, A_B_re, A_B_im, A_C_re, A_C_im, A_log_dt, A_Dskip,
    B_q, B_k, B_v, B_shift_k, B_ssm_k, B_ssm_D,
):
    del B_q
    x2 = A_x.reshape(S, D)
    k2 = B_k.reshape(S, D)
    v2 = B_v.reshape(S, D)
    shkT = B_shift_k.T
    hbm = pl.BlockSpec(memory_space=pltpu.HBM)
    vm = pl.BlockSpec(memory_space=pltpu.VMEM)
    sm = pl.BlockSpec(memory_space=pltpu.SMEM)
    out = pl.pallas_call(
        _kernel,
        out_shape=jax.ShapeDtypeStruct((S, D), F32),
        in_specs=[vm] * 7 + [sm] + [hbm] * 10,
        out_specs=hbm,
        scratch_shapes=[
            pltpu.VMEM((S, D), BF16),
            pltpu.VMEM((4, D, D), BF16),
            pltpu.VMEM((D, D), I32),
            pltpu.VMEM((D // 2, 2 * D), I32),
            pltpu.VMEM((10, 8, D), F32),
            pltpu.VMEM((8, 8, D), F32),
            pltpu.VMEM((2, 2, 8, D), F32),
            pltpu.VMEM((NT, S, 128), BF16),
            pltpu.VMEM((NT, S, 128), BF16),
            pltpu.VMEM((NT, 128, S), BF16),
            pltpu.VMEM((NK1, 64, 128), I32),
            pltpu.VMEM((NK1, 64, 128), I32),
            pltpu.VMEM((S + 8, 128), F32),
            pltpu.VMEM((S + 8, 128), F32),
            pltpu.VMEM((S + 8, 128), F32),
            pltpu.VMEM((2 * 16 * 64, 256), I32),
            pltpu.VMEM((2 * 16 * 64, 256), I32),
            pltpu.VMEM((NK1 * 128 + 8, 128), F32),
            pltpu.VMEM((NK1 * 128 + 8, 128), F32),
            pltpu.VMEM((NCH, NT, PADR, 128), F32),
            pltpu.VMEM((S + 8, D), F32),
            pltpu.VMEM((T + 8, D), F32),
            pltpu.VMEM((T + 8, D), F32),
            pltpu.VMEM((T + 8, D), F32),
            pltpu.VMEM((T // 2, D), I32),
            pltpu.VMEM((T // 2, D), I32),
            pltpu.VMEM((T // 2, 256), I32),
            pltpu.VMEM((T // 2, 256), I32),
            pltpu.VMEM((T // 2, 256), I32),
            pltpu.VMEM((T // 2, 256), I32),
            pltpu.VMEM((NT, PADR, 128), F32),
            pltpu.VMEM((S, D), F32),
            pltpu.SemaphoreType.DMA((NCH,)),
            pltpu.SemaphoreType.DMA((4 * NT,)),
            pltpu.SemaphoreType.DMA((3 * NT,)),
            pltpu.SemaphoreType.DMA((2,)),
            pltpu.SemaphoreType.DMA((4,)),
        ],
        compiler_params=pltpu.CompilerParams(vmem_limit_bytes=100 * 1024 * 1024),
    )(A_Lambda_re, A_Lambda_im, A_log_dt, A_Dskip, shkT, B_ssm_D, _ZMASK, _ZS,
      x2, A_B_re, A_B_im, A_C_re, A_C_im, k2, v2, B_ssm_k, _FM, _GM)
    return out.reshape(1, S, D)
```

```python
import numpy as np
import jax
import jax.numpy as jnp
import jax.experimental.pallas as pl
import jax.experimental.pallas.tpu as pltpu

S, D = 2048, 640
NT = D // 128
TS = 32
T = 8 * TS
NCH = S // T
PITCH = TS + 1
PADR = 304
NFFT = 4096
NK1 = 33
C8 = float(np.sqrt(0.5))
F32 = jnp.float32
BF16 = jnp.bfloat16


class Bf:
    def __init__(self):
        self.tab = {}; self.keep = []
    def _plus(self, va, vb):
        key = ('+',) + tuple(sorted((id(va), id(vb))))
        if key not in self.tab:
            self.tab[key] = va + vb; self.keep.append((va, vb))
        return self.tab[key]
    def _minus(self, va, vb):
        k1 = ('-', id(va), id(vb)); k2 = ('-', id(vb), id(va))
        if k1 in self.tab: return (1, self.tab[k1])
        if k2 in self.tab: return (-1, self.tab[k2])
        self.tab[k1] = va - vb; self.keep.append((va, vb))
        return (1, self.tab[k1])
    def _times(self, va, c):
        key = ('*', id(va), c)
        if key not in self.tab:
            self.tab[key] = va * c; self.keep.append(va)
        return self.tab[key]
    def radd(self, a, b):
        if a is None: return b
        if b is None: return a
        sa, va = a; sb, vb = b
        if sa == sb: return (sa, self._plus(va, vb))
        s, v = self._minus(va, vb)
        return (s * sa, v)
    @staticmethod
    def rneg(a):
        return None if a is None else (-a[0], a[1])
    def rsub(self, a, b):
        return self.radd(a, self.rneg(b))
    def rmul(self, a, c):
        if a is None or c == 0.0: return None
        s = 1 if c > 0 else -1
        c = abs(c)
        if c == 1.0: return (a[0] * s, a[1])
        return (a[0] * s, self._times(a[1], c))
    def cadd(self, a, b): return (self.radd(a[0], b[0]), self.radd(a[1], b[1]))
    def csub(self, a, b): return (self.rsub(a[0], b[0]), self.rsub(a[1], b[1]))
    def cconj(self, a): return (a[0], self.rneg(a[1]))
    def cmuli(self, a, p):
        p %= 4
        if p == 0: return a
        if p == 1: return (self.rneg(a[1]), a[0])
        if p == 2: return (self.rneg(a[0]), self.rneg(a[1]))
        return (a[1], self.rneg(a[0]))
    def cmul_w(self, a, num, den):
        num %= den
        if (4 * num) % den == 0: return self.cmuli(a, 4 * num // den)
        if (8 * num) % den == 0:
            o = 8 * num // den
            re = self.rmul(self.rsub(a[0], a[1]), C8)
            im = self.rmul(self.radd(a[0], a[1]), C8)
            return self.cmuli((re, im), (o - 1) // 2)
        wr = float(np.cos(2 * np.pi * num / den)); wi = float(np.sin(2 * np.pi * num / den))
        re = self.rsub(self.rmul(a[0], wr), self.rmul(a[1], wi))
        im = self.radd(self.rmul(a[0], wi), self.rmul(a[1], wr))
        return (re, im)
    def fft(self, x, sgn):
        n = len(x)
        def get(v): return v() if callable(v) else v
        if n == 1: return [get(x[0])]
        if n == 2:
            a, b = get(x[0]), get(x[1])
            return [self.cadd(a, b), self.csub(a, b)]
        if n == 4:
            x0, x2 = get(x[0]), get(x[2])
            a = self.cadd(x0, x2); b = self.csub(x0, x2)
            x1, x3 = get(x[1]), get(x[3])
            c = self.cadd(x1, x3); d = self.csub(x1, x3)
            wd = self.cmuli(d, sgn)
            return [self.cadd(a, c), self.cadd(b, wd), self.csub(a, c), self.csub(b, wd)]
        m = n // 4
        u = [self.fft([x[b2 + m * b1] for b1 in range(4)], sgn) for b2 in range(m)]
        out = [None] * n
        for k1 in range(4):
            t = [self.cmul_w(u[b2][k1], sgn * b2 * k1, n) for b2 in range(m)]
            y = self.fft(t, sgn)
            for k2 in range(m):
                out[k1 + 4 * k2] = y[k2]
        return out

    def odd_fwd(self, d, N, emit, scale):
        q = N // 4
        def z(b):
            def th():
                p = d[b]() if callable(d[b]) else d[b]
                r = d[b + q]() if callable(d[b + q]) else d[b + q]
                return self.cmul_w((p, self.rneg(r)), -b, N)
            return th
        Y = self.fft([z(b) for b in range(q)], -1)
        for j in range(q):
            k = 4 * j + 1
            if 2 * k <= N: emit(k * scale, Y[j])
            else: emit((N - k) * scale, self.cconj(Y[j]))
    def real_fwd(self, x, N, emit, scale):
        if N == 2:
            emit(0, (self.radd(x[0], x[1]), None)); emit(scale, (self.rsub(x[0], x[1]), None)); return
        h = N // 2
        s = [self.radd(x[b], x[b + h]) for b in range(h)]
        d = [self.rsub(x[b], x[b + h]) for b in range(h)]
        if N == 4:
            emit(scale, (d[0], self.rneg(d[1])))
        else:
            self.odd_fwd(d, N, emit, scale)
        self.real_fwd(s, h, emit, 2 * scale)

    def odd_inv(self, V, N, scale):
        q = N // 4
        def U(j):
            k = 4 * j + 1
            if 2 * k <= N: return lambda: V(k * scale)
            return lambda: self.cconj(V((N - k) * scale))
        zt = self.fft([U(j) for j in range(q)], +1)
        out = [None] * (2 * q)
        for b in range(q):
            t = self.cmul_w(zt[b], b, N)
            out[b] = t[0]; out[b + q] = self.rneg(t[1])
        return out
    def real_inv(self, V, N, scale):
        if N == 2:
            a, b = V(0)[0], V(scale)[0]
            return [self.radd(a, b), self.rsub(a, b)]
        h = N // 2
        if N == 4:
            v1 = V(scale)
            qq = [v1[0], self.rneg(v1[1])]
        else:
            qq = self.odd_inv(V, N, scale)
        p = self.real_inv(V, h, 2 * scale)
        return [self.radd(p[b], qq[b]) for b in range(h)] + [self.rsub(p[b], qq[b]) for b in range(h)]


def _vals(*cs):
    out = []
    for c in cs:
        for p in c:
            if p is not None:
                out.append(p[1])
    return out


class BfH(Bf):
    def __init__(self):
        super().__init__()
        self.n0 = 0

    def dw(self):
        n = len(self.tab)
        w, self.n0 = n - self.n0, n
        return w

    def odd_fwd_g(self, d, N, emit, scale):
        q = N // 4

        def z(b):
            def th():
                p = d[b]() if callable(d[b]) else d[b]
                r = d[b + q]() if callable(d[b + q]) else d[b + q]
                return self.cmul_w((p, self.rneg(r)), -b, N)
            return th
        zs = [z(b) for b in range(q)]
        m = q // 4
        u = []
        for b2 in range(m):
            g = self.fft([zs[b2 + m * b1] for b1 in range(4)], -1)
            u.append(g)
            yield _vals(g[3])[:1], self.dw() + 8
        for k1 in range(4):
            t = [self.cmul_w(u[b2][k1], -b2 * k1, q) for b2 in range(m)]
            y = self.fft(t, -1)
            outs = []
            for k2 in range(m):
                k = 4 * (k1 + 4 * k2) + 1
                if 2 * k <= N:
                    outs.append((k * scale, y[k2]))
                else:
                    outs.append(((N - k) * scale, self.cconj(y[k2])))
            dd = emit(outs)
            yield dd, self.dw() + 12

    def fwd_q2(self, x, emit):
        def d(b):
            return lambda: self.rsub(x[b](), x[b + 16]())
        yield from self.odd_fwd_g([d(b) for b in range(16)], 32, emit, 2)

    def fwd_q0(self, x, emit):
        s = [None] * 16
        for b in range(8):
            s[b] = self.radd(x[b](), x[b + 16]())
            s[b + 8] = self.radd(x[b + 8](), x[b + 24]())
        outs = []
        self.real_fwd(s, 16, lambda k, c: outs.append((k, c)), 4)
        outs.sort(key=lambda kc: (kc[0] not in (0, 32), kc[0]))
        w = self.dw()
        yield emit(outs[:5]), w + 12
        yield emit(outs[5:]), 12

    def fwd_even_g(self, x, emit):
        s = [self.radd(x[b], x[b + 16]) for b in range(16)]
        d = [self.rsub(x[b], x[b + 16]) for b in range(16)]
        yield from self.odd_fwd_g(d, 32, emit, 2)
        outs = []
        self.real_fwd(s, 16, lambda k, c: outs.append((k, c)), 4)
        outs.sort(key=lambda kc: (kc[0] not in (0, 32), kc[0]))
        w = self.dw()
        yield emit(outs[:5]), w + 12
        yield emit(outs[5:]), 12

    def inv_g(self, V, emit, rel=lambda: None):
        def odd_stage1(N, scale):
            q = N // 4
            m = q // 4

            def U(j):
                k = 4 * j + 1
                if 2 * k <= N:
                    return lambda: V(k * scale)
                return lambda: self.cconj(V((N - k) * scale))
            u = []
            deps = []
            for b2 in range(m):
                g = self.fft([U(b2 + m * b1) for b1 in range(4)], +1)
                u.append(g)
                deps.append((_vals(g[3])[:1], self.dw() + 8))
            return u, deps

        def odd_stage2(u, N, k1):
            q = N // 4
            m = q // 4
            t = [self.cmul_w(u[b2][k1], b2 * k1, q) for b2 in range(m)]
            y = self.fft(t, +1)
            res = {}
            for k2 in range(m):
                b = k1 + 4 * k2
                tt = self.cmul_w(y[k2], b, N)
                res[b] = tt[0]
                res[b + q] = self.rneg(tt[1])
            return res
        rel()
        uo, deps = odd_stage1(64, 1)
        for dd in deps:
            yield dd
        o = {}
        for k1 in range(4):
            o.update(odd_stage2(uo, 64, k1))
            yield [o[b][1] for b in sorted(o) if b % 4 == k1 and (b // 4) % 2 == 0], self.dw() + 4
        rel()
        uq, deps = odd_stage1(32, 2)
        for dd in deps:
            yield dd
        y1 = {}
        for k1 in range(4):
            qq = odd_stage2(uq, 32, k1)
            for b in sorted(qq):
                y1[b] = self.radd(o[b], qq[b])
                y1[b + 16] = self.rsub(o[b + 16], qq[b])
            yield [y1[b][1] for b in sorted(qq)], self.dw() + 4
        rel()
        p = self.real_inv(V, 16, 4)
        yield [p[5][1]], self.dw() + 16
        for k1 in range(4):
            outs = []
            for b in range(k1, 32, 4):
                outs.append((b, self.radd(y1[b], p[b % 16])))
            dd = emit(outs)
            yield dd, self.dw() + 16


def _fwd_plan():
    Y = {}
    order = []

    def emit(outs):
        for k, c in outs:
            Y[k] = c
            if k != 32:
                order.append(k)
        return []
    xs = [(1, np.full((1,), float(i + 1) ** 1.37)) for i in range(32)]
    xl = [(lambda v=v: v) for v in xs]
    we = sum(w for _, w in BfH().fwd_q2(xl, emit)) + sum(w for _, w in BfH().fwd_q0(xl, emit))
    wo = sum(w for _, w in BfH().odd_fwd_g(xs, 64, emit, 1))
    full = {k: ((1, np.full((1,), 1.0 + k)), None if k in (0, 32) else (1, np.full((1,), 2.5 + k)))
            for k in range(NK1)}
    wi = sum(w for _, w in BfH().inv_g(lambda k: full[k], lambda o: []))
    sg = {k: tuple(0 if c is None else c[0] for c in Y[k]) for k in range(NK1)}
    slot = {k: (i // 2, i % 2) for i, k in enumerate(order)}
    slot[32] = slot[0]
    return sg, slot, we + wo, wi


_FSG, _FSLOT, _W_FWD, _W_INV = _fwd_plan()

def _pack_rows(m):
    b = m.astype(np.float32).astype(jnp.bfloat16).view(np.uint16).astype(np.uint32)
    w = b[..., 0::2, :] | (b[..., 1::2, :] << 16)
    return w.view(np.int32)


def _dft_matrices():
    r = np.arange(64)
    k2 = np.arange(64)
    Fm = np.zeros((NK1, 128, 128), np.float64)
    Gm = np.zeros((NK1, 128, 128), np.float64)
    col = (16 * (r // 8) + (r % 8))
    for k1 in range(NK1):
        th = 2 * np.pi * np.outer(k1 + 64 * k2, r) / NFFT
        c, s = np.cos(th), np.sin(th)
        sr, si = _FSG[k1]
        Fr, Fi = np.zeros((64, 128)), np.zeros((64, 128))
        if k1 == 0:
            Fr[:, col] = c * sr
            Fi[:, col] = -s * sr
        elif k1 == 32:
            Fr[:, col + 8] = c * sr
            Fi[:, col + 8] = -s * sr
        else:
            Fr[:, col] = c * sr
            Fr[:, col + 8] = s * si
            Fi[:, col] = -s * sr
            Fi[:, col + 8] = c * si
        Fm[k1][col] = Fr
        Fm[k1][col + 8] = Fi
        sc = (1.0 if k1 in (0, 32) else 2.0) / NFFT
        ct, st = c.T * sc, s.T * sc
        Gm[k1][0:64][:, col] = ct
        Gm[k1][0:64][:, col + 8] = -st
        Gm[k1][64:128][:, col] = st
        Gm[k1][64:128][:, col + 8] = ct
    return _pack_rows(Fm), _pack_rows(Gm)


_FM, _GM = _dft_matrices()


def _cmul(ar, ai, br, bi):
    return ar * br - ai * bi, ar * bi + ai * br


def _cmul_add(lr, li, hr, hi, ur, ui):
    return (lr * hr - li * hi) + ur, (lr * hi + li * hr) + ui


def _layernorm(x):
    m = jnp.mean(x, axis=-1, keepdims=True)
    xc = x - m
    v = jnp.mean(xc * xc, axis=-1, keepdims=True)
    return xc * jax.lax.rsqrt(v + 1e-5)


def _nt_dot(a, b):
    return jax.lax.dot_general(a, b, (((1,), (1,)), ((), ())), preferred_element_type=F32)


I32 = jnp.int32
import os as _os
CFG = dict(
    bench=_os.environ.get("BENCH", ""),
    opq=int(_os.environ.get("OPQ", "0")),
    pin_scan=int(_os.environ.get("PINSCAN", "0")),
    nch=int(_os.environ.get("NCHB", "4")),
    orw=int(_os.environ.get("ORW", "1")),
    lock=int(_os.environ.get("LOCKB", "1")),
    gate=int(_os.environ.get("GATE", "0")),
    glag=int(_os.environ.get("GLAG", "2")),
    o_kvc=int(_os.environ.get("OKVC", "2")),
    o_pre=int(_os.environ.get("OPRE", "2")),
    o_post=int(_os.environ.get("OPOST", "2")),
    o_exit=int(_os.environ.get("OEXIT", "4")),
    ssa=int(_os.environ.get("SSA", "0")),
    rel=int(_os.environ.get("REL", "0")),
    lhs2=int(_os.environ.get("LHS2", "0")),
    sc0=int(_os.environ.get("SC0", "700")),
    scw=int(_os.environ.get("SCW", "650")),
    rslot=int(_os.environ.get("RSLOT", "0")),
    skip=_os.environ.get("SKIP", "").split(","),
    lhs=int(_os.environ.get("LHS", "0")),
    orw_tr=int(_os.environ.get("ORWTR", "4")),
    orw_fin=int(_os.environ.get("ORWFIN", "2")),
    orw_s1=int(_os.environ.get("ORWS1", "2")),
    scopes=int(_os.environ.get("SCOPES", "0")),
    nodma=int(_os.environ.get("NODMA", "0")),
    lead1=int(_os.environ.get("LEAD1", "300")),
    lead2=int(_os.environ.get("LEAD2", "500")),
    slotmax=int(_os.environ.get("SLOTMAX", "384")),
)


LOCK, UNLOCK = object(), object()


class _Dot:
    def __init__(self, t0, slots, emit):
        self.t0 = t0
        self.slots = sorted(((t0 + rt, key) for rt, key in slots), key=lambda tk: tk[0])
        self.emit = emit
        self.att = {}
        self.requires = []


class _Barrier:
    def __init__(self, f):
        self.f = f
        self.emitted = False
        self.requires = []


class _Stream:
    def __init__(self, gen, wtot, t0, t1, after=(), needs=(), orw=None):
        self.gen, self.wtot, self.t0, self.t1 = gen, float(wtot), t0, t1
        self.after, self.needs = list(after), list(needs)
        self.orw = orw or CFG["orw"]
        self.cum = 0.0
        self.done = False

    def now(self):
        return self.t0 + (self.t1 - self.t0) * min(1.0, self.cum / self.wtot)


class _Sched:
    def __init__(self):
        self.items, self.streams = [], []
        self.t, self.pos = 0.0, 0
        self.lock = None
        self.scope, self.nseg = None, 0
        self.dropped = 0
        self.cur = None
        self.tokens = []

    def fn(self, f):
        self.items.append(f)

    def barrier(self, f):
        b = _Barrier(f)
        self.items.append(b)
        return b

    def dot(self, dur, slots, emit):
        d = _Dot(self.t, slots, emit)
        self.items.append(d)
        self.t += dur
        return d

    def stream(self, gen, wtot, t0, t1, after=(), needs=(), orw=None):
        s = _Stream(gen, wtot, t0, t1, after, needs, orw)
        self.streams.append(s)
        return s

    def token_at(self, t):
        best = None
        for ts, th in self.tokens[-400:]:
            if ts <= t and (best is None or ts > best[0]):
                best = (ts, th)
        return best

    def _attach1(self, t, d):
        stop = self.pos
        while stop < len(self.items) and not isinstance(self.items[stop], _Barrier):
            stop += 1
        for it in self.items[self.pos:stop]:
            if isinstance(it, _Dot):
                for ts, key in it.slots:
                    if ts >= t and key not in it.att:
                        it.att[key] = d
                        return ts
        for it in reversed(self.items[self.pos:stop]):
            if isinstance(it, _Dot):
                for ts, key in reversed(it.slots):
                    if key not in it.att:
                        it.att[key] = d
                        return ts
        self.dropped += 1
        return t

    def _attach(self, t0, t1, deps, n):
        if not deps:
            return
        if isinstance(deps[0], list):
            chunks = deps
        else:
            chunks = [deps[i:i + n] for i in range(0, len(deps), n)]
        for i, ch in enumerate(chunks):
            d = None
            for v in ch:
                vi = v if v.dtype == I32 else pltpu.bitcast(v, I32)
                d = vi if d is None else d | vi
            self._attach1(t0 + (t1 - t0) * (i + 1.0) / len(chunks), d)

    def _step(self, s):
        for b in s.needs:
            while not b.emitted:
                self._emit_next()
        for a in s.after:
            self._drain(a)
        try:
            self.cur = s
            deps, w = next(s.gen)
        except StopIteration:
            s.done = True
            if self.lock is s:
                self.lock = None
            return
        if deps is LOCK:
            self.lock = s
            return
        if deps is UNLOCK:
            self.lock = None
            return
        ta = s.now()
        s.cum += w
        self._attach(ta, s.now(), deps, s.orw)

    def _drain(self, s):
        while not s.done:
            self._step(s)

    def _emit_next(self):
        it = self.items[self.pos]
        if isinstance(it, _Dot):
            for s in it.requires:
                self._drain(s)
            self.pos += 1
            it.emit(it.att)
        elif isinstance(it, _Barrier):
            for s in it.requires:
                self._drain(s)
            self.pos += 1
            if CFG["scopes"]:
                if self.scope is not None:
                    self.scope.__exit__(None, None, None)
                self.nseg += 1
                with jax.named_scope("s_wait%02d" % self.nseg):
                    it.f()
                self.scope = jax.named_scope("s_seg%02d" % self.nseg)
                self.scope.__enter__()
            else:
                it.f()
            it.emitted = True
        else:
            self.pos += 1
            it()

    def _advance(self, t):
        while self.pos < len(self.items):
            it = self.items[self.pos]
            if isinstance(it, _Dot) and any(ts >= t and key not in it.att for ts, key in it.slots):
                return
            self._emit_next()

    def run(self):
        while True:
            live = [s for s in self.streams if not s.done]
            if not live:
                break
            s = self.lock if self.lock is not None else min(live, key=lambda z: z.now())
            self._advance(s.now())
            if not s.done:
                self._step(s)
        while self.pos < len(self.items):
            self._emit_next()
        if self.scope is not None:
            self.scope.__exit__(None, None, None)


def _kernel(lre_ref, lim_ref, ldt_ref, dsk_ref, shk_ref, sD_ref, zm_ref, zs_ref,
            x_hbm, bre_hbm, bim_hbm, cre_hbm, cim_hbm, k_hbm, v_hbm, sk_hbm, f_hbm, g_hbm,
            o_hbm,
            xin, wst, bw, cw, tab, par, carry, kin, vin, skin, fm, gm,
            kf, kvf, skt, ybf0, ybf1, vscr0, vscr1, yscr, x1, xa0, xa1, xa2, lnb0, lnb1, hb0, hb1, hb2, hb3, pad, ostg,
            sem_x, sem_w, sem_kv, sem_fg, sem_o):

    started = set()

    class _Cp:
        def __init__(self, key, desc):
            self.key, self.desc = key, desc

        def start(self):
            assert self.key not in started, self.key
            started.add(self.key)
            if not CFG["nodma"]:
                self.desc.start()

        def wait(self):
            assert self.key in started, self.key
            started.remove(self.key)
            if not CFG["nodma"]:
                self.desc.wait()

    def cp_x(c):
        rs = pl.ds(T * c, T)
        return _Cp(("x", c), pltpu.make_async_copy(x_hbm.at[rs, :], xin.at[rs, :], sem_x.at[c]))

    def cp_w(n, which):
        src = (bre_hbm, bim_hbm, cre_hbm, cim_hbm)[which]
        if which < 2:
            return _Cp(("w", n, which), pltpu.make_async_copy(
                src.at[pl.ds(128 * n, 128), :], wst.at[which, pl.ds(128 * n, 128), :], sem_w.at[4 * n + which]))
        return _Cp(("w", n, which), pltpu.make_async_copy(
            src.at[:, pl.ds(128 * n, 128)], wst.at[which, :, pl.ds(128 * n, 128)], sem_w.at[4 * n + which]))

    def cp_kv(c, which):
        src, dst = ((k_hbm.at[:, pl.ds(128 * c, 128)], kin), (v_hbm.at[:, pl.ds(128 * c, 128)], vin),
                    (sk_hbm.at[pl.ds(128 * c, 128), :], skin))[which]
        return _Cp(("kv", c, which), pltpu.make_async_copy(src, dst.at[c], sem_kv.at[3 * c + which]))

    cp_f = _Cp(("f",), pltpu.make_async_copy(f_hbm, fm, sem_fg.at[0]))
    cp_g = _Cp(("g",), pltpu.make_async_copy(g_hbm, gm, sem_fg.at[1]))
    OSPLIT = ((0, 4), (4, 6), (6, 7), (7, 8))

    def cp_o(i):
        lo, hi = OSPLIT[i]
        rs = pl.ds(T * lo, T * (hi - lo))
        return _Cp(("o", i), pltpu.make_async_copy(ostg.at[rs, :], o_hbm.at[rs, :], sem_o.at[i]))

    def tile_start(c):
        for w in range(3):
            cp_kv(c, w).start()

    def tile_wait(c):
        for w in range(3):
            cp_kv(c, w).wait()

    if CFG["bench"] == "":
        cp_x(0).start()
        for w in range(4):
            cp_w(0, w).start()

    def row(ref):
        return ref[...].astype(F32)[None, :]

    lre, lim, ldt = row(lre_ref), row(lim_ref), row(ldt_ref)
    dt = jnp.exp(ldt).astype(BF16).astype(F32)
    zr, zi = dt * lre, dt * lim
    mag = jnp.exp(zr)
    lbr, lbi = mag * jnp.cos(zi), mag * jnp.sin(zi)
    inv = 1.0 / (lre * lre + lim * lim)
    nr, ni = lbr - 1.0, lbi
    fr, fi = (nr * lre + ni * lim) * inv, (ni * lre - nr * lim) * inv
    sub = jax.lax.broadcasted_iota(jnp.int32, (8, D), 0)

    def b8(v):
        return jnp.broadcast_to(v, (8, D))

    tab[0] = b8(lbr)
    tab[1] = b8(lbi)
    pr, pi = lbr, lbi
    for _ in range(5):
        pr, pi = _cmul(pr, pi, pr, pi)
    tab[2] = b8(pr)
    tab[3] = b8(pi)
    for q, sh in enumerate((1, 2, 4)):
        tab[4 + 2 * q] = jnp.where(sub >= sh, b8(pr), 0.0)
        tab[5 + 2 * q] = jnp.where(sub >= sh, b8(pi), 0.0)
        pr, pi = _cmul(pr, pi, pr, pi)
    par[0] = b8(row(dsk_ref))
    par[1] = b8(row(sD_ref))
    shk = shk_ref[...].astype(F32)
    for lag in range(4):
        par[2 + lag] = b8(shk[lag:lag + 1, :])
    par[6] = b8(2.0 * fr)
    par[7] = b8(2.0 * fi)
    carry[...] = jnp.zeros(carry.shape, F32)
    kf[0:8, :] = jnp.zeros((8, 128), F32)

    fmask = zm_ref[:, 0:128] != 0
    z8 = pl.multiple_of(zs_ref[0], 8)

    def lt(n):
        return slice(128 * n, 128 * (n + 1))

    def tiles(v):
        r, l = v.shape
        return [v[8 * i:8 * i + 8, 128 * j:128 * (j + 1)] for i in range(r // 8) for j in range(l // 128)]

    def grp(deps, n):
        return [deps[i:i + n] for i in range(0, len(deps), n)]

    def opq(r0, n, bit=1):
        if not (CFG["opq"] & bit):
            return pl.ds(r0, n)
        return pl.ds(pl.multiple_of(z8 + r0, 8), n)

    def dyn(r0, n, stride=None):
        if stride is None:
            return pl.ds(pl.multiple_of(z8 + r0, 8), n)
        return pl.ds(z8 + r0, n, stride=stride)

    zvec = zm_ref[:, 0:128]

    def release(lead, kind=1):
        if not (CFG["rel"] & kind):
            return None
        tk = sc.token_at(sc.cur.now() - lead)
        if tk is None:
            return None
        v = pltpu.bitcast(tk[1](), I32) & zvec
        return pl.multiple_of(v[0, 0], 8)

    def at(z, r0, n, stride=None, aligned=True):
        if z is None:
            return pl.ds(r0, n) if stride is None else pl.ds(r0, n, stride=stride)
        if stride is not None:
            return pl.ds(z + r0, n, stride=stride)
        if aligned:
            return pl.ds(pl.multiple_of(z + r0, 8), n)
        return pl.ds(z + r0, n)

    def add_tokens(val, t0, tmap):
        r, l = val.shape
        for j in range(0, r // 8, 4):
            for i in range(l // 128):
                sc.tokens.append((t0 + tmap(j, i), lambda j=j, i=i: val[8 * j:8 * j + 8, 128 * i:128 * (i + 1)]))

    class Gate:
        def __init__(self, lag):
            self.lag, self.hist = lag, []

        def done(self, token):
            self.hist.append(token)

        def open(self, *stores):
            if len(self.hist) >= self.lag:
                tok = self.hist[-self.lag]
                for f in stores:
                    f(tok)

    def load_hooked(get, nrb, nk, att, keyf):
        rows_ = []
        for rb in range(nrb):
            cols = []
            for kk in range(nk):
                w = get(rb, kk)
                key = keyf(rb, kk)
                if key in att:
                    w = jnp.where(fmask, att[key], w)
                cols.append(w)
            rows_.append(cols[0] if nk == 1 else jnp.concatenate(cols, axis=1))
        return pltpu.bitcast(jnp.concatenate(rows_, axis=0), BF16)

    def a_slots(nk, it):
        sl_ = [(64 * tau - 256 + 32 * p, (tau, 7 - p)) for tau in range(10) for p in range(8)
               if 64 * tau - 256 + 32 * p < CFG["slotmax"]]
        lm = CFG["lhs"] if SEQ[min(it, NIT - 1)][0] == 0 else CFG["lhs2"]
        if lm & (1 if nk == 5 else 2):
            sl_ += [(64 * k + 16 * a, ("l", k, a)) for k in range(nk) for a in range(16)]
        return sl_

    sc = _Sched()
    st = {}

    def mm1(g, att):
        l, c, n = dec(g)
        lb = (lnb0, lnb1)[c % 2]
        lhs = jnp.concatenate(st["ln", l, c], axis=0) if CFG["ssa"] & 2 else load_hooked(lambda rb, kk: lb[pl.ds(8 * rb, 8), pl.ds(128 * kk, 128)], 16, 5, att,
                          lambda rb, kk: ("l", kk, rb))
        rhs = load_hooked(lambda rb, kk: bw[pl.ds(128 * n + 8 * rb, 8), pl.ds(128 * kk, 128)], 16, 5, att,
                          lambda rb, kk: (5 * (rb // 8) + kk, rb % 8))
        st["u", g] = _nt_dot(lhs, rhs)
        add_tokens(st["u", g], mm1_d[g].t0, lambda j, i: 64 * (5 * i + 4) + 8 * j + 60)

    hbufs = (hb0, hb1, hb2, hb3)
    ybfs = (ybf0, ybf1)
    vscrs = (vscr0, vscr1)
    xas = (xa0, xa1, xa2)

    W_SCAN = 8 * 36 + 70 + 16 * 24

    def scan(g):
        layer, c, n = dec(g)
        u = st.pop(("u", g))
        sl = lt(n)
        lr, li = tab[0, :, sl], tab[1, :, sl]
        ur = [u[8 * j:8 * j + 8, 0:128] for j in range(TS)]
        ui = [u[8 * j:8 * j + 8, 128:256] for j in range(TS)]
        er, ei = ur[0], ui[0]
        for j in range(1, TS):
            er, ei = _cmul_add(lr, li, er, ei, ur[j], ui[j])
            if j % 4 == 3:
                yield [er], 36
        sub1 = jax.lax.broadcasted_iota(jnp.int32, (8, 128), 0)
        gr = jnp.where(sub1 == 0, carry[layer, 0, :, sl], pltpu.roll(er, 1, 0))
        gi = jnp.where(sub1 == 0, carry[layer, 1, :, sl], pltpu.roll(ei, 1, 0))
        for q, sh in enumerate((1, 2, 4)):
            gr, gi = _cmul_add(tab[4 + 2 * q, :, sl], tab[5 + 2 * q, :, sl],
                               pltpu.roll(gr, sh, 0), pltpu.roll(gi, sh, 0), gr, gi)
        nr_, ni_ = _cmul_add(tab[2, :, sl], tab[3, :, sl], gr, gi, er, ei)
        cr_ = jnp.broadcast_to(nr_[7:8, :], (8, 128))
        ci_ = jnp.broadcast_to(ni_[7:8, :], (8, 128))
        carry[layer, 0, :, sl] = cr_
        carry[layer, 1, :, sl] = ci_
        yield [gr, gi, cr_, ci_], 70
        hr, hi = gr, gi
        for a in range(TS // 2):
            two = []
            for j in (2 * a, 2 * a + 1):
                hr, hi = _cmul_add(lr, li, hr, hi, ur[j], ui[j])
                two.append(jnp.concatenate([hr, hi], axis=1))
            if CFG["ssa"] & 1:
                st.setdefault(("h", g), []).append(jnp.concatenate(two, axis=0).astype(BF16))
                yield [hr, hi], 24
                continue
            hbuf = hbufs[g % 4]
            hbuf[pl.ds(8 * a, 8), :] = pltpu.bitcast(jnp.concatenate(two, axis=0).astype(BF16), I32)
            yield [hbuf[pl.ds(8 * a, 8), pl.ds(128 * h_, 128)] for h_ in range(2)], 24

    def mm2(g, att):
        layer, c, n = dec(g)
        hb = hbufs[g % 4]
        h = jnp.concatenate(st.pop(("h", g)), axis=0) if CFG["ssa"] & 1 else load_hooked(lambda rb, kk: hb[pl.ds(8 * rb, 8), pl.ds(128 * kk, 128)], 16, 2, att,
                        lambda rb, kk: ("l", kk, rb))
        rhs = load_hooked(lambda rb, kk: cw[pl.ds(8 * rb, 8), pl.ds(256 * n + 128 * kk, 128)], 40, 2, att,
                          lambda rb, kk: (2 * (rb // 8) + kk, rb % 8))
        yn = _nt_dot(h, rhs)
        add_tokens(yn, mm2_d[g].t0, lambda j, i: 64 * (2 * i + 1) + 8 * j + 60)
        st["y", layer, c] = yn if n == 0 else st["y", layer, c] + yn

    def wwait(n):
        for w in range(4):
            cp_w(n, w).wait()
        if n + 2 < NT:
            for w in range(4):
                cp_w(n + 2, w).start()
        if n == 1:
            cp_x(2).start()
        if n == 2:
            cp_x(1).wait()
        if n == 3:
            tile_start(0)
        if n == NT - 1:
            cp_x(2).wait()
            cp_x(3).start()

    def wprep(n):
        for w in range(2):
            bw[pl.ds(128 * n + 64 * w, 64), :] = pltpu.bitcast(wst[w, pl.ds(128 * n, 128), :], I32)
        cr = wst[2, :, lt(n)].astype(F32)
        ci = wst[3, :, lt(n)].astype(F32)
        f_r, f_i = par[6, 0:1, lt(n)], par[7, 0:1, lt(n)]
        cc_ = jnp.concatenate([cr * f_r - ci * f_i, -(cr * f_i + ci * f_r)], axis=1).astype(BF16)
        cw[:, 256 * n:256 * (n + 1)] = pltpu.bitcast(cc_, I32)

    def yrow(c, sig, p):
        return (sig * 16 + p) * 64

    W_S1 = 32 * 80 + 16 * _W_FWD

    def conv_tr(c):
        for m in range(16 if "tr" not in CFG["skip"] else 0):
            z = release(330, 2)
            val = skin[c if z is None else z + c, :, pl.ds(128 * m, 128)].astype(F32).T
            if CFG["ssa"] & 16:
                for i_, t_ in enumerate(tiles(val)):
                    st["sk", c, 16 * m + i_] = t_
            else:
                skt[pl.ds(128 * m, 128), :] = val
            yield tiles(val), 1

    def conv_s1(c):
        w = [par[2 + lag, :, lt(c)] for lag in range(4)]
        for m in range(32 if "kvc" not in CFG["skip"] else 0):
            z = release(110, 4)
            kf[pl.ds(8 + 64 * m, 64), :] = kin[c if z is None else z + c, pl.ds(64 * m, 64), :].astype(F32)
            vv = vin[c if z is None else z + c, pl.ds(64 * m, 64), :].astype(F32)
            deps = []
            for i in range(8):
                t0 = 8 + 64 * m + 8 * i
                acc = kf[at(z, t0 - 3, 8, aligned=False), :] * w[3]
                acc = acc + kf[at(z, t0 - 2, 8, aligned=False), :] * w[2]
                acc = acc + kf[at(z, t0 - 1, 8, aligned=False), :] * w[1]
                acc = acc + kf[at(z, t0, 8), :] * w[0]
                kv = acc * vv[8 * i:8 * i + 8, :]
                if CFG["ssa"] & 16:
                    st["kv", c, 8 * m + i] = kv
                else:
                    kvf[pl.ds(t0 - 8, 8), :] = kv
                deps.append(kv)
            yield grp(deps, CFG["o_kvc"]), 90
        for sig in ((0, 1) if "cols" not in CFG["skip"] else ()):
            if sig == 1:
                sc._drain(tr_s[c])
                sc.cur = s1_s[c]
            src = kvf if sig == 0 else skt
            for rho in range(8):
                pend = {}

                def emit(outs):
                    vals = []
                    for k1, v in outs:
                        if k1 in (0, 32):
                            pend[k1] = v[0]
                            if len(pend) == 2:
                                vals.append((0, pend[0][1], pend[32][1]))
                        else:
                            vals.append((k1, v[0][1], v[1][1]))
                    deps = []
                    for i in range(0, len(vals), 2):
                        r0 = yrow(c, sig, _FSLOT[vals[i][0]][0]) + 8 * rho
                        two = jnp.concatenate(
                            [jnp.concatenate([vals[i + e][1], vals[i + e][2]], axis=0) for e in range(2)], axis=1)
                        if CFG["ssa"] & 32:
                            st["yb", c, sig, _FSLOT[vals[i][0]][0], rho] = two.astype(BF16)
                            deps += [vals[i + e][k_] for e in range(2) for k_ in (1, 2)]
                            continue
                        ybf = ybfs[c % 2]
                        ybf[pl.ds(r0, 8), :] = pltpu.bitcast(two.astype(BF16), I32)
                        deps += [ybf[pl.ds(r0, 8), pl.ds(128 * h_, 128)] for h_ in range(2)]
                    return deps

                def xs(z):
                    if CFG["ssa"] & 16:
                        return [(lambda b=b: (1, st["kv" if sig == 0 else "sk", c, 8 * b + rho])) for b in range(32)]
                    return [(lambda b=b: (1, src[at(z, 64 * b + 8 * rho, 8), :])) for b in range(32)]
                for part in range(3):
                    if CFG["lock"]:
                        yield LOCK, 0
                    z = release(90, 8)
                    if part == 0:
                        yield from BfH().fwd_q2(xs(z), emit)
                    elif part == 1:
                        yield from BfH().fwd_q0(xs(z), emit)
                    else:
                        yield from BfH().odd_fwd_g(xs(z), 64, emit, 1)
                    if CFG["lock"]:
                        yield UNLOCK, 0

    def f_slots(n):
        return [(8 * a, (0, a)) for a in range(n)]

    def conv_mx_steps(c):
        def fwd(k1, att):
            lhs = load_hooked(lambda rb, kk: fm[k1, pl.ds(8 * rb, 8), :], 8, 1, att, lambda rb, kk: (0, rb))
            p, s_ = _FSLOT[k1]
            if CFG["ssa"] & 32:
                rhs = jnp.concatenate(
                    [jnp.concatenate([st["yb", c, sig, p, rho][:, 128 * s_:128 * (s_ + 1)] for rho in range(8)], axis=0)
                     for sig in range(2)], axis=1)
            else:
                rhs = load_hooked(lambda rb, kk: ybfs[c % 2][pl.ds(yrow(c, kk, p) + 8 * rb, 8), pl.ds(128 * s_, 128)],
                                  8, 2, att, lambda rb, kk: ("r", kk, rb))
            st["z", c, k1] = jnp.dot(lhs, rhs, preferred_element_type=F32)

        def pw(k1):
            z = st.pop(("z", c, k1))
            dD = par[1, :, lt(c)]
            parts = []
            for g in range(8):
                ur = z[16 * g:16 * g + 8, 0:128]
                ui = z[16 * g + 8:16 * g + 16, 0:128]
                kr = z[16 * g:16 * g + 8, 128:256] + dD
                ki = z[16 * g + 8:16 * g + 16, 128:256]
                pr_, pi_ = _cmul(ur, ui, kr, ki)
                parts += [pr_, pi_]
            st["p", c, k1] = jnp.concatenate(parts, axis=0).astype(BF16)

        def inv_(k1, att):
            p = st.pop(("p", c, k1))
            nrb = 4 if k1 in (0, 32) else 8
            lhs = load_hooked(lambda rb, kk: gm[k1, pl.ds(8 * rb, 8), :], nrb, 1, att, lambda rb, kk: (0, rb))
            if CFG["ssa"] & 64:
                st["V", c, k1] = jnp.dot(lhs, p, preferred_element_type=F32)
            else:
                vscrs[c % 2][pl.ds(k1 * 128, 16 * nrb), :] = jnp.dot(lhs, p, preferred_element_type=F32)

        steps = []
        for i in range(NK1 + 2):
            def f(i=i):
                first = None
                if i < NK1:
                    first = sc.dot(64, f_slots(8) + [(-100 + 32 * kk + 8 * a, ("r", kk, a)) for kk in range(2) for a in range(8)
                                                     if CFG["rslot"]],
                                   lambda att, i=i: fwd(i, att))
                if 1 <= i <= NK1:
                    sc.fn(lambda i=i: pw(i - 1))
                if i >= 2:
                    sc.dot(32, f_slots(4 if i - 2 in (0, 32) else 8), lambda att, i=i: inv_(i - 2, att))
                return first
            steps.append(f)
        return steps

    W_FIN = 8 * _W_INV

    def conv_fin(c):
        vscr = vscrs[c % 2]
        for rho in range(8 if "fin" not in CFG["skip"] else 0):
            zz = {}

            def V(k1):
                r0 = k1 * 128 + 8 * rho
                if CFG["ssa"] & 64:
                    vv_ = st["V", c, k1]
                    return ((1, vv_[8 * rho:8 * rho + 8, :]),
                            None if k1 in (0, 32) else (1, vv_[64 + 8 * rho:72 + 8 * rho, :]))
                re = (1, vscr[at(zz["z"], r0, 8), :])
                im = None if k1 in (0, 32) else (1, vscr[at(zz["z"], r0 + 64, 8), :])
                return (re, im)

            def emit(outs):
                deps = []
                for b, (s_, v_) in outs:
                    tau = 64 * (b % 4) + 8 * rho
                    val = v_ if s_ > 0 else -v_
                    yscr[b // 4, c, pl.ds(PITCH * (tau // TS) + tau % TS, 8), :] = val
                    deps.append(val)
                return deps

            def rel():
                zz["z"] = release(90, 16)
            if CFG["lock"]:
                yield LOCK, 0
            yield from BfH().inv_g(V, emit, rel)
            if CFG["lock"]:
                yield UNLOCK, 0

    def gather16(ref_fn, q, z):
        return jnp.concatenate(
            [jnp.concatenate([ref_fn(ct)[at(z, 2 * q + e, 8, PITCH), :] for ct in range(NT)], axis=1)
             for e in range(2)], axis=0)

    def ln_to_mm(c, q, x, l):
        ln = _layernorm(x)
        lb = (lnb0, lnb1)[c % 2]
        dsk = par[0]
        xr = x + ln * jnp.concatenate([dsk, dsk], axis=0)
        if CFG["ssa"] & 4:
            st["xa", l, c, q] = xr
        else:
            xas[(l * NCH + c) % 3][pl.ds(16 * q, 16), :] = xr
        if CFG["ssa"] & 2:
            st.setdefault(("ln", l, c), []).append(ln.astype(BF16))
            return grp(tiles(ln), 2) + grp(tiles(xr), CFG["o_pre"])
        lb[pl.ds(8 * q, 8), :] = pltpu.bitcast(ln.astype(BF16), I32)
        return grp([lb[pl.ds(8 * q, 8), lt(ct)] for ct in range(NT)], 1) + grp(tiles(xr), CFG["o_pre"])

    def pre1(c):
        for i in range(4 if "prepost" not in CFG["skip"] else 0):
            z = release(CFG["lead1"] + 60, 32)
            for ct in range(NT):
                for s_ in range(8):
                    pad[ct, pl.ds(PITCH * s_ + 8 * i, 8), :] = \
                        xin[at(z, T * c + TS * s_ + 8 * i, 8), lt(ct)].astype(F32)
            for q in range(4 * i, 4 * i + 4):
                if q % 4:
                    z = release(CFG["lead1"], 32)
                yield ln_to_mm(c, q, gather16(lambda ct: pad.at[ct], q, z), 0), 1

    def post1(c):
        y = st["y", 0, c]
        for q in range(16 if "prepost" not in CFG["skip"] else 0):
            z = release(60, 32)
            xa = st.pop(("xa", 0, c, q)) if CFG["ssa"] & 4 else xas[c % 3][at(z, 16 * q, 16), :]
            v_ = xa + y[16 * q:16 * q + 16, :]
            if CFG["ssa"] & 8:
                st["x1", c, q] = v_
            else:
                x1[pl.ds(T * c + 16 * q, 16), :] = v_
            yield grp(tiles(v_), CFG["o_post"]), 1

    def pre2(c):
        for q in range(16):
            z = release(CFG["lead2"], 64)
            x = st.pop(("x1", c, q)) if (CFG["ssa"] & 8 and FULL) else x1[at(z, T * c + 16 * q, 16), :]
            yc = gather16(lambda ct: yscr.at[c, ct], q, z)
            x = x + _layernorm(x) * yc
            yield ln_to_mm(c, q, x, 1), 1

    def post2(c):
        y = st["y", 1, c]
        for i in range(4):
            for q in range(4 * i, 4 * i + 4):
                z = release(CFG["lead1"], 64)
                xa = st.pop(("xa", 1, c, q)) if CFG["ssa"] & 4 else xas[(NCH + c) % 3][at(z, 16 * q, 16), :]
                x = xa + y[16 * q:16 * q + 16, :]
                yc = gather16(lambda ct: yscr.at[c, ct], q, z)
                x = x + _layernorm(x) * yc
                for ct in range(NT):
                    for e in range(2):
                        pad[ct, pl.ds(2 * q + e, 8, stride=PITCH), :] = x[8 * e:8 * e + 8, lt(ct)]
                yield grp(tiles(x), CFG["o_post"]), 2
            deps = []
            z = release(80, 64)
            for ct in range(NT):
                for s_ in range(8):
                    v_ = pad[ct, at(z, PITCH * s_ + 8 * i, 8, aligned=False), :]
                    ostg[pl.ds(T * c + TS * s_ + 8 * i, 8), lt(ct)] = v_
                    deps.append(v_)
            yield grp(deps, CFG["o_exit"]), 1

    if CFG["bench"] == "p2":
        SEQ = [(1, c) for c in range(CFG["nch"])]
    elif CFG["bench"] in ("p1", "f"):
        SEQ = [(0, c) for c in range(CFG["nch"])]
    else:
        SEQ = [(l, c) for l in range(2) for c in range(NCH)]
    NIT = len(SEQ)
    G = NIT * NT
    FULL = CFG["bench"] == ""
    FFT_TILES = list(range(NT)) if FULL else ([0, 1] if CFG["bench"] == "f" else [])

    def dec(g):
        return SEQ[g // NT] + (g % NT,)

    TS1, DELTA = (float(_os.environ.get("TS1", "9000")) if FULL else 0.0), float(_os.environ.get("DELTA", "9000"))
    m_start = {c: TS1 + (c + 1) * DELTA for c in range(NT)}
    m_quota = {c: (int(_os.environ.get("MQ", "4")) if c < NT - 1 else int(_os.environ.get("MQL", "7"))) for c in range(NT)}
    m_steps = {c: (conv_mx_steps(c) if c in FFT_TILES else []) for c in range(NT)}
    mx_first, mx_end = {}, {}

    def b_a():
        tile_wait(0)
        cp_x(3).wait()
        tile_start(1)
        cp_f.start()
        cp_g.start()
        cp_x(4).start()

    def b_tile(c):
        def f():
            tile_wait(c)
            cp_x(c + 3).wait()
            if c == 1:
                cp_f.wait()
                cp_g.wait()
            if c + 1 < NT:
                tile_start(c + 1)
                cp_x(c + 4).start()
        return f
    timed = [(TS1, "t0", b_a)] + [(TS1 + c * DELTA, "t%d" % c, b_tile(c)) for c in range(1, NT)]
    if not FULL:
        timed = []
    bar = {}
    tr_s = {}

    def before_dot():
        while timed and sc.t >= timed[0][0]:
            _, name, f = timed.pop(0)
            bar[name] = sc.barrier(f)

    def after_dot():
        before_dot()
        for c in range(NT):
            if sc.t >= m_start[c] and m_steps[c]:
                for _ in range(m_quota[c]):
                    if m_steps[c]:
                        f0 = m_steps[c].pop(0)()
                        if c not in mx_first:
                            mx_first[c] = f0
                if not m_steps[c]:
                    mx_end[c] = sc.t
                break

    t_it, mm1_d, mm2_d = {}, {}, {}
    if FULL:
        def x0w():
            cp_x(0).wait()
            for w in range(4):
                cp_w(1, w).start()
            cp_x(1).start()
        bar["x0"] = sc.barrier(x0w)
    for it in range(NIT + 1):
        t_it[it] = sc.t
        if FULL and it == 13:
            bar["o0"] = sc.barrier(lambda: cp_o(0).start())
        if FULL and it == 15:
            bar["o1"] = sc.barrier(lambda: cp_o(1).start())
        if FULL and it == 16:
            bar["o2"] = sc.barrier(lambda: cp_o(2).start())
        for n in range(NT):
            g = NT * it + n
            if g < G:
                before_dot()
                if FULL and g < NT:
                    bar["w%d" % n] = sc.barrier(lambda n=n: wwait(n))
                    sc.fn(lambda n=n: wprep(n))
                mm1_d[g] = sc.dot(640, a_slots(5, it), lambda att, g=g: mm1(g, att))
                after_dot()
            if 2 <= g < G + 2:
                before_dot()
                mm2_d[g - 2] = sc.dot(640, a_slots(2, it), lambda att, g=g: mm2(g - 2, att))
                after_dot()
    t_it[NIT + 1] = sc.t

    prev = None
    for g in range(G):
        if CFG["pin_scan"] & (1 << SEQ[g // NT][0]):
            s_ = sc.stream(scan(g), W_SCAN, mm1_d[g].t0 + CFG["sc0"],
                           min(mm2_d[g].t0 - 100, mm1_d[g].t0 + CFG["sc0"] + CFG["scw"]), after=[prev] if prev else [])
        else:
            def nat(g=g):
                for _ in scan(g):
                    pass
                return
                yield
            s_ = sc.stream(nat(g), 1, mm1_d[g].t0 + 700, mm1_d[g].t0 + 700, after=[prev] if prev else [])
        mm2_d[g].requires.append(s_)
        prev = s_
    s1_s, fin_s = {}, {}
    for c in FFT_TILES:
        s1_s[c] = sc.stream(conv_s1(c), W_S1, TS1 + c * DELTA, TS1 + (c + 1) * DELTA - 200,
                            after=[s1_s[c - 1]] if c else [], needs=[bar["t%d" % c]] if FULL else [], orw=CFG["orw_s1"])
        tr_s[c] = sc.stream(conv_tr(c), 16, TS1 + c * DELTA, TS1 + (c + 0.5) * DELTA,
                            after=[s1_s[c - 1]] if c else [], needs=[bar["t%d" % c]] if FULL else [],
                            orw=CFG["orw_tr"])
        mx_first[c].requires.append(s1_s[c])
        span = int(_os.environ.get("FSPAN", "5500")) if c < NT - 1 else int(_os.environ.get("FSPANL", "3000"))
        fin_s[c] = sc.stream(conv_fin(c), W_FIN, mx_end[c] + 200, mx_end[c] + 200 + span,
                             after=[fin_s[c - 1]] if c else [], orw=CFG["orw_fin"])
    pre_s, post_s = {}, {}
    for it in range(NIT):
        l, c = SEQ[it]
        gen = pre1(c) if l == 0 else pre2(c)
        if it == 0:
            pre_s[it] = sc.stream(gen, 16, -2000, -1000, needs=[bar["x0"]] if FULL else [])
        else:
            t0 = t_it[it - 1] + 100
            aft = [pre_s[it - 1]]
            nd = []
            if not FULL:
                pass
            elif it == 1:
                t0 = t_it[0] + 0.5 * (t_it[1] - t_it[0])
                nd = [bar["w2"]]
            elif it == 2:
                nd = [bar["w4"]]
            elif it == 3:
                nd = [bar["t0"]]
            elif 4 <= it <= 7:
                nd = [bar["t%d" % (it - 3)]]
            if it >= 3:
                aft.append(post_s[it - 3])
            if FULL and it == NCH:
                t0 = max(t0, fin_s[NT - 1].t1)
                aft.append(fin_s[NT - 1])
            pre_s[it] = sc.stream(gen, 16, t0, t_it[it] - 450, after=aft, needs=nd)
        mm1_d[NT * it].requires.append(pre_s[it])
        gen = post1(c) if l == 0 else post2(c)
        t0 = mm2_d[NT * it + NT - 1].t0 + 640 + 150
        t1 = t_it[it + 2] - 100 if it + 2 <= NIT else t0 + 1000
        post_s[it] = sc.stream(gen, 16 if l == 0 else 36, t0, t1, after=[post_s[it - 1]] if it else [])
    if FULL:
        bar["o0"].requires.append(post_s[NCH + OSPLIT[0][1] - 1])
        bar["o1"].requires.append(post_s[NCH + OSPLIT[1][1] - 1])
        bar["o2"].requires.append(post_s[NCH + OSPLIT[2][1] - 1])
    sc.run()
    if _os.environ.get("VERBOSE"):
        print("dropped pins:", sc.dropped)
    if FULL:
        cp_o(3).start()
        for i in range(4):
            cp_o(i).wait()
        assert not started


_ZMASK = np.concatenate([np.zeros((8, 128), np.int32), np.arange(1024, dtype=np.int32).reshape(8, 128)], axis=1)
_ZS = np.array([0, 7, 3, 11], np.int32)


@jax.jit
def pallas_interleave_layers__ssm_conv_s5__ssm_conv_h3__prompt_kernel(
    A_x, A_Lambda_re, A_Lambda_im, A_B_re, A_B_im, A_C_re, A_C_im, A_log_dt, A_Dskip,
    B_q, B_k, B_v, B_shift_k, B_ssm_k, B_ssm_D,
):
    del B_q
    x2 = A_x.reshape(S, D)
    k2 = B_k.reshape(S, D)
    v2 = B_v.reshape(S, D)
    shkT = B_shift_k.T
    hbm = pl.BlockSpec(memory_space=pltpu.HBM)
    vm = pl.BlockSpec(memory_space=pltpu.VMEM)
    sm = pl.BlockSpec(memory_space=pltpu.SMEM)
    out = pl.pallas_call(
        _kernel,
        out_shape=jax.ShapeDtypeStruct((S, D), F32),
        in_specs=[vm] * 7 + [sm] + [hbm] * 10,
        out_specs=hbm,
        scratch_shapes=[
            pltpu.VMEM((S, D), BF16),
            pltpu.VMEM((4, D, D), BF16),
            pltpu.VMEM((D, D), I32),
            pltpu.VMEM((D // 2, 2 * D), I32),
            pltpu.VMEM((10, 8, D), F32),
            pltpu.VMEM((8, 8, D), F32),
            pltpu.VMEM((2, 2, 8, D), F32),
            pltpu.VMEM((NT, S, 128), BF16),
            pltpu.VMEM((NT, S, 128), BF16),
            pltpu.VMEM((NT, 128, S), BF16),
            pltpu.VMEM((NK1, 64, 128), I32),
            pltpu.VMEM((NK1, 64, 128), I32),
            pltpu.VMEM((S + 8, 128), F32),
            pltpu.VMEM((S + 8, 128), F32),
            pltpu.VMEM((S + 8, 128), F32),
            pltpu.VMEM((2 * 16 * 64, 256), I32),
            pltpu.VMEM((2 * 16 * 64, 256), I32),
            pltpu.VMEM((NK1 * 128 + 8, 128), F32),
            pltpu.VMEM((NK1 * 128 + 8, 128), F32),
            pltpu.VMEM((NCH, NT, PADR, 128), F32),
            pltpu.VMEM((S + 8, D), F32),
            pltpu.VMEM((T + 8, D), F32),
            pltpu.VMEM((T + 8, D), F32),
            pltpu.VMEM((T + 8, D), F32),
            pltpu.VMEM((T // 2, D), I32),
            pltpu.VMEM((T // 2, D), I32),
            pltpu.VMEM((T // 2, 256), I32),
            pltpu.VMEM((T // 2, 256), I32),
            pltpu.VMEM((T // 2, 256), I32),
            pltpu.VMEM((T // 2, 256), I32),
            pltpu.VMEM((NT, PADR, 128), F32),
            pltpu.VMEM((S, D), F32),
            pltpu.SemaphoreType.DMA((NCH,)),
            pltpu.SemaphoreType.DMA((4 * NT,)),
            pltpu.SemaphoreType.DMA((3 * NT,)),
            pltpu.SemaphoreType.DMA((2,)),
            pltpu.SemaphoreType.DMA((4,)),
        ],
        compiler_params=pltpu.CompilerParams(vmem_limit_bytes=100 * 1024 * 1024),
    )(A_Lambda_re, A_Lambda_im, A_log_dt, A_Dskip, shkT, B_ssm_D, _ZMASK, _ZS,
      x2, A_B_re, A_B_im, A_C_re, A_C_im, k2, v2, B_ssm_k, _FM, _GM)
    return out.reshape(1, S, D)
```

```python
import numpy as np
import jax
import jax.numpy as jnp
import jax.experimental.pallas as pl
import jax.experimental.pallas.tpu as pltpu

S, D = 2048, 640
NT = D // 128
TS = 32
T = 8 * TS
NCH = S // T
PITCH = TS + 1
PADR = 304
NFFT = 4096
NK1 = 33
C8 = float(np.sqrt(0.5))
F32 = jnp.float32
BF16 = jnp.bfloat16


class Bf:
    def __init__(self):
        self.tab = {}; self.keep = []
    def _plus(self, va, vb):
        key = ('+',) + tuple(sorted((id(va), id(vb))))
        if key not in self.tab:
            self.tab[key] = va + vb; self.keep.append((va, vb))
        return self.tab[key]
    def _minus(self, va, vb):
        k1 = ('-', id(va), id(vb)); k2 = ('-', id(vb), id(va))
        if k1 in self.tab: return (1, self.tab[k1])
        if k2 in self.tab: return (-1, self.tab[k2])
        self.tab[k1] = va - vb; self.keep.append((va, vb))
        return (1, self.tab[k1])
    def _times(self, va, c):
        key = ('*', id(va), c)
        if key not in self.tab:
            self.tab[key] = va * c; self.keep.append(va)
        return self.tab[key]
    def radd(self, a, b):
        if a is None: return b
        if b is None: return a
        sa, va = a; sb, vb = b
        if sa == sb: return (sa, self._plus(va, vb))
        s, v = self._minus(va, vb)
        return (s * sa, v)
    @staticmethod
    def rneg(a):
        return None if a is None else (-a[0], a[1])
    def rsub(self, a, b):
        return self.radd(a, self.rneg(b))
    def rmul(self, a, c):
        if a is None or c == 0.0: return None
        s = 1 if c > 0 else -1
        c = abs(c)
        if c == 1.0: return (a[0] * s, a[1])
        return (a[0] * s, self._times(a[1], c))
    def cadd(self, a, b): return (self.radd(a[0], b[0]), self.radd(a[1], b[1]))
    def csub(self, a, b): return (self.rsub(a[0], b[0]), self.rsub(a[1], b[1]))
    def cconj(self, a): return (a[0], self.rneg(a[1]))
    def cmuli(self, a, p):
        p %= 4
        if p == 0: return a
        if p == 1: return (self.rneg(a[1]), a[0])
        if p == 2: return (self.rneg(a[0]), self.rneg(a[1]))
        return (a[1], self.rneg(a[0]))
    def cmul_w(self, a, num, den):
        num %= den
        if (4 * num) % den == 0: return self.cmuli(a, 4 * num // den)
        if (8 * num) % den == 0:
            o = 8 * num // den
            re = self.rmul(self.rsub(a[0], a[1]), C8)
            im = self.rmul(self.radd(a[0], a[1]), C8)
            return self.cmuli((re, im), (o - 1) // 2)
        wr = float(np.cos(2 * np.pi * num / den)); wi = float(np.sin(2 * np.pi * num / den))
        re = self.rsub(self.rmul(a[0], wr), self.rmul(a[1], wi))
        im = self.radd(self.rmul(a[0], wi), self.rmul(a[1], wr))
        return (re, im)
    def fft(self, x, sgn):
        n = len(x)
        def get(v): return v() if callable(v) else v
        if n == 1: return [get(x[0])]
        if n == 2:
            a, b = get(x[0]), get(x[1])
            return [self.cadd(a, b), self.csub(a, b)]
        if n == 4:
            x0, x2 = get(x[0]), get(x[2])
            a = self.cadd(x0, x2); b = self.csub(x0, x2)
            x1, x3 = get(x[1]), get(x[3])
            c = self.cadd(x1, x3); d = self.csub(x1, x3)
            wd = self.cmuli(d, sgn)
            return [self.cadd(a, c), self.cadd(b, wd), self.csub(a, c), self.csub(b, wd)]
        m = n // 4
        u = [self.fft([x[b2 + m * b1] for b1 in range(4)], sgn) for b2 in range(m)]
        out = [None] * n
        for k1 in range(4):
            t = [self.cmul_w(u[b2][k1], sgn * b2 * k1, n) for b2 in range(m)]
            y = self.fft(t, sgn)
            for k2 in range(m):
                out[k1 + 4 * k2] = y[k2]
        return out

    def odd_fwd(self, d, N, emit, scale):
        q = N // 4
        def z(b):
            def th():
                p = d[b]() if callable(d[b]) else d[b]
                r = d[b + q]() if callable(d[b + q]) else d[b + q]
                return self.cmul_w((p, self.rneg(r)), -b, N)
            return th
        Y = self.fft([z(b) for b in range(q)], -1)
        for j in range(q):
            k = 4 * j + 1
            if 2 * k <= N: emit(k * scale, Y[j])
            else: emit((N - k) * scale, self.cconj(Y[j]))
    def real_fwd(self, x, N, emit, scale):
        if N == 2:
            emit(0, (self.radd(x[0], x[1]), None)); emit(scale, (self.rsub(x[0], x[1]), None)); return
        h = N // 2
        s = [self.radd(x[b], x[b + h]) for b in range(h)]
        d = [self.rsub(x[b], x[b + h]) for b in range(h)]
        if N == 4:
            emit(scale, (d[0], self.rneg(d[1])))
        else:
            self.odd_fwd(d, N, emit, scale)
        self.real_fwd(s, h, emit, 2 * scale)

    def odd_inv(self, V, N, scale):
        q = N // 4
        def U(j):
            k = 4 * j + 1
            if 2 * k <= N: return lambda: V(k * scale)
            return lambda: self.cconj(V((N - k) * scale))
        zt = self.fft([U(j) for j in range(q)], +1)
        out = [None] * (2 * q)
        for b in range(q):
            t = self.cmul_w(zt[b], b, N)
            out[b] = t[0]; out[b + q] = self.rneg(t[1])
        return out
    def real_inv(self, V, N, scale):
        if N == 2:
            a, b = V(0)[0], V(scale)[0]
            return [self.radd(a, b), self.rsub(a, b)]
        h = N // 2
        if N == 4:
            v1 = V(scale)
            qq = [v1[0], self.rneg(v1[1])]
        else:
            qq = self.odd_inv(V, N, scale)
        p = self.real_inv(V, h, 2 * scale)
        return [self.radd(p[b], qq[b]) for b in range(h)] + [self.rsub(p[b], qq[b]) for b in range(h)]


def _vals(*cs):
    out = []
    for c in cs:
        for p in c:
            if p is not None:
                out.append(p[1])
    return out


class BfH(Bf):
    def __init__(self):
        super().__init__()
        self.n0 = 0

    def dw(self):
        n = len(self.tab)
        w, self.n0 = n - self.n0, n
        return w

    def odd_fwd_g(self, d, N, emit, scale):
        q = N // 4

        def z(b):
            def th():
                p = d[b]() if callable(d[b]) else d[b]
                r = d[b + q]() if callable(d[b + q]) else d[b + q]
                return self.cmul_w((p, self.rneg(r)), -b, N)
            return th
        zs = [z(b) for b in range(q)]
        m = q // 4
        u = []
        for b2 in range(m):
            g = self.fft([zs[b2 + m * b1] for b1 in range(4)], -1)
            u.append(g)
            yield _vals(g[3])[:1], self.dw() + 8
        for k1 in range(4):
            t = [self.cmul_w(u[b2][k1], -b2 * k1, q) for b2 in range(m)]
            y = self.fft(t, -1)
            outs = []
            for k2 in range(m):
                k = 4 * (k1 + 4 * k2) + 1
                if 2 * k <= N:
                    outs.append((k * scale, y[k2]))
                else:
                    outs.append(((N - k) * scale, self.cconj(y[k2])))
            dd = emit(outs)
            yield dd, self.dw() + 12

    def fwd_q2(self, x, emit):
        def d(b):
            return lambda: self.rsub(x[b](), x[b + 16]())
        yield from self.odd_fwd_g([d(b) for b in range(16)], 32, emit, 2)

    def fwd_q0(self, x, emit):
        s = [None] * 16
        for b in range(8):
            s[b] = self.radd(x[b](), x[b + 16]())
            s[b + 8] = self.radd(x[b + 8](), x[b + 24]())
        outs = []
        self.real_fwd(s, 16, lambda k, c: outs.append((k, c)), 4)
        outs.sort(key=lambda kc: (kc[0] not in (0, 32), kc[0]))
        w = self.dw()
        yield emit(outs[:5]), w + 12
        yield emit(outs[5:]), 12

    def fwd_even_g(self, x, emit):
        s = [self.radd(x[b], x[b + 16]) for b in range(16)]
        d = [self.rsub(x[b], x[b + 16]) for b in range(16)]
        yield from self.odd_fwd_g(d, 32, emit, 2)
        outs = []
        self.real_fwd(s, 16, lambda k, c: outs.append((k, c)), 4)
        outs.sort(key=lambda kc: (kc[0] not in (0, 32), kc[0]))
        w = self.dw()
        yield emit(outs[:5]), w + 12
        yield emit(outs[5:]), 12

    def inv_g(self, V, emit):
        def odd_stage1(N, scale):
            q = N // 4
            m = q // 4

            def U(j):
                k = 4 * j + 1
                if 2 * k <= N:
                    return lambda: V(k * scale)
                return lambda: self.cconj(V((N - k) * scale))
            u = []
            deps = []
            for b2 in range(m):
                g = self.fft([U(b2 + m * b1) for b1 in range(4)], +1)
                u.append(g)
                deps.append((_vals(g[3])[:1], self.dw() + 8))
            return u, deps

        def odd_stage2(u, N, k1):
            q = N // 4
            m = q // 4
            t = [self.cmul_w(u[b2][k1], b2 * k1, q) for b2 in range(m)]
            y = self.fft(t, +1)
            res = {}
            for k2 in range(m):
                b = k1 + 4 * k2
                tt = self.cmul_w(y[k2], b, N)
                res[b] = tt[0]
                res[b + q] = self.rneg(tt[1])
            return res
        uo, deps = odd_stage1(64, 1)
        for dd in deps:
            yield dd
        o = {}
        for k1 in range(4):
            o.update(odd_stage2(uo, 64, k1))
            yield [o[b][1] for b in sorted(o) if b % 4 == k1 and (b // 4) % 2 == 0], self.dw() + 4
        uq, deps = odd_stage1(32, 2)
        for dd in deps:
            yield dd
        y1 = {}
        for k1 in range(4):
            qq = odd_stage2(uq, 32, k1)
            for b in sorted(qq):
                y1[b] = self.radd(o[b], qq[b])
                y1[b + 16] = self.rsub(o[b + 16], qq[b])
            yield [y1[b][1] for b in sorted(qq)], self.dw() + 4
        p = self.real_inv(V, 16, 4)
        yield [p[5][1]], self.dw() + 16
        for k1 in range(4):
            outs = []
            for b in range(k1, 32, 4):
                outs.append((b, self.radd(y1[b], p[b % 16])))
            dd = emit(outs)
            yield dd, self.dw() + 16


def _fwd_plan():
    Y = {}
    order = []

    def emit(outs):
        for k, c in outs:
            Y[k] = c
            if k != 32:
                order.append(k)
        return []
    xs = [(1, np.full((1,), float(i + 1) ** 1.37)) for i in range(32)]
    xl = [(lambda v=v: v) for v in xs]
    we = sum(w for _, w in BfH().fwd_q2(xl, emit)) + sum(w for _, w in BfH().fwd_q0(xl, emit))
    wo = sum(w for _, w in BfH().odd_fwd_g(xs, 64, emit, 1))
    full = {k: ((1, np.full((1,), 1.0 + k)), None if k in (0, 32) else (1, np.full((1,), 2.5 + k)))
            for k in range(NK1)}
    wi = sum(w for _, w in BfH().inv_g(lambda k: full[k], lambda o: []))
    sg = {k: tuple(0 if c is None else c[0] for c in Y[k]) for k in range(NK1)}
    slot = {k: (i // 2, i % 2) for i, k in enumerate(order)}
    slot[32] = slot[0]
    return sg, slot, we + wo, wi


_FSG, _FSLOT, _W_FWD, _W_INV = _fwd_plan()

def _pack_rows(m):
    b = m.astype(np.float32).astype(jnp.bfloat16).view(np.uint16).astype(np.uint32)
    w = b[..., 0::2, :] | (b[..., 1::2, :] << 16)
    return w.view(np.int32)


def _dft_matrices():
    r = np.arange(64)
    k2 = np.arange(64)
    Fm = np.zeros((NK1, 128, 128), np.float64)
    Gm = np.zeros((NK1, 128, 128), np.float64)
    col = (16 * (r // 8) + (r % 8))
    for k1 in range(NK1):
        th = 2 * np.pi * np.outer(k1 + 64 * k2, r) / NFFT
        c, s = np.cos(th), np.sin(th)
        sr, si = _FSG[k1]
        Fr, Fi = np.zeros((64, 128)), np.zeros((64, 128))
        if k1 == 0:
            Fr[:, col] = c * sr
            Fi[:, col] = -s * sr
        elif k1 == 32:
            Fr[:, col + 8] = c * sr
            Fi[:, col + 8] = -s * sr
        else:
            Fr[:, col] = c * sr
            Fr[:, col + 8] = s * si
            Fi[:, col] = -s * sr
            Fi[:, col + 8] = c * si
        Fm[k1][col] = Fr
        Fm[k1][col + 8] = Fi
        sc = (1.0 if k1 in (0, 32) else 2.0) / NFFT
        ct, st = c.T * sc, s.T * sc
        Gm[k1][0:64][:, col] = ct
        Gm[k1][0:64][:, col + 8] = -st
        Gm[k1][64:128][:, col] = st
        Gm[k1][64:128][:, col + 8] = ct
    return _pack_rows(Fm), _pack_rows(Gm)


_FM, _GM = _dft_matrices()


def _cmul(ar, ai, br, bi):
    return ar * br - ai * bi, ar * bi + ai * br


def _cmul_add(lr, li, hr, hi, ur, ui):
    return (lr * hr - li * hi) + ur, (lr * hi + li * hr) + ui


def _layernorm(x):
    m = jnp.mean(x, axis=-1, keepdims=True)
    xc = x - m
    v = jnp.mean(xc * xc, axis=-1, keepdims=True)
    return xc * jax.lax.rsqrt(v + 1e-5)


def _nt_dot(a, b):
    return jax.lax.dot_general(a, b, (((1,), (1,)), ((), ())), preferred_element_type=F32)


I32 = jnp.int32

LOCK, UNLOCK = object(), object()


class _Dot:
    def __init__(self, t0, slots, emit):
        self.t0 = t0
        self.slots = sorted(((t0 + rt, key) for rt, key in slots), key=lambda tk: tk[0])
        self.emit = emit
        self.att = {}
        self.requires = []


class _Barrier:
    def __init__(self, f):
        self.f = f
        self.emitted = False
        self.requires = []


class _Stream:
    def __init__(self, gen, wtot, t0, t1, after=(), needs=(), orw=None):
        self.gen, self.wtot, self.t0, self.t1 = gen, float(wtot), t0, t1
        self.after, self.needs = list(after), list(needs)
        self.orw = orw or 1
        self.cum = 0.0
        self.done = False

    def now(self):
        return self.t0 + (self.t1 - self.t0) * min(1.0, self.cum / self.wtot)


class _Sched:
    def __init__(self):
        self.items, self.streams = [], []
        self.t, self.pos = 0.0, 0
        self.lock = None

    def fn(self, f):
        self.items.append(f)

    def barrier(self, f):
        b = _Barrier(f)
        self.items.append(b)
        return b

    def dot(self, dur, slots, emit):
        d = _Dot(self.t, slots, emit)
        self.items.append(d)
        self.t += dur
        return d

    def stream(self, gen, wtot, t0, t1, after=(), needs=(), orw=None):
        s = _Stream(gen, wtot, t0, t1, after, needs, orw)
        self.streams.append(s)
        return s

    def _attach1(self, t, d):
        stop = self.pos
        while stop < len(self.items) and not isinstance(self.items[stop], _Barrier):
            stop += 1
        for it in self.items[self.pos:stop]:
            if isinstance(it, _Dot):
                for ts, key in it.slots:
                    if ts >= t and key not in it.att:
                        it.att[key] = d
                        return ts
        for it in reversed(self.items[self.pos:stop]):
            if isinstance(it, _Dot):
                for ts, key in reversed(it.slots):
                    if key not in it.att:
                        it.att[key] = d
                        return ts
        return t

    def _attach(self, t0, t1, deps, n):
        if not deps:
            return
        if isinstance(deps[0], list):
            chunks = deps
        else:
            chunks = [deps[i:i + n] for i in range(0, len(deps), n)]
        for i, ch in enumerate(chunks):
            d = None
            for v in ch:
                vi = v if v.dtype == I32 else pltpu.bitcast(v, I32)
                d = vi if d is None else d | vi
            self._attach1(t0 + (t1 - t0) * (i + 1.0) / len(chunks), d)

    def _step(self, s):
        for b in s.needs:
            while not b.emitted:
                self._emit_next()
        for a in s.after:
            self._drain(a)
        try:
            deps, w = next(s.gen)
        except StopIteration:
            s.done = True
            if self.lock is s:
                self.lock = None
            return
        if deps is LOCK:
            self.lock = s
            return
        if deps is UNLOCK:
            self.lock = None
            return
        ta = s.now()
        s.cum += w
        self._attach(ta, s.now(), deps, s.orw)

    def _drain(self, s):
        while not s.done:
            self._step(s)

    def _emit_next(self):
        it = self.items[self.pos]
        if isinstance(it, _Dot):
            for s in it.requires:
                self._drain(s)
            self.pos += 1
            it.emit(it.att)
        elif isinstance(it, _Barrier):
            for s in it.requires:
                self._drain(s)
            self.pos += 1
            it.f()
            it.emitted = True
        else:
            self.pos += 1
            it()

    def _advance(self, t):
        while self.pos < len(self.items):
            it = self.items[self.pos]
            if isinstance(it, _Dot) and any(ts >= t and key not in it.att for ts, key in it.slots):
                return
            self._emit_next()

    def run(self):
        while True:
            live = [s for s in self.streams if not s.done]
            if not live:
                break
            s = self.lock if self.lock is not None else min(live, key=lambda z: z.now())
            self._advance(s.now())
            if not s.done:
                self._step(s)
        while self.pos < len(self.items):
            self._emit_next()


def _kernel(lre_hbm, lim_hbm, ldt_hbm, dsk_hbm, shk_hbm, sD_hbm, zm_hbm,
            x_hbm, bre_hbm, bim_hbm, cre_hbm, cim_hbm, k_hbm, v_hbm, sk_hbm, f_hbm, g_hbm,
            o_hbm,
            lre_ref, lim_ref, ldt_ref, dsk_ref, shk_ref, sD_ref, zm_ref,
            xin, wst, bw, cw, tab, par, carry, kin, vin, skin, fm, gm,
            kf, kvf, skt, ybf0, ybf1, vscr0, vscr1, yscr, x1, xa0, xa1, xa2, lnb0, lnb1, hb0, hb1, hb2, hb3, pad, ostg,
            sem_x, sem_w, sem_kv, sem_fg, sem_o, sem_p):

    started = set()
    small = [pltpu.make_async_copy(a, b, sem_p.at[i]) for i, (a, b) in enumerate(
        ((lre_hbm, lre_ref), (lim_hbm, lim_ref), (ldt_hbm, ldt_ref), (dsk_hbm, dsk_ref),
         (shk_hbm, shk_ref), (sD_hbm, sD_ref), (zm_hbm, zm_ref)))]
    for d_ in small:
        d_.start()

    class _Cp:
        def __init__(self, key, desc):
            self.key, self.desc = key, desc

        def start(self):
            assert self.key not in started, self.key
            started.add(self.key)
            self.desc.start()

        def wait(self):
            assert self.key in started, self.key
            started.remove(self.key)
            self.desc.wait()

    def cp_x(c):
        rs = pl.ds(T * c, T)
        return _Cp(("x", c), pltpu.make_async_copy(x_hbm.at[rs, :], xin.at[rs, :], sem_x.at[c]))

    def cp_w(n, which):
        src = (bre_hbm, bim_hbm, cre_hbm, cim_hbm)[which]
        if which < 2:
            return _Cp(("w", n, which), pltpu.make_async_copy(
                src.at[pl.ds(128 * n, 128), :], wst.at[which, pl.ds(128 * n, 128), :], sem_w.at[4 * n + which]))
        return _Cp(("w", n, which), pltpu.make_async_copy(
            src.at[:, pl.ds(128 * n, 128)], wst.at[which, :, pl.ds(128 * n, 128)], sem_w.at[4 * n + which]))

    def cp_kv(c, which):
        src, dst = ((k_hbm.at[:, pl.ds(128 * c, 128)], kin), (v_hbm.at[:, pl.ds(128 * c, 128)], vin),
                    (sk_hbm.at[pl.ds(128 * c, 128), :], skin))[which]
        return _Cp(("kv", c, which), pltpu.make_async_copy(src, dst.at[c], sem_kv.at[3 * c + which]))

    cp_f = _Cp(("f",), pltpu.make_async_copy(f_hbm, fm, sem_fg.at[0]))
    cp_g = _Cp(("g",), pltpu.make_async_copy(g_hbm, gm, sem_fg.at[1]))
    OSPLIT = ((0, 4), (4, 6), (6, 7), (7, 8))

    def cp_o(i):
        lo, hi = OSPLIT[i]
        rs = pl.ds(T * lo, T * (hi - lo))
        return _Cp(("o", i), pltpu.make_async_copy(ostg.at[rs, :], o_hbm.at[rs, :], sem_o.at[i]))

    def tile_start(c):
        for w in range(3):
            cp_kv(c, w).start()

    def tile_wait(c):
        for w in range(3):
            cp_kv(c, w).wait()

    cp_x(0).start()
    for w in range(4):
        cp_w(0, w).start()

    for d_ in small:
        d_.wait()

    def row(ref):
        return ref[...].astype(F32)[None, :]

    lre, lim, ldt = row(lre_ref), row(lim_ref), row(ldt_ref)
    dt = jnp.exp(ldt).astype(BF16).astype(F32)
    zr, zi = dt * lre, dt * lim
    mag = jnp.exp(zr)
    lbr, lbi = mag * jnp.cos(zi), mag * jnp.sin(zi)
    inv = 1.0 / (lre * lre + lim * lim)
    nr, ni = lbr - 1.0, lbi
    fr, fi = (nr * lre + ni * lim) * inv, (ni * lre - nr * lim) * inv
    sub = jax.lax.broadcasted_iota(jnp.int32, (8, D), 0)

    def b8(v):
        return jnp.broadcast_to(v, (8, D))

    tab[0] = b8(lbr)
    tab[1] = b8(lbi)
    pr, pi = lbr, lbi
    for _ in range(5):
        pr, pi = _cmul(pr, pi, pr, pi)
    tab[2] = b8(pr)
    tab[3] = b8(pi)
    for q, sh in enumerate((1, 2, 4)):
        tab[4 + 2 * q] = jnp.where(sub >= sh, b8(pr), 0.0)
        tab[5 + 2 * q] = jnp.where(sub >= sh, b8(pi), 0.0)
        pr, pi = _cmul(pr, pi, pr, pi)
    par[0] = b8(row(dsk_ref))
    par[1] = b8(row(sD_ref))
    shk = shk_ref[...].astype(F32)
    for lag in range(4):
        par[2 + lag] = b8(shk[lag:lag + 1, :])
    par[6] = b8(2.0 * fr)
    par[7] = b8(2.0 * fi)
    carry[...] = jnp.zeros(carry.shape, F32)
    kf[0:8, :] = jnp.zeros((8, 128), F32)

    fmask = zm_ref[:, 0:128] != 0

    def lt(n):
        return slice(128 * n, 128 * (n + 1))

    def tiles(v):
        r, l = v.shape
        return [v[8 * i:8 * i + 8, 128 * j:128 * (j + 1)] for i in range(r // 8) for j in range(l // 128)]

    def grp(deps, n):
        return [deps[i:i + n] for i in range(0, len(deps), n)]

    def at(r0, n, stride=None):
        return pl.ds(r0, n) if stride is None else pl.ds(r0, n, stride=stride)

    def load_hooked(get, nrb, nk, att, keyf):
        rows_ = []
        for rb in range(nrb):
            cols = []
            for kk in range(nk):
                w = get(rb, kk)
                key = keyf(rb, kk)
                if key in att:
                    w = jnp.where(fmask, att[key], w)
                cols.append(w)
            rows_.append(cols[0] if nk == 1 else jnp.concatenate(cols, axis=1))
        return pltpu.bitcast(jnp.concatenate(rows_, axis=0), BF16)

    def a_slots():
        return [(64 * tau - 256 + 32 * p, (tau, 7 - p)) for tau in range(10) for p in range(8)
                if 64 * tau - 256 + 32 * p < 384]

    sc = _Sched()
    st = {}

    def mm1(g, att):
        l, c, n = dec(g)
        lhs = pltpu.bitcast((lnb0, lnb1)[c % 2][...], BF16)
        rhs = load_hooked(lambda rb, kk: bw[pl.ds(128 * n + 8 * rb, 8), pl.ds(128 * kk, 128)], 16, 5, att,
                          lambda rb, kk: (5 * (rb // 8) + kk, rb % 8))
        st["u", g] = _nt_dot(lhs, rhs)

    hbufs = (hb0, hb1, hb2, hb3)
    ybfs = (ybf0, ybf1)
    vscrs = (vscr0, vscr1)
    xas = (xa0, xa1, xa2)

    W_SCAN = 8 * 36 + 70 + 16 * 24

    def scan(g):
        layer, c, n = dec(g)
        u = st.pop(("u", g))
        sl = lt(n)
        lr, li = tab[0, :, sl], tab[1, :, sl]
        ur = [u[8 * j:8 * j + 8, 0:128] for j in range(TS)]
        ui = [u[8 * j:8 * j + 8, 128:256] for j in range(TS)]
        er, ei = ur[0], ui[0]
        for j in range(1, TS):
            er, ei = _cmul_add(lr, li, er, ei, ur[j], ui[j])
            if j % 4 == 3:
                yield [er], 36
        sub1 = jax.lax.broadcasted_iota(jnp.int32, (8, 128), 0)
        gr = jnp.where(sub1 == 0, carry[layer, 0, :, sl], pltpu.roll(er, 1, 0))
        gi = jnp.where(sub1 == 0, carry[layer, 1, :, sl], pltpu.roll(ei, 1, 0))
        for q, sh in enumerate((1, 2, 4)):
            gr, gi = _cmul_add(tab[4 + 2 * q, :, sl], tab[5 + 2 * q, :, sl],
                               pltpu.roll(gr, sh, 0), pltpu.roll(gi, sh, 0), gr, gi)
        nr_, ni_ = _cmul_add(tab[2, :, sl], tab[3, :, sl], gr, gi, er, ei)
        cr_ = jnp.broadcast_to(nr_[7:8, :], (8, 128))
        ci_ = jnp.broadcast_to(ni_[7:8, :], (8, 128))
        carry[layer, 0, :, sl] = cr_
        carry[layer, 1, :, sl] = ci_
        yield [gr, gi, cr_, ci_], 70
        hr, hi = gr, gi
        for a in range(TS // 2):
            two = []
            for j in (2 * a, 2 * a + 1):
                hr, hi = _cmul_add(lr, li, hr, hi, ur[j], ui[j])
                two.append(jnp.concatenate([hr, hi], axis=1))
            hbuf = hbufs[g % 4]
            hbuf[pl.ds(8 * a, 8), :] = pltpu.bitcast(jnp.concatenate(two, axis=0).astype(BF16), I32)
            yield [hbuf[pl.ds(8 * a, 8), pl.ds(128 * h_, 128)] for h_ in range(2)], 24

    def mm2(g, att):
        layer, c, n = dec(g)
        h = pltpu.bitcast(hbufs[g % 4][...], BF16)
        rhs = load_hooked(lambda rb, kk: cw[pl.ds(8 * rb, 8), pl.ds(256 * n + 128 * kk, 128)], 40, 2, att,
                          lambda rb, kk: (2 * (rb // 8) + kk, rb % 8))
        yn = _nt_dot(h, rhs)
        st["y", layer, c] = yn if n == 0 else st["y", layer, c] + yn

    def wwait(n):
        for w in range(4):
            cp_w(n, w).wait()
        if n + 2 < NT:
            for w in range(4):
                cp_w(n + 2, w).start()
        if n == 1:
            cp_x(2).start()
        if n == 2:
            cp_x(1).wait()
        if n == 3:
            tile_start(0)
        if n == NT - 1:
            cp_x(2).wait()
            cp_x(3).start()

    def wprep(n):
        for w in range(2):
            bw[pl.ds(128 * n + 64 * w, 64), :] = pltpu.bitcast(wst[w, pl.ds(128 * n, 128), :], I32)
        cr = wst[2, :, lt(n)].astype(F32)
        ci = wst[3, :, lt(n)].astype(F32)
        f_r, f_i = par[6, 0:1, lt(n)], par[7, 0:1, lt(n)]
        cc_ = jnp.concatenate([cr * f_r - ci * f_i, -(cr * f_i + ci * f_r)], axis=1).astype(BF16)
        cw[:, 256 * n:256 * (n + 1)] = pltpu.bitcast(cc_, I32)

    def yrow(c, sig, p):
        return (sig * 16 + p) * 64

    W_S1 = 32 * 80 + 16 * _W_FWD

    def conv_tr(c):
        for m in range(16):
            val = skin[c, :, pl.ds(128 * m, 128)].astype(F32).T
            skt[pl.ds(128 * m, 128), :] = val
            yield tiles(val), 1

    def conv_s1(c):
        w = [par[2 + lag, :, lt(c)] for lag in range(4)]
        for m in range(32):
            kf[pl.ds(8 + 64 * m, 64), :] = kin[c, pl.ds(64 * m, 64), :].astype(F32)
            vv = vin[c, pl.ds(64 * m, 64), :].astype(F32)
            deps = []
            for i in range(8):
                t0 = 8 + 64 * m + 8 * i
                acc = kf[at(t0 - 3, 8), :] * w[3]
                acc = acc + kf[at(t0 - 2, 8), :] * w[2]
                acc = acc + kf[at(t0 - 1, 8), :] * w[1]
                acc = acc + kf[at(t0, 8), :] * w[0]
                kv = acc * vv[8 * i:8 * i + 8, :]
                kvf[pl.ds(t0 - 8, 8), :] = kv
                deps.append(kv)
            yield grp(deps, 2), 90
        for sig in (0, 1):
            if sig == 1:
                sc._drain(tr_s[c])
            src = kvf if sig == 0 else skt
            for rho in range(8):
                pend = {}

                def emit(outs):
                    vals = []
                    for k1, v in outs:
                        if k1 in (0, 32):
                            pend[k1] = v[0]
                            if len(pend) == 2:
                                vals.append((0, pend[0][1], pend[32][1]))
                        else:
                            vals.append((k1, v[0][1], v[1][1]))
                    deps = []
                    for i in range(0, len(vals), 2):
                        r0 = yrow(c, sig, _FSLOT[vals[i][0]][0]) + 8 * rho
                        two = jnp.concatenate(
                            [jnp.concatenate([vals[i + e][1], vals[i + e][2]], axis=0) for e in range(2)], axis=1)
                        ybf = ybfs[c % 2]
                        ybf[pl.ds(r0, 8), :] = pltpu.bitcast(two.astype(BF16), I32)
                        deps += [ybf[pl.ds(r0, 8), pl.ds(128 * h_, 128)] for h_ in range(2)]
                    return deps

                def xs():
                    return [(lambda b=b: (1, src[at(64 * b + 8 * rho, 8), :])) for b in range(32)]
                for part in range(3):
                    yield LOCK, 0
                    if part == 0:
                        yield from BfH().fwd_q2(xs(), emit)
                    elif part == 1:
                        yield from BfH().fwd_q0(xs(), emit)
                    else:
                        yield from BfH().odd_fwd_g(xs(), 64, emit, 1)
                    yield UNLOCK, 0

    def f_slots(n):
        return [(8 * a, (0, a)) for a in range(n)]

    def conv_mx_steps(c):
        def fwd(k1, att):
            lhs = load_hooked(lambda rb, kk: fm[k1, pl.ds(8 * rb, 8), :], 8, 1, att, lambda rb, kk: (0, rb))
            p, s_ = _FSLOT[k1]
            rhs = pltpu.bitcast(jnp.concatenate(
                [ybfs[c % 2][pl.ds(yrow(c, sig, p), 64), pl.ds(128 * s_, 128)] for sig in range(2)], axis=1), BF16)
            st["z", c, k1] = jnp.dot(lhs, rhs, preferred_element_type=F32)

        def pw(k1):
            z = st.pop(("z", c, k1))
            dD = par[1, :, lt(c)]
            parts = []
            for g in range(8):
                ur = z[16 * g:16 * g + 8, 0:128]
                ui = z[16 * g + 8:16 * g + 16, 0:128]
                kr = z[16 * g:16 * g + 8, 128:256] + dD
                ki = z[16 * g + 8:16 * g + 16, 128:256]
                pr_, pi_ = _cmul(ur, ui, kr, ki)
                parts += [pr_, pi_]
            st["p", c, k1] = jnp.concatenate(parts, axis=0).astype(BF16)

        def inv_(k1, att):
            p = st.pop(("p", c, k1))
            nrb = 4 if k1 in (0, 32) else 8
            lhs = load_hooked(lambda rb, kk: gm[k1, pl.ds(8 * rb, 8), :], nrb, 1, att, lambda rb, kk: (0, rb))
            vscrs[c % 2][pl.ds(k1 * 128, 16 * nrb), :] = jnp.dot(lhs, p, preferred_element_type=F32)

        steps = []
        for i in range(NK1 + 2):
            def f(i=i):
                first = None
                if i < NK1:
                    first = sc.dot(64, f_slots(8), lambda att, i=i: fwd(i, att))
                if 1 <= i <= NK1:
                    sc.fn(lambda i=i: pw(i - 1))
                if i >= 2:
                    sc.dot(32, f_slots(4 if i - 2 in (0, 32) else 8), lambda att, i=i: inv_(i - 2, att))
                return first
            steps.append(f)
        return steps

    W_FIN = 8 * _W_INV

    def conv_fin(c):
        vscr = vscrs[c % 2]
        for rho in range(8):
            def V(k1):
                r0 = k1 * 128 + 8 * rho
                re = (1, vscr[at(r0, 8), :])
                im = None if k1 in (0, 32) else (1, vscr[at(r0 + 64, 8), :])
                return (re, im)

            def emit(outs):
                deps = []
                for b, (s_, v_) in outs:
                    tau = 64 * (b % 4) + 8 * rho
                    val = v_ if s_ > 0 else -v_
                    yscr[b // 4, c, pl.ds(PITCH * (tau // TS) + tau % TS, 8), :] = val
                    deps.append(val)
                return deps

            yield LOCK, 0
            yield from BfH().inv_g(V, emit)
            yield UNLOCK, 0

    def gather16(ref_fn, q):
        return jnp.concatenate(
            [jnp.concatenate([ref_fn(ct)[at(2 * q + e, 8, PITCH), :] for ct in range(NT)], axis=1)
             for e in range(2)], axis=0)

    def ln_to_mm(c, q, x, l):
        ln = _layernorm(x)
        lb = (lnb0, lnb1)[c % 2]
        dsk = par[0]
        xr = x + ln * jnp.concatenate([dsk, dsk], axis=0)
        xas[(l * NCH + c) % 3][pl.ds(16 * q, 16), :] = xr
        lb[pl.ds(8 * q, 8), :] = pltpu.bitcast(ln.astype(BF16), I32)
        return grp([lb[pl.ds(8 * q, 8), lt(ct)] for ct in range(NT)], 1) + grp(tiles(xr), 2)

    def pre1(c):
        for i in range(4):
            for ct in range(NT):
                for s_ in range(8):
                    pad[ct, pl.ds(PITCH * s_ + 8 * i, 8), :] = \
                        xin[at(T * c + TS * s_ + 8 * i, 8), lt(ct)].astype(F32)
            for q in range(4 * i, 4 * i + 4):
                yield ln_to_mm(c, q, gather16(lambda ct: pad.at[ct], q), 0), 1

    def post1(c):
        y = st["y", 0, c]
        for q in range(16):
            v_ = xas[c % 3][at(16 * q, 16), :] + y[16 * q:16 * q + 16, :]
            x1[pl.ds(T * c + 16 * q, 16), :] = v_
            yield grp(tiles(v_), 2), 1

    def pre2(c):
        for q in range(16):
            x = x1[at(T * c + 16 * q, 16), :]
            yc = gather16(lambda ct: yscr.at[c, ct], q)
            x = x + _layernorm(x) * yc
            yield ln_to_mm(c, q, x, 1), 1

    def post2(c):
        y = st["y", 1, c]
        for i in range(4):
            for q in range(4 * i, 4 * i + 4):
                x = xas[(NCH + c) % 3][at(16 * q, 16), :] + y[16 * q:16 * q + 16, :]
                yc = gather16(lambda ct: yscr.at[c, ct], q)
                x = x + _layernorm(x) * yc
                for ct in range(NT):
                    for e in range(2):
                        pad[ct, pl.ds(2 * q + e, 8, stride=PITCH), :] = x[8 * e:8 * e + 8, lt(ct)]
                yield grp(tiles(x), 2), 2
            deps = []
            for ct in range(NT):
                for s_ in range(8):
                    v_ = pad[ct, at(PITCH * s_ + 8 * i, 8), :]
                    ostg[pl.ds(T * c + TS * s_ + 8 * i, 8), lt(ct)] = v_
                    deps.append(v_)
            yield grp(deps, 4), 1

    SEQ = [(l, c) for l in range(2) for c in range(NCH)]
    NIT = len(SEQ)
    G = NIT * NT

    def dec(g):
        return SEQ[g // NT] + (g % NT,)

    TS1, DELTA = 8000.0, 9500.0
    m_start = {c: TS1 + (c + 1) * DELTA for c in range(NT)}
    m_quota = {c: (6 if c < NT - 1 else 7) for c in range(NT)}
    m_steps = {c: conv_mx_steps(c) for c in range(NT)}
    mx_first, mx_end = {}, {}

    def b_a():
        tile_wait(0)
        cp_x(3).wait()
        tile_start(1)
        cp_f.start()
        cp_g.start()
        cp_x(4).start()

    def b_tile(c):
        def f():
            tile_wait(c)
            cp_x(c + 3).wait()
            if c == 1:
                cp_f.wait()
                cp_g.wait()
            if c + 1 < NT:
                tile_start(c + 1)
                cp_x(c + 4).start()
        return f
    timed = [(TS1, "t0", b_a)] + [(TS1 + c * DELTA, "t%d" % c, b_tile(c)) for c in range(1, NT)]
    bar = {}
    tr_s = {}

    def before_dot():
        while timed and sc.t >= timed[0][0]:
            _, name, f = timed.pop(0)
            bar[name] = sc.barrier(f)

    def after_dot():
        before_dot()
        for c in range(NT):
            if sc.t >= m_start[c] and m_steps[c]:
                for _ in range(m_quota[c]):
                    if m_steps[c]:
                        f0 = m_steps[c].pop(0)()
                        if c not in mx_first:
                            mx_first[c] = f0
                if not m_steps[c]:
                    mx_end[c] = sc.t
                break

    t_it, mm1_d, mm2_d = {}, {}, {}
    def x0w():
        cp_x(0).wait()
        for w in range(4):
            cp_w(1, w).start()
        cp_x(1).start()
    bar["x0"] = sc.barrier(x0w)
    for it in range(NIT + 1):
        t_it[it] = sc.t
        if it == 13:
            bar["o0"] = sc.barrier(lambda: cp_o(0).start())
        if it == 15:
            bar["o1"] = sc.barrier(lambda: cp_o(1).start())
        if it == 16:
            bar["o2"] = sc.barrier(lambda: cp_o(2).start())
        for n in range(NT):
            g = NT * it + n
            if g < G:
                before_dot()
                if g < NT:
                    bar["w%d" % n] = sc.barrier(lambda n=n: wwait(n))
                    sc.fn(lambda n=n: wprep(n))
                mm1_d[g] = sc.dot(640, a_slots(), lambda att, g=g: mm1(g, att))
                after_dot()
            if 2 <= g < G + 2:
                before_dot()
                mm2_d[g - 2] = sc.dot(640, a_slots(), lambda att, g=g: mm2(g - 2, att))
                after_dot()
    t_it[NIT + 1] = sc.t

    prev = None
    for g in range(G):
        def nat(g=g):
            for _ in scan(g):
                pass
            return
            yield
        s_ = sc.stream(nat(g), 1, mm1_d[g].t0 + 700, mm1_d[g].t0 + 700, after=[prev] if prev else [])
        mm2_d[g].requires.append(s_)
        prev = s_
    s1_s, fin_s = {}, {}
    for c in range(NT):
        s1_s[c] = sc.stream(conv_s1(c), W_S1, TS1 + c * DELTA, TS1 + (c + 1) * DELTA - 200,
                            after=[s1_s[c - 1]] if c else [], needs=[bar["t%d" % c]], orw=2)
        tr_s[c] = sc.stream(conv_tr(c), 16, TS1 + c * DELTA, TS1 + (c + 0.5) * DELTA,
                            after=[s1_s[c - 1]] if c else [], needs=[bar["t%d" % c]],
                            orw=4)
        mx_first[c].requires.append(s1_s[c])
        span = 5500 if c < NT - 1 else 3000
        fin_s[c] = sc.stream(conv_fin(c), W_FIN, mx_end[c] + 200, mx_end[c] + 200 + span,
                             after=[fin_s[c - 1]] if c else [], orw=2)
    pre_s, post_s = {}, {}
    for it in range(NIT):
        l, c = SEQ[it]
        gen = pre1(c) if l == 0 else pre2(c)
        if it == 0:
            pre_s[it] = sc.stream(gen, 16, -2000, -1000, needs=[bar["x0"]])
        else:
            t0 = t_it[it - 1] + 100
            aft = [pre_s[it - 1]]
            nd = []
            if it == 1:
                t0 = t_it[0] + 0.5 * (t_it[1] - t_it[0])
                nd = [bar["w2"]]
            elif it == 2:
                nd = [bar["w4"]]
            elif it == 3:
                nd = [bar["t0"]]
            elif 4 <= it <= 7:
                nd = [bar["t%d" % (it - 3)]]
            if it >= 3:
                aft.append(post_s[it - 3])
            if it == NCH:
                t0 = max(t0, fin_s[NT - 1].t1)
                aft.append(fin_s[NT - 1])
            pre_s[it] = sc.stream(gen, 16, t0, t_it[it] - 450, after=aft, needs=nd)
        mm1_d[NT * it].requires.append(pre_s[it])
        gen = post1(c) if l == 0 else post2(c)
        t0 = mm2_d[NT * it + NT - 1].t0 + 640 + 150
        t1 = t_it[it + 2] - 100 if it + 2 <= NIT else t0 + 1000
        post_s[it] = sc.stream(gen, 16 if l == 0 else 36, t0, t1, after=[post_s[it - 1]] if it else [])
    for i in range(3):
        bar["o%d" % i].requires.append(post_s[NCH + OSPLIT[i][1] - 1])
    sc.run()
    cp_o(3).start()
    for i in range(4):
        cp_o(i).wait()
    assert not started


_ZMASK = np.concatenate([np.zeros((8, 128), np.int32), np.arange(1024, dtype=np.int32).reshape(8, 128)], axis=1)


@jax.jit
def pallas_interleave_layers__ssm_conv_s5__ssm_conv_h3__prompt_kernel(
    A_x, A_Lambda_re, A_Lambda_im, A_B_re, A_B_im, A_C_re, A_C_im, A_log_dt, A_Dskip,
    B_q, B_k, B_v, B_shift_k, B_ssm_k, B_ssm_D,
):
    del B_q
    x2 = A_x.reshape(S, D)
    k2 = B_k.reshape(S, D)
    v2 = B_v.reshape(S, D)
    shkT = B_shift_k.T
    hbm = pl.BlockSpec(memory_space=pltpu.HBM)
    out = pl.pallas_call(
        _kernel,
        out_shape=jax.ShapeDtypeStruct((S, D), F32),
        in_specs=[hbm] * 17,
        out_specs=hbm,
        scratch_shapes=[
            pltpu.VMEM((D,), BF16), pltpu.VMEM((D,), BF16), pltpu.VMEM((D,), BF16), pltpu.VMEM((D,), BF16),
            pltpu.VMEM((4, D), BF16), pltpu.VMEM((D,), BF16), pltpu.VMEM((8, 256), I32),
            pltpu.VMEM((S, D), BF16),
            pltpu.VMEM((4, D, D), BF16),
            pltpu.VMEM((D, D), I32),
            pltpu.VMEM((D // 2, 2 * D), I32),
            pltpu.VMEM((10, 8, D), F32),
            pltpu.VMEM((8, 8, D), F32),
            pltpu.VMEM((2, 2, 8, D), F32),
            pltpu.VMEM((NT, S, 128), BF16),
            pltpu.VMEM((NT, S, 128), BF16),
            pltpu.VMEM((NT, 128, S), BF16),
            pltpu.VMEM((NK1, 64, 128), I32),
            pltpu.VMEM((NK1, 64, 128), I32),
            pltpu.VMEM((S + 8, 128), F32),
            pltpu.VMEM((S + 8, 128), F32),
            pltpu.VMEM((S + 8, 128), F32),
            pltpu.VMEM((2 * 16 * 64, 256), I32),
            pltpu.VMEM((2 * 16 * 64, 256), I32),
            pltpu.VMEM((NK1 * 128 + 8, 128), F32),
            pltpu.VMEM((NK1 * 128 + 8, 128), F32),
            pltpu.VMEM((NCH, NT, PADR, 128), F32),
            pltpu.VMEM((S + 8, D), F32),
            pltpu.VMEM((T + 8, D), F32),
            pltpu.VMEM((T + 8, D), F32),
            pltpu.VMEM((T + 8, D), F32),
            pltpu.VMEM((T // 2, D), I32),
            pltpu.VMEM((T // 2, D), I32),
            pltpu.VMEM((T // 2, 256), I32),
            pltpu.VMEM((T // 2, 256), I32),
            pltpu.VMEM((T // 2, 256), I32),
            pltpu.VMEM((T // 2, 256), I32),
            pltpu.VMEM((NT, PADR, 128), F32),
            pltpu.VMEM((S, D), F32),
            pltpu.SemaphoreType.DMA((NCH,)),
            pltpu.SemaphoreType.DMA((4 * NT,)),
            pltpu.SemaphoreType.DMA((3 * NT,)),
            pltpu.SemaphoreType.DMA((2,)),
            pltpu.SemaphoreType.DMA((4,)),
            pltpu.SemaphoreType.DMA((7,)),
        ],
        compiler_params=pltpu.CompilerParams(vmem_limit_bytes=100 * 1024 * 1024),
    )(A_Lambda_re, A_Lambda_im, A_log_dt, A_Dskip, shkT, B_ssm_D, _ZMASK,
      x2, A_B_re, A_B_im, A_C_re, A_C_im, k2, v2, B_ssm_k, _FM, _GM)
    return out.reshape(1, S, D)
```
